```python
import jax
import jax.numpy as jnp

def _softmax(x, axis=-1):
    return jax.nn.softmax(x, axis=axis)
def _gelu(x):
    return jax.nn.gelu(x, approximate=True)
def _silu(x):
    return jax.nn.silu(x)
def _sigmoid(x):
    return jax.nn.sigmoid(x)
def _layernorm(x, axis=-1, eps=1e-5):
    m = jnp.mean(x, axis=axis, keepdims=True)
    v = jnp.var(x, axis=axis, keepdims=True)
    return (x - m) / jnp.sqrt(v + eps)
def _scatter_add(tgt, idx, src, axis=0):
    return tgt.at[idx].add(src)
def _segment_sum(src, seg, n):
    return jax.ops.segment_sum(src, seg, n)
class _Rng:
    def __init__(self, key):
        self._k = key
    def _next(self):
        self._k, sub = jax.random.split(self._k)
        return sub
    def normal(self, shape):
        return jax.random.normal(self._next(), shape, dtype=jnp.bfloat16)
    def randint(self, lo, hi, shape):
        return jax.random.randint(self._next(), shape, lo, hi, dtype=jnp.int32)
    def uniform(self, shape, lo=0.0, hi=1.0):
        return jax.random.uniform(self._next(), shape, jnp.bfloat16, lo, hi)
    def permutation(self, n):
        return jax.random.permutation(self._next(), n)


kernel_name = 'gated_mix__ssm_conv_h3__compressed_kv_cla__prompt'

def setup_inputs():
    _rng = _Rng(jax.random.key(int.from_bytes(__import__("os").urandom(4), "little")))
    _w = (lambda a: (lambda t: t.astype(jnp.bfloat16) if jnp.issubdtype(t.dtype, jnp.floating) else t)(jnp.asarray(a)))
    def _A_setup():
        B, S, D = 1, 2048, 1024
        ks = 4
        return {
            "q": _w((lambda *s: _rng.normal(s) * 0.05)(B, S, D)),
            "k": _w((lambda *s: _rng.normal(s) * 0.05)(B, S, D)),
            "v": _w((lambda *s: _rng.normal(s) * 0.05)(B, S, D)),
            "shift_k": _w((lambda *s: _rng.normal(s) * 0.05)(D, ks) * 0.5),
            "ssm_k": _w((lambda *s: _rng.normal(s) * 0.05)(D, S) * (1.0 / S ** 0.5)),
            "ssm_D": _w((lambda *s: _rng.normal(s) * 0.05)(D)),
        }
    _A_in = _A_setup()

    def _B_setup():
        B, H, Sq, Sk, D, M = 1, 32, 2048, 2048, 128, 1024
        Dc = 4 * D
        return {
            "x": _w((lambda *s: _rng.normal(s) * 0.05)(B, Sq, M)),
            "c_kv": _w((lambda *s: _rng.normal(s) * 0.05)(B, Sk, Dc)),
            "w_q": _w((lambda *s: _rng.normal(s) * 0.05)(M, H, D) * (M ** -0.5)),
            "w_uk": _w((lambda *s: _rng.normal(s) * 0.05)(Dc, H, D) * (Dc ** -0.5)),
            "w_uv": _w((lambda *s: _rng.normal(s) * 0.05)(Dc, H, D) * (Dc ** -0.5)),
            "w_o": _w((lambda *s: _rng.normal(s) * 0.05)(H, D, M) * ((H * D) ** -0.5)),
        }
    _B_in = _B_setup()

    return {
        "A_q": _A_in["q"],
        "A_k": _A_in["k"],
        "A_v": _A_in["v"],
        "A_shift_k": _A_in["shift_k"],
        "A_ssm_k": _A_in["ssm_k"],
        "A_ssm_D": _A_in["ssm_D"],
        "B_x": _B_in["x"],
        "B_c_kv": _B_in["c_kv"],
        "B_w_q": _B_in["w_q"],
        "B_w_uk": _B_in["w_uk"],
        "B_w_uv": _B_in["w_uv"],
        "B_w_o": _B_in["w_o"],
        "gate_w": _w((lambda *s: _rng.normal(s) * 0.05)(1024)),
    }

def reference(A_q, A_k, A_v, A_shift_k, A_ssm_k, A_ssm_D, B_x, B_c_kv, B_w_q, B_w_uk, B_w_uv, B_w_o, gate_w):
    def _A_ref(q, k, v, shift_k, ssm_k, ssm_D):
        B, S, D = q.shape
        ks = shift_k.shape[-1]
        k_pad = jnp.pad(k, ((0, 0), (ks - 1, 0), (0, 0)))
        k_shift = jnp.zeros_like(k)
        for t in range(ks):
            k_shift = k_shift + k_pad[:, t:t + S, :] * shift_k[:, ks - 1 - t][None, None, :]
        kv = k_shift * v
        L = 2 * S
        kv_pad = jnp.pad(kv, ((0, 0), (0, S), (0, 0)))
        kf_pad = jnp.pad(ssm_k, ((0, 0), (0, S)))
        kv_f = (lambda x, axes=(-2,-1): jnp.fft.rfft2(x.astype(jnp.float32), axes=axes))(kv_pad[:, None, :, :], axes=(1, 2))
        kf_f = (lambda x, axes=(-2,-1): jnp.fft.rfft2(x.astype(jnp.float32), axes=axes))(kf_pad[:, None, :], axes=(1, 2))
        kf_f = (lambda x, *d: x.transpose(*d))(kf_f, 1, 2, 0)
        y_f = kv_f * kf_f[None, :, :, :]
        y = (lambda x, s, axes=(-2,-1): jnp.fft.irfft2(x, s=s, axes=axes).astype(jnp.bfloat16))(y_f, (1, L), axes=(1, 2))[:, 0, :S, :]
        y = y + kv * ssm_D[None, None, :]
        return q * y

    def _B_ref(x, c_kv, w_q, w_uk, w_uv, w_o):
        B, Sq, M = x.shape[0], x.shape[1], x.shape[2]
        Sk = c_kv.shape[1]
        H, D = w_q.shape[1], w_q.shape[2]
        q = jnp.einsum("bqm,mhd->bhqd", x, w_q)
        k = jnp.einsum("bkc,chd->bhkd", c_kv, w_uk)
        v = jnp.einsum("bkc,chd->bhkd", c_kv, w_uv)
        scores = jnp.einsum("bhqd,bhkd->bhqk", q, k) * (D ** -0.5)
        off = Sk - Sq
        qi = jnp.arange(Sq)[:, None]
        kj = jnp.arange(Sk)[None, :]
        cmask = kj <= (qi + off)
        scores = jnp.where(cmask[None, None], scores, -1e9)
        p = _softmax(scores, axis=-1)
        ctx = jnp.einsum("bhqk,bhkd->bhqd", p, v)
        return jnp.einsum("bhqd,hdm->bqm", ctx, w_o)

    x = A_q
    g = _sigmoid((x * gate_w).sum(-1, keepdims=True))
    a = _A_ref(x, A_k, A_v, A_shift_k, A_ssm_k, A_ssm_D)
    b = _B_ref(x, B_c_kv, B_w_q, B_w_uk, B_w_uv, B_w_o)
    return g * a + (1 - g) * b
```

```python
import math

import jax
import jax.numpy as jnp
import numpy as np
from jax import lax
import jax.experimental.pallas as pl
import jax.experimental.pallas.tpu as pltpu

S = 2048
DM = 1024
H = 32
DH = 128
DC = 512
T = 128
NB = S // T
NC = DM // T
RB = 256
KG = 4

F32, BF16, U32 = jnp.float32, jnp.bfloat16, jnp.uint32
Q_SCALE = (DH ** -0.5) * math.log2(math.e)
NEG = -1e30
NT_DIMS = (((1,), (1,)), ((), ()))


def _dft_matrices():
    g = np.arange(16)[:, None]
    s = np.arange(8)[None, :]
    f = 2 * (8 * (g // 2) + s) + g % 2
    th = 2.0 * np.pi * (f[..., None] + 0.5) * np.arange(T) / (2 * T)
    fwd = np.stack([np.cos(th), -np.sin(th)], axis=1).reshape(2 * T, T)
    inv = np.stack([np.cos(th), -np.sin(th)], axis=2).reshape(2 * T, T).T / T
    return fwd.astype(BF16), np.ascontiguousarray(inv).astype(BF16)


_FWD, _INV = _dft_matrices()


def _bf(words):
    return pltpu.bitcast(words, BF16)


def _words(x):
    return pltpu.bitcast(x.astype(BF16), U32)


def _lo(words):
    return pltpu.bitcast(words << 16, F32)


def _hi(words):
    return pltpu.bitcast(words & jnp.uint32(0xFFFF0000), F32)


def _dot(a, b):
    return jnp.dot(a, b, preferred_element_type=F32)


def _kernel(x_hbm, k_hbm, v_hbm, sk_ref, h_hbm, d_ref, c_hbm, wq_hbm, wk_hbm, wv_hbm, wo_hbm,
            gw_ref, fwd_ref, inv_ref, out_hbm,
            xs32, cs32, w_raw, wo32, ks32, vs32, hs32,
            w_cur, q_buf, k_buf, v_buf, s_buf0, s_buf1, mx_buf, m_buf0, m_buf1, l_buf, o_buf,
            ctx, xh, hh, yp, shift_buf, f_buf, g_buf, out_buf,
            sem_x, sem_c, sem_w, sem_wo, sem_conv, sem_out):
    x_hbm, k_hbm, v_hbm, h_hbm, c_hbm, wq_hbm, wk_hbm, wv_hbm, wo_hbm = (
        r.bitcast(U32) for r in (x_hbm, k_hbm, v_hbm, h_hbm, c_hbm, wq_hbm, wk_hbm, wv_hbm, wo_hbm))
    s_bufs, m_bufs = (s_buf0, s_buf1), (m_buf0, m_buf1)
    HP = T // 2

    def lanes(j):
        return pl.ds(j * T, T)

    def rows32(i):
        return pl.ds(i * HP, HP)

    x_cp = [pltpu.make_async_copy(x_hbm.at[0, :, lanes(j)], xs32.at[j], sem_x.at[j]) for j in range(NC)]
    c_cp = [pltpu.make_async_copy(c_hbm.at[0, :, lanes(j)], cs32.at[j], sem_c.at[j])
            for j in range(DC // T)]
    wo_cp = [pltpu.make_async_copy(wo_hbm.at[:, lanes(j)], wo32.at[j], sem_wo.at[j]) for j in range(NC)]

    def w_cp(p):
        return [pltpu.make_async_copy(src.at[:, p, :], w_raw.at[p % 2, pl.ds(r0, n)], sem_w.at[p % 2, i])
                for i, (src, r0, n) in enumerate(
                    ((wq_hbm, 0, DM), (wk_hbm, DM, DC), (wv_hbm, DM + DC, DC)))]

    def conv_cp(c):
        col = pl.ds(pl.multiple_of(c * T, T), T)
        return (
            pltpu.make_async_copy(k_hbm.at[0, :, col], ks32.at[c, pl.ds(8, S // 2)], sem_conv.at[0, c]),
            pltpu.make_async_copy(v_hbm.at[0, :, col], vs32.at[c], sem_conv.at[1, c]),
            pltpu.make_async_copy(h_hbm.at[pl.ds(pl.multiple_of(c * HP, HP), HP)], hs32.at[c],
                                  sem_conv.at[2, c]),
        )

    def unpack_weights(h):
        slot = (h // 2) % 2
        sh = ((h % 2) * 16).astype(U32)
        for t in range(16):
            even = w_raw[slot, pl.ds(t * T, HP, stride=2), :]
            odd = w_raw[slot, pl.ds(t * T + 1, HP, stride=2), :]
            w_cur[t] = ((even >> sh) & jnp.uint32(0xFFFF)) | ((odd >> sh) << 16)

    def lhs_cat(src, i, j0, n):
        return jnp.concatenate([_bf(src[j0 + j, rows32(i), :]) for j in range(n)], axis=1)

    def w_cat(t0, n):
        return jnp.concatenate([_bf(w_cur[t0 + j]) for j in range(n)], axis=0)

    def proj_q(i):
        q = _dot(lhs_cat(xs32, i, 0, 4), w_cat(0, 4)) + _dot(lhs_cat(xs32, i, 4, 4), w_cat(4, 4))
        q_buf[i] = _words(q * Q_SCALE)

    def proj_k(i):
        k_buf[i] = _words(_dot(lhs_cat(cs32, i, 0, 4), w_cat(8, 4)))

    def proj_v(i):
        v_buf[i] = _words(_dot(lhs_cat(cs32, i, 0, 4), w_cat(12, 4)))

    def key_groups(i):
        return [(j0, min(KG, i + 1 - j0)) for j0 in range(0, i + 1, KG)]

    def scores(i, j0, n):
        kk = jnp.concatenate([_bf(k_buf[j0 + j]) for j in range(n)], axis=0)
        s = lax.dot_general(_bf(q_buf[i]), kk, NT_DIMS, preferred_element_type=F32)
        tiles = [s[:, j * T:(j + 1) * T] for j in range(n)]
        if j0 + n == i + 1:
            row = lax.broadcasted_iota(jnp.int32, (T, T), 0)
            col = lax.broadcasted_iota(jnp.int32, (T, T), 1)
            tiles[-1] = jnp.where(col <= row, tiles[-1], NEG)
        mx = None if j0 == 0 else mx_buf[...]
        for j, t in enumerate(tiles):
            s_bufs[i % 2][j0 + j] = t
            mx = t if mx is None else jnp.maximum(mx, t)
        if j0 + n == i + 1:
            m_bufs[i % 2][...] = jnp.broadcast_to(jnp.max(mx, axis=1, keepdims=True), (T, T))
        else:
            mx_buf[...] = mx

    def attend(h, i, j0, n):
        m = m_bufs[i % 2][...]
        l = None if j0 == 0 else l_buf[...]
        ps = []
        for j in range(n):
            p = jnp.exp2(s_bufs[i % 2][j0 + j] - m)
            l = p if l is None else l + p
            ps.append(p.astype(BF16))
        vv = jnp.concatenate([_bf(v_buf[j0 + j]) for j in range(n)], axis=0)
        o = _dot(jnp.concatenate(ps, axis=1), vv)
        if j0 > 0:
            o = o + o_buf[...]
        if j0 + n == i + 1:
            ctx[h, rows32(i), :] = _words(o / jnp.sum(l, axis=1, keepdims=True))
        else:
            l_buf[...] = l
            o_buf[...] = o

    def forward_x(c, a):
        r = pl.multiple_of(a * HP, HP)
        w0 = ks32[c, pl.ds(r + 8, HP), :]
        w1 = ks32[c, pl.ds(r + 7, HP), :]
        w2 = ks32[c, pl.ds(r + 6, HP), :]
        e0, o0, e1, o1, o2 = _lo(w0), _hi(w0), _lo(w1), _hi(w1), _hi(w2)
        s0, s1, s2, s3 = (shift_buf[c, j:j + 1, :] for j in range(4))
        even = s3 * o2 + s2 * e1 + s1 * o1 + s0 * e0
        odd = s3 * e1 + s2 * o1 + s1 * e0 + s0 * o0
        vw = vs32[c, pl.ds(r, HP), :]
        kv = pltpu.pack_elementwise([even * _lo(vw), odd * _hi(vw)], packed_dtype=BF16)
        return kv, _dot(_bf(f_buf[...]), _bf(kv))

    def forward_h(c, a):
        taps = _bf(hs32[c, :, pl.ds(pl.multiple_of(a * T, T), T)])
        return lax.dot_general(_bf(f_buf[...]), taps, NT_DIMS, preferred_element_type=F32)

    def product(c, par, g, odd, a0, prev):
        re = pl.ds(pl.multiple_of(g * 16, 8), 8)
        im = pl.ds(pl.multiple_of(g * 16 + 8, 8), 8)
        hcache = {}
        yr, yi = [None] * 4, [None] * 4
        for b in range(a0 + 3, -1, -1):
            xr, xi = xh[par, b, re, :], xh[par, b, im, :]
            for a in range(max(a0, b), a0 + 4):
                if a - b not in hcache:
                    hcache[a - b] = (hh[par, a - b, re, :], hh[par, a - b, im, :])
                hr, hi = hcache[a - b]
                pr, pi = hr * xr - hi * xi, hr * xi + hi * xr
                u = a - a0
                yr[u] = pr if yr[u] is None else yr[u] + pr
                yi[u] = pi if yi[u] is None else yi[u] + pi
        for u in range(4):
            zr, zi = yr[u], yi[u]
            if prev is not None:
                zr, zi = (zr + prev[1], zi - prev[0]) if odd else (zr - prev[1], zi + prev[0])
            yp[c, a0 + u, pl.ds(pl.multiple_of(g * 8, 8), 8), :] = pltpu.pack_elementwise(
                [zr, zi], packed_dtype=BF16)
            prev = (yr[u], yi[u])
        return prev

    for cp in c_cp + w_cp(0) + x_cp + list(conv_cp(0)) + list(conv_cp(1)):
        cp.start()
    f_buf[...] = pltpu.bitcast(fwd_ref[...], U32)
    ks32[:, 0:8, :] = jnp.zeros((NC, 8, T), U32)
    eye = (lax.broadcasted_iota(jnp.int32, (16, 4), 0) == lax.broadcasted_iota(jnp.int32, (16, 4), 1))
    sk_t = lax.dot_general(eye.astype(BF16), sk_ref[...], NT_DIMS, preferred_element_type=F32)
    for j in range(NC):
        shift_buf[j] = sk_t[0:8, j * T:(j + 1) * T]
    for cp in c_cp + w_cp(0) + x_cp:
        cp.wait()
    unpack_weights(jnp.int32(0))
    proj_q(0)
    proj_k(0)
    proj_q(1)
    proj_k(1)
    proj_v(0)
    scores(0, 0, 1)
    for cp in conv_cp(0):
        cp.wait()
    for a in range(NB):
        kv, spec = forward_x(0, a)
        vs32[0, rows32(a), :] = kv
        xh[0, a] = spec
        hh[0, a] = forward_h(0, a)
    for cp in wo_cp:
        cp.start()

    def head(h, carry):
        c, quarter = h // 4, h % 4
        cn = jnp.minimum(c + 1, NC - 1)

        @pl.when(quarter == 0)
        def _():
            @pl.when(c + 1 < NC)
            def _():
                for cp in conv_cp(cn):
                    cp.wait()

            @pl.when(c + 2 < NC)
            def _():
                for cp in conv_cp(jnp.minimum(c + 2, NC - 1)):
                    cp.start()

        @pl.when(jnp.logical_and(h % 2 == 0, h + 2 < H))
        def _():
            for cp in w_cp(h // 2 + 1):
                cp.start()

        @pl.when(jnp.logical_and(h % 2 == 1, h + 1 < H))
        def _():
            for cp in w_cp(jnp.minimum(h // 2 + 1, H // 2 - 1)):
                cp.wait()

        prev = None
        for i in range(NB):
            nxt = (i + 1) % NB
            qk, pv = key_groups(nxt), key_groups(i)
            if i == NB - 2:
                unpack_weights(jnp.minimum(h + 1, H - 1))
            for u in range(max(len(qk), len(pv))):
                if u < len(qk):
                    scores(nxt, *qk[u])
                if u < len(pv):
                    attend(h, i, *pv[u])
            proj_q((i + 2) % NB)
            proj_k((i + 2) % NB)
            proj_v(nxt)
            if i < 8:
                gi = i // 2
                for blk in (2 * (i % 2), 2 * (i % 2) + 1):
                    prev = product(c, c % 2, quarter * 4 + gi, gi % 2, 4 * blk, prev if blk else None)
            elif i < 12:
                a = quarter * 4 + i - 8
                hh[(c + 1) % 2, a] = forward_h(cn, a)
            else:
                a = quarter * 4 + i - 12
                kv, spec = forward_x(cn, a)
                xh[(c + 1) % 2, a] = spec
                vs32[c + 1, pl.ds(pl.multiple_of(a * HP, HP), HP), :] = kv
        return carry

    lax.fori_loop(0, H, head, 0)

    for cp in wo_cp:
        cp.wait()
    f_buf[:, :] = pltpu.bitcast(jnp.concatenate([inv_ref[:, :T], inv_ref[:, T:]], axis=0), U32)
    gate_w = gw_ref[...].astype(F32).reshape(1, DM)
    skip_d = d_ref[...].astype(F32).reshape(1, DM)
    for j in range(NC):
        shift_buf[j, 0:1, :] = gate_w[:, j * T:(j + 1) * T]
        shift_buf[j, 1:2, :] = skip_d[:, j * T:(j + 1) * T]

    def out_cp(r, slot):
        return pltpu.make_async_copy(
            out_buf.at[slot], out_hbm.at[0, pl.ds(pl.multiple_of(r * RB, RB), RB), :], sem_out.at[slot])

    def mix(r, carry):
        slot = r % 2
        rp = pl.ds(pl.multiple_of(r * (RB // 2), RB // 2), RB // 2)

        @pl.when(r >= 2)
        def _():
            out_cp(r - 2, slot).wait()

        logit = None
        for j in range(NC):
            t = _bf(xs32[j, rp, :]).astype(F32) * shift_buf[j, 0:1, :]
            logit = t if logit is None else logit + t
        gate = 1.0 / (1.0 + jnp.exp(-jnp.sum(logit, axis=1, keepdims=True)))
        g_buf[...] = jnp.broadcast_to(gate, (RB, T))
        inv = jnp.concatenate([_bf(f_buf[0:HP, :]), _bf(f_buf[HP:T, :])], axis=1)
        for j in range(NC):
            b = None
            for h0 in range(0, H, 4):
                lhs = jnp.concatenate([_bf(ctx[h0 + u, rp, :]) for u in range(4)], axis=1)
                t = _dot(lhs, _bf(wo32[j, pl.ds(h0 * HP, 4 * HP), :]))
                b = t if b is None else b + t
            y = jnp.concatenate(
                [_dot(inv, _bf(yp[j, r * (RB // T) + u])) for u in range(RB // T)], axis=0)
            kv = _bf(vs32[j, rp, :]).astype(F32)
            a = _bf(xs32[j, rp, :]).astype(F32) * (y + kv * shift_buf[j, 1:2, :])
            g = g_buf[...]
            out_buf[slot, :, lanes(j)] = (g * a + (1.0 - g) * b).astype(BF16)
        out_cp(r, slot).start()
        return carry

    lax.fori_loop(0, S // RB, mix, 0)
    for r in (S // RB - 2, S // RB - 1):
        out_cp(r, r % 2).wait()


@jax.jit
def pallas_gated_mix__ssm_conv_h3__compressed_kv_cla__prompt_kernel(
    A_q, A_k, A_v, A_shift_k, A_ssm_k, A_ssm_D, B_x, B_c_kv, B_w_q, B_w_uk, B_w_uv, B_w_o, gate_w,
):
    del B_x
    hbm = pl.BlockSpec(memory_space=pl.ANY)
    vmem = pl.BlockSpec(memory_space=pltpu.VMEM)
    HP = T // 2
    scratch = [
        pltpu.VMEM((NC, S // 2, T), U32),
        pltpu.VMEM((DC // T, S // 2, T), U32),
        pltpu.VMEM((2, DM + 2 * DC, T), U32),
        pltpu.VMEM((NC, H * HP, T), U32),
        pltpu.VMEM((NC, 8 + S // 2, T), U32),
        pltpu.VMEM((NC + 1, S // 2, T), U32),
        pltpu.VMEM((NC, HP, S), U32),
        pltpu.VMEM((16, HP, T), U32),
        pltpu.VMEM((NB, HP, T), U32),
        pltpu.VMEM((NB, HP, T), U32),
        pltpu.VMEM((NB, HP, T), U32),
        pltpu.VMEM((NB, T, T), F32),
        pltpu.VMEM((NB, T, T), F32),
        pltpu.VMEM((T, T), F32),
        pltpu.VMEM((T, T), F32),
        pltpu.VMEM((T, T), F32),
        pltpu.VMEM((T, T), F32),
        pltpu.VMEM((T, T), F32),
        pltpu.VMEM((H, S // 2, T), U32),
        pltpu.VMEM((2, NB, 2 * T, T), F32),
        pltpu.VMEM((2, NB, 2 * T, T), F32),
        pltpu.VMEM((NC, NB, T, T), U32),
        pltpu.VMEM((NC, 8, T), F32),
        pltpu.VMEM((T, T), U32),
        pltpu.VMEM((RB, T), F32),
        pltpu.VMEM((2, RB, DM), BF16),
        pltpu.SemaphoreType.DMA((NC,)),
        pltpu.SemaphoreType.DMA((DC // T,)),
        pltpu.SemaphoreType.DMA((2, 3)),
        pltpu.SemaphoreType.DMA((NC,)),
        pltpu.SemaphoreType.DMA((3, NC)),
        pltpu.SemaphoreType.DMA((2,)),
    ]
    return pl.pallas_call(
        _kernel,
        out_shape=jax.ShapeDtypeStruct((1, S, DM), BF16),
        in_specs=[hbm, hbm, hbm, vmem, hbm, vmem, hbm, hbm, hbm, hbm, hbm, vmem, vmem, vmem],
        out_specs=hbm,
        scratch_shapes=scratch,
        compiler_params=pltpu.CompilerParams(vmem_limit_bytes=110 * 1024 * 1024),
        name="gated_mix_h3_cla",
    )(
        A_q, A_k, A_v, A_shift_k, A_ssm_k, A_ssm_D, B_c_kv,
        B_w_q, B_w_uk, B_w_uv, B_w_o.reshape(H * DH, DM), gate_w, _FWD, _INV,
    )
```

```python
import math

import jax
import jax.numpy as jnp
import numpy as np
from jax import lax
import jax.experimental.pallas as pl
import jax.experimental.pallas.tpu as pltpu

S = 2048
DM = 1024
H = 32
DH = 128
DC = 512
T = 128
NB = S // T
NC = DM // T
RB = 256
KG = 4

F32, BF16, U32 = jnp.float32, jnp.bfloat16, jnp.uint32
Q_SCALE = (DH ** -0.5) * math.log2(math.e)
NEG = -1e30
NT_DIMS = (((1,), (1,)), ((), ()))


def _dft_matrices():
    g = np.arange(16)[:, None]
    s = np.arange(8)[None, :]
    f = 2 * (8 * (g // 2) + s) + g % 2
    th = 2.0 * np.pi * (f[..., None] + 0.5) * np.arange(T) / (2 * T)
    fwd = np.stack([np.cos(th), -np.sin(th)], axis=1).reshape(2 * T, T)
    inv = np.stack([np.cos(th), -np.sin(th)], axis=2).reshape(2 * T, T).T / T
    return fwd.astype(BF16), np.ascontiguousarray(inv).astype(BF16)


_FWD, _INV = _dft_matrices()


def _bf(words):
    return pltpu.bitcast(words, BF16)


def _words(x):
    return pltpu.bitcast(x.astype(BF16), U32)


def _lo(words):
    return pltpu.bitcast(words << 16, F32)


def _hi(words):
    return pltpu.bitcast(words & jnp.uint32(0xFFFF0000), F32)


def _dot(a, b):
    return jnp.dot(a, b, preferred_element_type=F32)


def _kernel(x_hbm, k_hbm, v_hbm, sk_ref, h_hbm, d_ref, c_hbm, wq_hbm, wk_hbm, wv_hbm, wo_hbm,
            gw_ref, fwd_ref, inv_ref, out_hbm,
            xs32, cs32, w_raw, wo32, ks32, vs32, hs32,
            w_cur, q_buf, k_buf, v_buf, s_buf0, s_buf1, mx_buf, m_buf0, m_buf1, l_buf, o_buf,
            ctx, xh, hh, yp, shift_buf, f_buf, g_buf, out_buf,
            sem_x, sem_c, sem_w, sem_wo, sem_conv, sem_out):
    x_hbm, k_hbm, v_hbm, h_hbm, c_hbm, wq_hbm, wk_hbm, wv_hbm, wo_hbm = (
        r.bitcast(U32) for r in (x_hbm, k_hbm, v_hbm, h_hbm, c_hbm, wq_hbm, wk_hbm, wv_hbm, wo_hbm))
    s_bufs, m_bufs = (s_buf0, s_buf1), (m_buf0, m_buf1)
    HP = T // 2

    def lanes(j):
        return pl.ds(j * T, T)

    def rows32(i):
        return pl.ds(i * HP, HP)

    x_cp = [pltpu.make_async_copy(x_hbm.at[0, :, lanes(j)], xs32.at[j], sem_x.at[j]) for j in range(NC)]
    c_cp = [pltpu.make_async_copy(c_hbm.at[0, :, lanes(j)], cs32.at[j], sem_c.at[j])
            for j in range(DC // T)]
    wo_cp = [pltpu.make_async_copy(wo_hbm.at[:, lanes(j)], wo32.at[j], sem_wo.at[j]) for j in range(NC)]

    def w_cp(p):
        return [pltpu.make_async_copy(src.at[:, p, :], w_raw.at[p % 2, pl.ds(r0, n)], sem_w.at[p % 2, i])
                for i, (src, r0, n) in enumerate(
                    ((wq_hbm, 0, DM), (wk_hbm, DM, DC), (wv_hbm, DM + DC, DC)))]

    def conv_cp(c):
        col = pl.ds(pl.multiple_of(c * T, T), T)
        return (
            pltpu.make_async_copy(k_hbm.at[0, :, col], ks32.at[c, pl.ds(8, S // 2)], sem_conv.at[0, c]),
            pltpu.make_async_copy(v_hbm.at[0, :, col], vs32.at[c], sem_conv.at[1, c]),
            pltpu.make_async_copy(h_hbm.at[pl.ds(pl.multiple_of(c * HP, HP), HP)], hs32.at[c],
                                  sem_conv.at[2, c]),
        )

    def unpack_weights(h, tiles):
        slot = (h // 2) % 2
        sh = ((h % 2) * 16).astype(U32)
        for t in tiles:
            even = w_raw[slot, pl.ds(t * T, HP, stride=2), :]
            odd = w_raw[slot, pl.ds(t * T + 1, HP, stride=2), :]
            w_cur[t] = ((even >> sh) & jnp.uint32(0xFFFF)) | ((odd >> sh) << 16)

    def lhs_cat(src, i, j0, n):
        return jnp.concatenate([_bf(src[j0 + j, rows32(i), :]) for j in range(n)], axis=1)

    def w_cat(t0, n):
        return jnp.concatenate([_bf(w_cur[t0 + j]) for j in range(n)], axis=0)

    def proj_q(i):
        q = _dot(lhs_cat(xs32, i, 0, 4), w_cat(0, 4)) + _dot(lhs_cat(xs32, i, 4, 4), w_cat(4, 4))
        q_buf[i] = _words(q * Q_SCALE)

    def proj_k(i):
        k_buf[i] = _words(_dot(lhs_cat(cs32, i, 0, 4), w_cat(8, 4)))

    def proj_v(i):
        v_buf[i] = _words(_dot(lhs_cat(cs32, i, 0, 4), w_cat(12, 4)))

    def key_groups(i):
        return [(j0, min(KG, i + 1 - j0)) for j0 in range(0, i + 1, KG)]

    def scores(i, j0, n):
        kk = jnp.concatenate([_bf(k_buf[j0 + j]) for j in range(n)], axis=0)
        s = lax.dot_general(_bf(q_buf[i]), kk, NT_DIMS, preferred_element_type=F32)
        tiles = [s[:, j * T:(j + 1) * T] for j in range(n)]
        if j0 + n == i + 1:
            row = lax.broadcasted_iota(jnp.int32, (T, T), 0)
            col = lax.broadcasted_iota(jnp.int32, (T, T), 1)
            tiles[-1] = jnp.where(col <= row, tiles[-1], NEG)
        mx = None if j0 == 0 else mx_buf[...]
        for j, t in enumerate(tiles):
            s_bufs[i % 2][j0 + j] = t
            mx = t if mx is None else jnp.maximum(mx, t)
        if j0 + n == i + 1:
            m_bufs[i % 2][...] = jnp.broadcast_to(jnp.max(mx, axis=1, keepdims=True), (T, T))
        else:
            mx_buf[...] = mx

    def attend(h, i, j0, n):
        m = m_bufs[i % 2][...]
        l = None if j0 == 0 else l_buf[...]
        ps = []
        for j in range(n):
            p = jnp.exp2(s_bufs[i % 2][j0 + j] - m)
            l = p if l is None else l + p
            ps.append(p.astype(BF16))
        vv = jnp.concatenate([_bf(v_buf[j0 + j]) for j in range(n)], axis=0)
        o = _dot(jnp.concatenate(ps, axis=1), vv)
        if j0 > 0:
            o = o + o_buf[...]
        if j0 + n == i + 1:
            ctx[h, rows32(i), :] = _words(o / jnp.sum(l, axis=1, keepdims=True))
        else:
            l_buf[...] = l
            o_buf[...] = o

    def forward_x(c, a):
        r = pl.multiple_of(a * HP, HP)
        w0 = ks32[c, pl.ds(r + 8, HP), :]
        w1 = ks32[c, pl.ds(r + 7, HP), :]
        w2 = ks32[c, pl.ds(r + 6, HP), :]
        e0, o0, e1, o1, o2 = _lo(w0), _hi(w0), _lo(w1), _hi(w1), _hi(w2)
        s0, s1, s2, s3 = (shift_buf[c, j:j + 1, :] for j in range(4))
        even = s3 * o2 + s2 * e1 + s1 * o1 + s0 * e0
        odd = s3 * e1 + s2 * o1 + s1 * e0 + s0 * o0
        vw = vs32[c, pl.ds(r, HP), :]
        kv = pltpu.pack_elementwise([even * _lo(vw), odd * _hi(vw)], packed_dtype=BF16)
        return kv, _dot(_bf(f_buf[...]), _bf(kv))

    def forward_h(c, a):
        taps = _bf(hs32[c, :, pl.ds(pl.multiple_of(a * T, T), T)])
        return lax.dot_general(_bf(f_buf[...]), taps, NT_DIMS, preferred_element_type=F32)

    def product(c, par, g, odd, a0, prev):
        re = pl.ds(pl.multiple_of(g * 16, 8), 8)
        im = pl.ds(pl.multiple_of(g * 16 + 8, 8), 8)
        hcache = {}
        yr, yi = [None] * 4, [None] * 4
        for b in range(a0 + 3, -1, -1):
            xr, xi = xh[par, b, re, :], xh[par, b, im, :]
            for a in range(max(a0, b), a0 + 4):
                if a - b not in hcache:
                    hcache[a - b] = (hh[par, a - b, re, :], hh[par, a - b, im, :])
                hr, hi = hcache[a - b]
                pr, pi = hr * xr - hi * xi, hr * xi + hi * xr
                u = a - a0
                yr[u] = pr if yr[u] is None else yr[u] + pr
                yi[u] = pi if yi[u] is None else yi[u] + pi
        for u in range(4):
            zr, zi = yr[u], yi[u]
            if prev is not None:
                zr, zi = (zr + prev[1], zi - prev[0]) if odd else (zr - prev[1], zi + prev[0])
            yp[c, a0 + u, pl.ds(pl.multiple_of(g * 8, 8), 8), :] = pltpu.pack_elementwise(
                [zr, zi], packed_dtype=BF16)
            prev = (yr[u], yi[u])
        return prev

    for cp in c_cp + w_cp(0) + x_cp + list(conv_cp(0)) + list(conv_cp(1)):
        cp.start()
    f_buf[...] = pltpu.bitcast(fwd_ref[...], U32)
    ks32[:, 0:8, :] = jnp.zeros((NC, 8, T), U32)
    shift_taps = sk_ref[...].astype(F32)
    for j in range(NC):
        shift_buf[j, 0:4, :] = shift_taps[:, j * T:(j + 1) * T]
    for cp in c_cp + w_cp(0) + x_cp:
        cp.wait()
    unpack_weights(jnp.int32(0), range(16))
    proj_q(0)
    proj_k(0)
    proj_q(1)
    proj_k(1)
    proj_v(0)
    scores(0, 0, 1)
    for cp in conv_cp(0):
        cp.wait()
    for a in range(NB):
        kv, spec = forward_x(0, a)
        vs32[0, rows32(a), :] = kv
        xh[0, a] = spec
        hh[0, a] = forward_h(0, a)
    for cp in wo_cp:
        cp.start()

    def head(h, carry):
        c, quarter = h // 4, h % 4
        cn = jnp.minimum(c + 1, NC - 1)

        @pl.when(quarter == 0)
        def _():
            @pl.when(c + 1 < NC)
            def _():
                for cp in conv_cp(cn):
                    cp.wait()

            @pl.when(c + 2 < NC)
            def _():
                for cp in conv_cp(jnp.minimum(c + 2, NC - 1)):
                    cp.start()

        @pl.when(jnp.logical_and(h % 2 == 0, h + 2 < H))
        def _():
            for cp in w_cp(h // 2 + 1):
                cp.start()

        @pl.when(jnp.logical_and(h % 2 == 1, h + 1 < H))
        def _():
            for cp in w_cp(jnp.minimum(h // 2 + 1, H // 2 - 1)):
                cp.wait()

        prev = None
        for i in range(NB):
            nxt = (i + 1) % NB
            qk, pv = key_groups(nxt), key_groups(i)
            if i == NB - 2:
                unpack_weights(jnp.minimum(h + 1, H - 1), range(12))
            if i == NB - 1:
                unpack_weights(jnp.minimum(h + 1, H - 1), range(12, 16))
            for u in range(max(len(qk), len(pv))):
                if u < len(qk):
                    scores(nxt, *qk[u])
                if u < len(pv):
                    attend(h, i, *pv[u])
            proj_q((i + 2) % NB)
            proj_k((i + 2) % NB)
            proj_v(nxt)
            if i < 8:
                gi = i // 2
                for blk in (2 * (i % 2), 2 * (i % 2) + 1):
                    prev = product(c, c % 2, quarter * 4 + gi, gi % 2, 4 * blk, prev if blk else None)
            elif i < 12:
                a = quarter * 4 + i - 8
                hh[(c + 1) % 2, a] = forward_h(cn, a)
            else:
                a = quarter * 4 + i - 12
                kv, spec = forward_x(cn, a)
                xh[(c + 1) % 2, a] = spec
                vs32[c + 1, pl.ds(pl.multiple_of(a * HP, HP), HP), :] = kv
        return carry

    lax.fori_loop(0, H, head, 0)

    for cp in wo_cp:
        cp.wait()
    f_buf[:, :] = pltpu.bitcast(jnp.concatenate([inv_ref[:, :T], inv_ref[:, T:]], axis=0), U32)
    gate_w = gw_ref[...].astype(F32).reshape(1, DM)
    skip_d = d_ref[...].astype(F32).reshape(1, DM)
    for j in range(NC):
        shift_buf[j, 0:1, :] = gate_w[:, j * T:(j + 1) * T]
        shift_buf[j, 1:2, :] = skip_d[:, j * T:(j + 1) * T]

    def out_cp(r, slot):
        return pltpu.make_async_copy(
            out_buf.at[slot], out_hbm.at[0, pl.ds(pl.multiple_of(r * RB, RB), RB), :], sem_out.at[slot])

    def mix(r, carry):
        slot = r % 2
        rp = pl.ds(pl.multiple_of(r * (RB // 2), RB // 2), RB // 2)

        @pl.when(r >= 2)
        def _():
            out_cp(r - 2, slot).wait()

        logit = None
        for j in range(NC):
            t = _bf(xs32[j, rp, :]).astype(F32) * shift_buf[j, 0:1, :]
            logit = t if logit is None else logit + t
        gate = 1.0 / (1.0 + jnp.exp(-jnp.sum(logit, axis=1, keepdims=True)))
        g_buf[...] = jnp.broadcast_to(gate, (RB, T))
        inv = jnp.concatenate([_bf(f_buf[0:HP, :]), _bf(f_buf[HP:T, :])], axis=1)
        for j in range(NC):
            b = None
            for h0 in range(0, H, 4):
                lhs = jnp.concatenate([_bf(ctx[h0 + u, rp, :]) for u in range(4)], axis=1)
                t = _dot(lhs, _bf(wo32[j, pl.ds(h0 * HP, 4 * HP), :]))
                b = t if b is None else b + t
            y = jnp.concatenate(
                [_dot(inv, _bf(yp[j, r * (RB // T) + u])) for u in range(RB // T)], axis=0)
            kv = _bf(vs32[j, rp, :]).astype(F32)
            a = _bf(xs32[j, rp, :]).astype(F32) * (y + kv * shift_buf[j, 1:2, :])
            g = g_buf[...]
            out_buf[slot, :, lanes(j)] = (g * a + (1.0 - g) * b).astype(BF16)
        out_cp(r, slot).start()
        return carry

    lax.fori_loop(0, S // RB, mix, 0)
    for r in (S // RB - 2, S // RB - 1):
        out_cp(r, r % 2).wait()


@jax.jit
def pallas_gated_mix__ssm_conv_h3__compressed_kv_cla__prompt_kernel(
    A_q, A_k, A_v, A_shift_k, A_ssm_k, A_ssm_D, B_x, B_c_kv, B_w_q, B_w_uk, B_w_uv, B_w_o, gate_w,
):
    del B_x
    hbm = pl.BlockSpec(memory_space=pl.ANY)
    vmem = pl.BlockSpec(memory_space=pltpu.VMEM)
    HP = T // 2
    scratch = [
        pltpu.VMEM((NC, S // 2, T), U32),
        pltpu.VMEM((DC // T, S // 2, T), U32),
        pltpu.VMEM((2, DM + 2 * DC, T), U32),
        pltpu.VMEM((NC, H * HP, T), U32),
        pltpu.VMEM((NC, 8 + S // 2, T), U32),
        pltpu.VMEM((NC + 1, S // 2, T), U32),
        pltpu.VMEM((NC, HP, S), U32),
        pltpu.VMEM((16, HP, T), U32),
        pltpu.VMEM((NB, HP, T), U32),
        pltpu.VMEM((NB, HP, T), U32),
        pltpu.VMEM((NB, HP, T), U32),
        pltpu.VMEM((NB, T, T), F32),
        pltpu.VMEM((NB, T, T), F32),
        pltpu.VMEM((T, T), F32),
        pltpu.VMEM((T, T), F32),
        pltpu.VMEM((T, T), F32),
        pltpu.VMEM((T, T), F32),
        pltpu.VMEM((T, T), F32),
        pltpu.VMEM((H, S // 2, T), U32),
        pltpu.VMEM((2, NB, 2 * T, T), F32),
        pltpu.VMEM((2, NB, 2 * T, T), F32),
        pltpu.VMEM((NC, NB, T, T), U32),
        pltpu.VMEM((NC, 8, T), F32),
        pltpu.VMEM((T, T), U32),
        pltpu.VMEM((RB, T), F32),
        pltpu.VMEM((2, RB, DM), BF16),
        pltpu.SemaphoreType.DMA((NC,)),
        pltpu.SemaphoreType.DMA((DC // T,)),
        pltpu.SemaphoreType.DMA((2, 3)),
        pltpu.SemaphoreType.DMA((NC,)),
        pltpu.SemaphoreType.DMA((3, NC)),
        pltpu.SemaphoreType.DMA((2,)),
    ]
    return pl.pallas_call(
        _kernel,
        out_shape=jax.ShapeDtypeStruct((1, S, DM), BF16),
        in_specs=[hbm, hbm, hbm, vmem, hbm, vmem, hbm, hbm, hbm, hbm, hbm, vmem, vmem, vmem],
        out_specs=hbm,
        scratch_shapes=scratch,
        compiler_params=pltpu.CompilerParams(vmem_limit_bytes=110 * 1024 * 1024),
        name="gated_mix_h3_cla",
    )(
        A_q, A_k, A_v, A_shift_k.T, A_ssm_k, A_ssm_D, B_c_kv,
        B_w_q, B_w_uk, B_w_uv, B_w_o.reshape(H * DH, DM), gate_w, _FWD, _INV,
    )
```

```python
import functools
import math

import jax
import jax.numpy as jnp
import numpy as np
from jax import lax
import jax.experimental.pallas as pl
import jax.experimental.pallas.tpu as pltpu

S = 2048
DM = 1024
H = 32
DH = 128
DC = 512
T = 128
NB = S // T
NC = DM // T
RB = 256
KG = 4

HP = T // 2
PIN_OFF = NB * T
RES_OFF = PIN_OFF + 4 * 8
K_PITCH = 8 + S // 2

import os
CFG = dict(lp=1, order=1, lag=5, prod=1, fwd=1, dmapos=15, nobc=1, pin=1, pb=4, where=0)
CFG.update({k: int(v) for k, v in (kv.split("=") for kv in os.environ.get("KCFG", "").split(",") if kv)})

F32, BF16, U32 = jnp.float32, jnp.bfloat16, jnp.uint32
Q_SCALE = (DH ** -0.5) * math.log2(math.e)
NEG = -1e30
NT_DIMS = (((1,), (1,)), ((), ()))


def _dft_matrices():
    g = np.arange(16)[:, None]
    s = np.arange(8)[None, :]
    f = 2 * (8 * (g // 2) + s) + g % 2
    th = 2.0 * np.pi * (f[..., None] + 0.5) * np.arange(T) / (2 * T)
    fwd = np.stack([np.cos(th), -np.sin(th)], axis=1).reshape(2 * T, T)
    inv = np.stack([np.cos(th), -np.sin(th)], axis=2).reshape(2 * T, T).T / T
    return fwd.astype(BF16), np.ascontiguousarray(inv).astype(BF16)


_FWD, _INV = _dft_matrices()


def _bf(words):
    return pltpu.bitcast(words, BF16)


def _lo(words):
    return pltpu.bitcast(words << 16, F32)


def _hi(words):
    return pltpu.bitcast(words & jnp.uint32(0xFFFF0000), F32)


def _dot(a, b):
    return jnp.dot(a, b, preferred_element_type=F32)


def _key_groups(i):
    return [(j0, min(KG, i + 1 - j0)) for j0 in range(0, i + 1, KG)]


def _head_program():
    steps = []
    for i in range(NB):
        nxt = (i + 1) % NB
        sc = [("scores", nxt) + grp for grp in _key_groups(nxt)]
        at = [("attend", i) + grp for grp in _key_groups(i)]
        q, k, v = ("q", (i + 2) % NB), ("k", (i + 2) % NB), ("v", nxt)
        rnd = [x for u in range(4) for x in sc[u:u + 1] + at[u:u + 1]]
        if i < NB - 2:
            if CFG["order"] == 0:
                rnd = [q, k, v] + rnd
            else:
                rnd = [q] + rnd[:1] + [k] + rnd[1:3] + [v] + rnd[3:]
            rnd.append(("max", nxt))
        elif i == NB - 2:
            rnd = [v] + rnd + [("max", nxt), q, k]
        else:
            rnd = [at[0], q, at[1], k, at[2], sc[0], at[3], v, ("max", nxt)]
        steps += rnd[:1] + [("weights", i)] + rnd[1:]
        if i == CFG["dmapos"]:
            steps.append(("dma", i))
    return steps


def _kernel(x_hbm, k_hbm, v_hbm, sk_ref, h_hbm, d_ref, c_hbm, wq_hbm, wk_hbm, wv_hbm, wo_hbm,
            gw_ref, fwd_ref, inv_ref, out_hbm,
            xs32, cs32, w_raw, wo32, ks32, vs32, hs32, spec, w_cur, buf0, buf1, mx_buf, l_buf, o_buf,
            ctx, shift_buf, f_buf, g_buf, out_buf,
            sem_x, sem_c, sem_w, sem_wo, sem_conv, sem_out, *qkv):
    q_buf, k_buf, v_buf = qkv[:NB], qkv[NB:2 * NB], qkv[2 * NB:]
    x_hbm, k_hbm, v_hbm, h_hbm, c_hbm, wq_hbm, wk_hbm, wv_hbm, wo_hbm = (
        r.bitcast(U32) for r in (x_hbm, k_hbm, v_hbm, h_hbm, c_hbm, wq_hbm, wk_hbm, wv_hbm, wo_hbm))
    bufs = (buf0, buf1)
    ctx32, m_buf = ctx.bitcast(U32), ctx.bitcast(F32)
    M_OFF = H * S // 2

    def lanes(j):
        return pl.ds(j * T, T)

    def rows8(start, n):
        return pl.ds(start if isinstance(start, int) else pl.multiple_of(start, 8), n)

    def load_f32(buf, start, n):
        return pltpu.bitcast(buf[rows8(start, n), :], F32)

    def store_f32(buf, start, value):
        buf[rows8(start, value.shape[0]), :] = pltpu.bitcast(value, U32)

    x_cp = [pltpu.make_async_copy(x_hbm.at[0, :, lanes(j)], xs32.at[j], sem_x.at[j]) for j in range(NC)]
    c_cp = [pltpu.make_async_copy(c_hbm.at[0, :, lanes(j)], cs32.at[j], sem_c.at[j])
            for j in range(DC // T)]
    wo_cp = [pltpu.make_async_copy(wo_hbm.at[:, lanes(j)], wo32.at[j], sem_wo.at[j]) for j in range(NC)]

    def w_cp(p):
        return [pltpu.make_async_copy(src.at[:, p, :], w_raw.at[p & 1, pl.ds(r0, n)], sem_w.at[p & 1, i])
                for i, (src, r0, n) in enumerate(
                    ((wq_hbm, 0, DM), (wk_hbm, DM, DC), (wv_hbm, DM + DC, DC)))]

    def conv_cp(c):
        col = pl.ds(pl.multiple_of(c * T, T), T)
        return (
            pltpu.make_async_copy(k_hbm.at[0, :, col], ks32.at[c, pl.ds(8, S // 2)], sem_conv.at[0, c]),
            pltpu.make_async_copy(v_hbm.at[0, :, col], vs32.at[c], sem_conv.at[1, c]),
            pltpu.make_async_copy(h_hbm.at[pl.ds(pl.multiple_of(c * HP, HP), HP)], hs32.at[c],
                                  sem_conv.at[2, c]),
        )

    def unpack_weights(h, t):
        slot = (h >> 1) & 1
        sh = ((h & 1) * 16).astype(U32)
        even = w_raw[slot, pl.ds(t * T, HP, stride=2), :]
        odd = w_raw[slot, pl.ds(t * T + 1, HP, stride=2), :]
        return ((even >> sh) & jnp.uint32(0xFFFF)) | ((odd >> sh) << 16)

    def lhs_cat(src, i, j0, n):
        return jnp.concatenate([_bf(src[j0 + j, pl.ds(i * HP, HP), :]) for j in range(n)], axis=1)

    def w_cat(h, t0, n):
        return _bf(w_cur[h & 1, pl.ds(t0 * HP, n * HP), :])

    def proj_q(z, h, i):
        q = _dot(lhs_cat(xs32, i, 0, 4), w_cat(h, 0, 4)) + _dot(lhs_cat(xs32, i, 4, 4), w_cat(h, 4, 4))
        q_buf[i][z] = (q * Q_SCALE).astype(BF16)

    def proj_k(z, h, i):
        k_buf[i][z] = _dot(lhs_cat(cs32, i, 0, 4), w_cat(h, 8, 4)).astype(BF16)

    def proj_v(z, h, i):
        v_buf[i][z] = _dot(lhs_cat(cs32, i, 0, 4), w_cat(h, 12, 4)).astype(BF16)

    def tiles_of(buf, j0, n):
        return _bf(jnp.concatenate([buf[j0 + j].bitcast(U32)[0] for j in range(n)], axis=0))

    def scores(z, i, j0, n):
        s = lax.dot_general(tiles_of(q_buf, i, 1), tiles_of(k_buf, j0, n), NT_DIMS,
                            preferred_element_type=F32)
        tiles = [s[:, j * T:(j + 1) * T] for j in range(n)]
        if j0 + n == i + 1:
            row = lax.broadcasted_iota(jnp.int32, (T, T), 0)
            col = lax.broadcasted_iota(jnp.int32, (T, T), 1)
            tiles[-1] = jnp.where(col <= row, tiles[-1], NEG)
        mx = None if j0 == 0 else mx_buf[...]
        for j, t in enumerate(tiles):
            store_f32(bufs[i % 2], z + (j0 + j) * T, t)
            mx = t if mx is None else jnp.maximum(mx, t)
        mx_buf[...] = mx

    def row_max(z, i):
        m_buf[rows8(z + M_OFF + i % 2 * T, T), :] = jnp.broadcast_to(
            jnp.max(mx_buf[...], axis=1, keepdims=True), (T, T))

    def attend(h, i, j0, n):
        m = m_buf[rows8(M_OFF + i % 2 * T, T), :]
        l = None if j0 == 0 else l_buf[...]
        ps = []
        for j in range(n):
            p = jnp.exp2(load_f32(bufs[i % 2], (j0 + j) * T, T) - m)
            l = p if l is None else l + p
            ps.append(p)
        o = _dot(jnp.concatenate(ps, axis=1).astype(BF16), tiles_of(v_buf, j0, n))
        if j0 > 0:
            o = o + o_buf[...]
        if j0 + n == i + 1:
            total = jnp.sum(l, axis=1, keepdims=True)
            r = pl.reciprocal(total, approx=True)
            r = r * (2.0 - total * r)
            ctx[pl.ds(pl.multiple_of(h * S + i * T, T), T), :] = (o * r).astype(BF16)
        else:
            l_buf[...] = l
            o_buf[...] = o

    def gate_kv(c, c_out, r8, n):
        r = r8 * 8
        w0, w1, w2 = ks32[c, rows8(r + 8, n), :], ks32[c, pl.ds(r + 7, n), :], ks32[c, pl.ds(r + 6, n), :]
        e0, o0, e1, o1, o2 = _lo(w0), _hi(w0), _lo(w1), _hi(w1), _hi(w2)
        s0, s1, s2, s3 = (shift_buf[c, j:j + 1, :] for j in range(4))
        even = s3 * o2 + s2 * e1 + s1 * o1 + s0 * e0
        odd = s3 * e1 + s2 * o1 + s1 * e0 + s0 * o0
        vw = vs32[c, rows8(r, n), :]
        buf1[rows8(RES_OFF + c_out * (S // 2) + r, n), :] = pltpu.pack_elementwise(
            [even * _lo(vw), odd * _hi(vw)], packed_dtype=BF16)

    def forward_x(c, a):
        return _dot(_bf(f_buf[...]), _bf(buf1[rows8(RES_OFF + c * (S // 2) + a * HP, HP), :]))

    def forward_h(c, a):
        taps = _bf(hs32[c, :, pl.ds(pl.multiple_of(a * T, T), T)])
        return lax.dot_general(_bf(f_buf[...]), taps, NT_DIMS, preferred_element_type=F32)

    def product(c, g, odd, a0, b0, b1, acc, pin):
        def load(which, chunk):
            slot = (which * 2 + (c & 1)) * NB + chunk
            return spec[slot, rows8(g * 16, 8), :], spec[slot, rows8(g * 16 + 8, 8), :]

        taps = {}
        for b in range(b0, b1):
            xr, xi = load(0, b)
            for a in range(max(a0, b), a0 + 2):
                if a - b not in taps:
                    taps[a - b] = load(1, a - b)
                hr, hi = taps[a - b]
                pr, pi = hr * xr - hi * xi, hr * xi + hi * xr
                acc[a] = (acc[a][0] + pr, acc[a][1] + pi) if b else (pr, pi)
        for u, a in enumerate((a0, a0 + 1)):
            zr, zi = acc[a]
            if b1 < a0 + 2:
                if CFG["pin"]:
                    store_f32(pin, (c >> 3) + PIN_OFF + 16 * u, zr)
                    store_f32(pin, (c >> 3) + PIN_OFF + 16 * u + 8, zi)
                continue
            if a:
                tr, ti = acc[a - 1]
                zr, zi = (zr + ti, zi - tr) if odd else (zr - ti, zi + tr)
            y = pltpu.pack_elementwise([zr, zi], packed_dtype=BF16)
            buf0[rows8(RES_OFF + (c * NB + a) * T + g * 8, 8), :] = y
            if pin is not buf0 and CFG['pin']:
                pin[rows8((c >> 3) + PIN_OFF + 8 * u, 8), :] = y

    for cp in c_cp + w_cp(0) + x_cp + list(conv_cp(0)) + list(conv_cp(1)) + w_cp(1):
        cp.start()
    f_buf[...] = pltpu.bitcast(fwd_ref[...], U32)
    ks32[:, 0:8, :] = jnp.zeros((NC, 8, T), U32)
    shift_taps = sk_ref[...].astype(F32)
    for j in range(NC):
        shift_buf[j, 0:4, :] = shift_taps[:, j * T:(j + 1) * T]
    for cp in c_cp + w_cp(0) + x_cp:
        cp.wait()
    for t in range(16):
        w_cur[0, pl.ds(t * HP, HP), :] = unpack_weights(jnp.int32(0), t)
    proj_q(0, 0, 0)
    proj_k(0, 0, 0)
    proj_q(0, 0, 1)
    proj_k(0, 0, 1)
    proj_v(0, 0, 0)
    scores(0, 0, 0, 1)
    row_max(0, 0)
    for cp in conv_cp(0):
        cp.wait()
    for a in range(NB):
        gate_kv(0, 0, a * HP // 8, HP)
        spec[a] = forward_x(0, a)
        spec[2 * NB + a] = forward_h(0, a)
    for cp in conv_cp(1):
        cp.wait()
    for cp in wo_cp:
        cp.start()

    def head(h, carry):
        c, quarter = h >> 2, h & 3
        cn = jnp.minimum(c + 1, NC - 1)
        hn = jnp.minimum(h + 1, H - 1)
        z = h >> 5

        def dma():
            @pl.when(jnp.logical_and(quarter == 3, c + 2 < NC))
            def _():
                for cp in conv_cp(jnp.minimum(c + 2, NC - 1)):
                    cp.wait()

            @pl.when(jnp.logical_and(quarter == 0, c + 2 < NC))
            def _():
                for cp in conv_cp(jnp.minimum(c + 2, NC - 1)):
                    cp.start()

            @pl.when(jnp.logical_and((h & 1) == 0, h + 2 < H))
            def _():
                for cp in w_cp(jnp.minimum((h >> 1) + 1, H // 2 - 1)):
                    cp.wait()

            @pl.when(jnp.logical_and((h & 1) == 1, h + 3 < H))
            def _():
                for cp in w_cp(jnp.minimum((h >> 1) + 2, H // 2 - 1)):
                    cp.start()

        steps = _head_program()
        users = [n for n, st in enumerate(steps) if st[0] in ("scores", "attend")]
        parity = [steps[n][1] % 2 for n in users]
        tasks = {n: [] for n in users}
        PB = CFG["pb"]
        pieces = [(gi, a0, b0, min(b0 + PB, a0 + 2))
                  for gi in range(4) for a0 in range(0, NB, 2) for b0 in range(0, a0 + 2, PB)]
        hosts = [n for n in users if CFG["where"] == 0 or steps[n][0] == ("scores", "attend")[CFG["where"] - 1]]
        acc, held = {}, {}
        for u, (gi, a0, b0, b1) in enumerate(pieces if CFG['prod'] else []):
            n = hosts[u * len(hosts) // len(pieces)]
            tasks[n].append(functools.partial(
                product, c, quarter * 4 + gi, gi % 2, a0, b0, b1, acc, bufs[steps[n][1] % 2]))

        def forward(name, fn, *args):
            held[name] = fn(*args)

        def spec_store(name, slot):
            spec[slot] = held.pop(name)

        odd = [n for n in users if steps[n][0] == "attend" and steps[n][1] % 2 == 1]
        even = [n for n in users if steps[n][0] == "attend" and steps[n][1] % 2 == 0]
        for u in range(4 * CFG['fwd']):
            a = quarter * 4 + u
            for r in range(4):
                tasks[odd[5 * u + r]].append(functools.partial(gate_kv, cn, c + 1, a * 8 + 2 * r, 16))
            for which, n, fn, tile in ((0, odd[5 * u + 3], forward_x, c + 1), (1, even[5 * u + 2], forward_h, cn)):
                tasks[n].append(functools.partial(forward, (which, u), fn, tile, a))
                after = min(n + CFG["lag"], len(steps) - 1)
                tasks.setdefault(after, []).insert(0, functools.partial(
                    spec_store, (which, u), (which * 2 + ((c + 1) & 1)) * NB + a))

        for n, st in enumerate(steps):
            for task in tasks.get(n, ()):
                task()
            kind, i = st[:2]
            if kind == "weights":
                w_cur[(h + 1) & 1, pl.ds(i * HP, HP), :] = unpack_weights(hn, i)
            elif kind == "dma":
                dma()
            elif kind == "scores":
                scores(z, *st[1:])
            elif kind == "attend":
                attend(h, *st[1:])
            elif kind == "max":
                row_max(z, i)
            elif kind == "v":
                proj_v(z, h + (i == 0), i)
            else:
                (proj_q if kind == "q" else proj_k)(z, h + (i < 2), i)
        return carry

    lax.fori_loop(0, H, head, 0)

    for cp in wo_cp:
        cp.wait()
    f_buf[:, :] = pltpu.bitcast(jnp.concatenate([inv_ref[:, :T], inv_ref[:, T:]], axis=0), U32)
    gate_w = gw_ref[...].astype(F32).reshape(1, DM)
    skip_d = d_ref[...].astype(F32).reshape(1, DM)
    for j in range(NC):
        shift_buf[j, 0:1, :] = gate_w[:, j * T:(j + 1) * T]
        shift_buf[j, 1:2, :] = skip_d[:, j * T:(j + 1) * T]

    def out_cp(r, slot):
        return pltpu.make_async_copy(
            out_buf.at[slot], out_hbm.at[0, pl.ds(pl.multiple_of(r * RB, RB), RB), :], sem_out.at[slot])

    def mix(r, carry):
        slot = r % 2
        rp = pl.ds(pl.multiple_of(r * (RB // 2), RB // 2), RB // 2)

        @pl.when(r >= 2)
        def _():
            out_cp(r - 2, slot).wait()

        logit = None
        for j in range(NC):
            t = _bf(xs32[j, rp, :]).astype(F32) * shift_buf[j, 0:1, :]
            logit = t if logit is None else logit + t
        gate = 1.0 / (1.0 + jnp.exp(-jnp.sum(logit, axis=1, keepdims=True)))
        g_buf[...] = jnp.broadcast_to(gate, (RB, T))
        inv = jnp.concatenate([_bf(f_buf[0:HP, :]), _bf(f_buf[HP:T, :])], axis=1)
        for j in range(NC):
            b = None
            for h0 in range(0, H, 4):
                lhs = jnp.concatenate(
                    [_bf(ctx32[rows8((h0 + u) * (S // 2) + r * (RB // 2), RB // 2), :]) for u in range(4)],
                    axis=1)
                t = _dot(lhs, _bf(wo32[j, pl.ds(h0 * HP, 4 * HP), :]))
                b = t if b is None else b + t
            y = jnp.concatenate(
                [_dot(inv, _bf(buf0[rows8(RES_OFF + (j * NB + r * (RB // T) + u) * T, T), :]))
                 for u in range(RB // T)], axis=0)
            kv = _bf(buf1[rows8(RES_OFF + j * (S // 2) + r * (RB // 2), RB // 2), :]).astype(F32)
            a = _bf(xs32[j, rp, :]).astype(F32) * (y + kv * shift_buf[j, 1:2, :])
            g = g_buf[...]
            out_buf[slot, :, lanes(j)] = (g * a + (1.0 - g) * b).astype(BF16)
        out_cp(r, slot).start()
        return carry

    lax.fori_loop(0, S // RB, mix, 0)
    for r in (S // RB - 2, S // RB - 1):
        out_cp(r, r % 2).wait()


@jax.jit
def pallas_gated_mix__ssm_conv_h3__compressed_kv_cla__prompt_kernel(
    A_q, A_k, A_v, A_shift_k, A_ssm_k, A_ssm_D, B_x, B_c_kv, B_w_q, B_w_uk, B_w_uv, B_w_o, gate_w,
):
    del B_x
    hbm = pl.BlockSpec(memory_space=pl.ANY)
    vmem = pl.BlockSpec(memory_space=pltpu.VMEM)
    scratch = [
        pltpu.VMEM((NC, S // 2, T), U32),
        pltpu.VMEM((DC // T, S // 2, T), U32),
        pltpu.VMEM((2, DM + 2 * DC, T), U32),
        pltpu.VMEM((NC, H * HP, T), U32),
        pltpu.VMEM((NC, K_PITCH, T), U32),
        pltpu.VMEM((NC, S // 2, T), U32),
        pltpu.VMEM((NC, HP, S), U32),
        pltpu.VMEM((4 * NB, 2 * T, T), F32),
        pltpu.VMEM((2, 16 * HP, T), U32),
        pltpu.VMEM((RES_OFF + NC * S, T), U32),
        pltpu.VMEM((RES_OFF + (NC + 1) * S // 2, T), U32),
        pltpu.VMEM((T, T), F32),
        pltpu.VMEM((T, T), F32),
        pltpu.VMEM((T, T), F32),
        pltpu.VMEM((H * S + 4 * T, T), BF16),
        pltpu.VMEM((NC, 8, T), F32),
        pltpu.VMEM((T, T), U32),
        pltpu.VMEM((RB, T), F32),
        pltpu.VMEM((2, RB, DM), BF16),
        pltpu.SemaphoreType.DMA((NC,)),
        pltpu.SemaphoreType.DMA((DC // T,)),
        pltpu.SemaphoreType.DMA((2, 3)),
        pltpu.SemaphoreType.DMA((NC,)),
        pltpu.SemaphoreType.DMA((3, NC)),
        pltpu.SemaphoreType.DMA((2,)),
    ] + [pltpu.VMEM((1, T, T), BF16)] * (3 * NB)
    return pl.pallas_call(
        _kernel,
        out_shape=jax.ShapeDtypeStruct((1, S, DM), BF16),
        in_specs=[hbm, hbm, hbm, vmem, hbm, vmem, hbm, hbm, hbm, hbm, hbm, vmem, vmem, vmem],
        out_specs=hbm,
        scratch_shapes=scratch,
        compiler_params=pltpu.CompilerParams(
            vmem_limit_bytes=110 * 1024 * 1024, disable_bounds_checks=bool(CFG['nobc']),
            flags={"XLA_TPU_FORCE_LP_LLO_SCHEDULER": True} if CFG["lp"] else None),
        name="gated_mix_h3_cla",
    )(
        A_q, A_k, A_v, A_shift_k.T, A_ssm_k, A_ssm_D, B_c_kv,
        B_w_q, B_w_uk, B_w_uv, B_w_o.reshape(H * DH, DM), gate_w, _FWD, _INV,
    )
```

```python
import functools
import math

import jax
import jax.numpy as jnp
import numpy as np
from jax import lax
import jax.experimental.pallas as pl
import jax.experimental.pallas.tpu as pltpu

S = 2048
DM = 1024
H = 32
DH = 128
DC = 512
T = 128
NB = S // T
NC = DM // T
RB = 256
KG = 4

HP = T // 2
PIN_OFF = NB * T
RES_OFF = PIN_OFF + 4 * 8
K_PITCH = 8 + S // 2

ROW_CHUNKS = (0, 2, 4, 8, 12, 16)
FWD_ROUND = 8

import os
CFG = dict(lp=0, order=1, lag=5, prod=1, fwd=1, dmapos=15, nobc=1, pin=2, pb=2, where=5, kg=4, accmem=0, opq=1, mround=0, peel=1, slab_s=128, slab_a=16, zmask=0, even=0, pace=1, lead=2, ppace=1, plead=0, gpace=1, glead=0)
CFG.update({k: int(v) for k, v in (kv.split("=") for kv in os.environ.get("KCFG", "").split(",") if kv)})

KG = CFG["kg"]
F32, BF16, U32 = jnp.float32, jnp.bfloat16, jnp.uint32
Q_SCALE = (DH ** -0.5) * math.log2(math.e)
NEG = -1e30
NT_DIMS = (((1,), (1,)), ((), ()))


def _dft_matrices():
    g = np.arange(16)[:, None]
    s = np.arange(8)[None, :]
    f = 2 * (8 * (g // 2) + s) + g % 2
    th = 2.0 * np.pi * (f[..., None] + 0.5) * np.arange(T) / (2 * T)
    fwd = np.stack([np.cos(th), -np.sin(th)], axis=1).reshape(2 * T, T)
    inv = np.stack([np.cos(th), -np.sin(th)], axis=2).reshape(2 * T, T).T / T
    return fwd.astype(BF16), np.ascontiguousarray(inv).astype(BF16)


_FWD, _INV = _dft_matrices()


def _bf(words):
    return pltpu.bitcast(words, BF16)


def _lo(words):
    return pltpu.bitcast(words << 16, F32)


def _hi(words):
    return pltpu.bitcast(words & jnp.uint32(0xFFFF0000), F32)


def _dot(a, b):
    return jnp.dot(a, b, preferred_element_type=F32)


def _key_groups(i):
    return [(j0, min(KG, i + 1 - j0)) for j0 in range(0, i + 1, KG)]


def _head_program():
    steps = []
    for i in range(NB):
        nxt = (i + 1) % NB
        sc = [("scores", nxt) + grp for grp in _key_groups(nxt)]
        at = [("attend", i) + grp for grp in _key_groups(i)]
        q, k, v = ("q", (i + 2) % NB), ("k", (i + 2) % NB), ("v", nxt)
        rnd = [x for u in range(NB) for x in sc[u:u + 1] + at[u:u + 1]]
        if i < NB - 2:
            if CFG["order"] == 0:
                rnd = [q, k, v] + rnd
            else:
                u = 4 // KG
                rnd = [q] + rnd[:u] + [k] + rnd[u:3 * u] + [v] + rnd[3 * u:]
            rnd.append(("max", nxt))
        elif i == NB - 2:
            rnd = [v] + rnd + [("max", nxt), q, k]
        else:
            u = 4 // KG
            rnd = at[:u] + [q] + at[u:2 * u] + [k] + at[2 * u:3 * u] + sc + at[3 * u:] + [v, ("max", nxt)]
        if i + 2 in ROW_CHUNKS[2:-1]:
            steps.append(("rows", ROW_CHUNKS.index(i + 2)))
        if i == FWD_ROUND:
            steps.append(("conv", i))
        steps += rnd[:1] + [("weights", i)] + rnd[1:]
        if i == CFG["dmapos"]:
            steps.append(("dma", i))
    return steps


def _kernel(zero_ref, x_hbm, k_hbm, v_hbm, sk_ref, h_hbm, d_ref, c_hbm, wq_hbm, wk_hbm, wv_hbm, wo_hbm,
            gw_ref, fwd_ref, inv_ref, out_hbm,
            xs32, cs32, w_raw, wo32, ks32, vs32, hs32, spec, w_cur, buf0, buf1, mx_buf, l_buf, o_buf,
            ctx, shift_buf, f_buf, g_buf, out_buf,
            sem_rows, sem_w, sem_wo, sem_conv, sem_out, *qkv):
    q_buf, k_buf, v_buf = qkv[:NB], qkv[NB:2 * NB], qkv[2 * NB:]
    x_hbm, k_hbm, v_hbm, h_hbm, c_hbm, wq_hbm, wk_hbm, wv_hbm, wo_hbm = (
        r.bitcast(U32) for r in (x_hbm, k_hbm, v_hbm, h_hbm, c_hbm, wq_hbm, wk_hbm, wv_hbm, wo_hbm))
    bufs = (buf0, buf1)
    ctx32, m_buf = ctx.bitcast(U32), ctx.bitcast(F32)
    M_OFF = H * S // 2

    def lanes(j):
        return pl.ds(j * T, T)

    def rows8(start, n):
        return pl.ds(start if isinstance(start, int) else pl.multiple_of(start, 8), n)

    def load_f32(buf, start, n):
        return pltpu.bitcast(buf[rows8(start, n), :], F32)

    def store_f32(buf, start, value):
        buf[rows8(start, value.shape[0]), :] = pltpu.bitcast(value, U32)

    def rows_cp(n):
        rows = pl.ds(ROW_CHUNKS[n] * HP, (ROW_CHUNKS[n + 1] - ROW_CHUNKS[n]) * HP)
        return [pltpu.make_async_copy(src.at[0, rows], dst.at[rows], sem_rows.at[i, n])
                for i, (src, dst) in enumerate(((c_hbm, cs32), (x_hbm, xs32)))]

    wo_cp = pltpu.make_async_copy(wo_hbm, wo32, sem_wo.at[0])

    def w_cp(p):
        return [pltpu.make_async_copy(src.at[:, p, :], w_raw.at[p & 1, pl.ds(r0, n)], sem_w.at[p & 1, i])
                for i, (src, r0, n) in enumerate(
                    ((wq_hbm, 0, DM), (wk_hbm, DM, DC), (wv_hbm, DM + DC, DC)))]

    def conv_cp(c):
        col = pl.ds(pl.multiple_of(c * T, T), T)
        return [
            pltpu.make_async_copy(k_hbm.at[0, :, col], ks32.at[c, pl.ds(8, S // 2)], sem_conv.at[0, c]),
            pltpu.make_async_copy(v_hbm.at[0, :, col], vs32.at[c], sem_conv.at[1, c]),
            pltpu.make_async_copy(h_hbm.at[pl.ds(pl.multiple_of(c * HP, HP), HP)], hs32.at[c],
                                  sem_conv.at[2, c]),
        ]

    def unpack_weights(h, t):
        slot = (h >> 1) & 1
        sh = ((h & 1) * 16).astype(U32)
        even = w_raw[slot, pl.ds(t * T, HP, stride=2), :]
        odd = w_raw[slot, pl.ds(t * T + 1, HP, stride=2), :]
        return ((even >> sh) & jnp.uint32(0xFFFF)) | ((odd >> sh) << 16)

    def lhs_cat(src, i, j0, n):
        return jnp.concatenate([_bf(src[pl.ds(i * HP, HP), lanes(j0 + j)]) for j in range(n)], axis=1)

    def w_cat(h, t0, n):
        return _bf(w_cur[h & 1, pl.ds(t0 * HP, n * HP), :])

    stream = []

    def recent(slab):
        n, r = divmod(slab, 8)
        if len(stream) < 2 - n:
            return None
        return stream[n - 2][16 * r + 8:16 * r + 16, 0:T]

    def proj_q(z, h, i):
        qa, qb = (_dot(lhs_cat(xs32, i, t, 4), w_cat(h, t, 4)) for t in (0, 4))
        q = qa + qb
        q_buf[i][z] = (q * Q_SCALE).astype(BF16)
        stream.extend([qa, qb])

    def proj_k(z, h, i):
        stream.append(_dot(lhs_cat(cs32, i, 0, 4), w_cat(h, 8, 4)))
        k_buf[i][z] = stream[-1].astype(BF16)

    def proj_v(z, h, i):
        stream.append(_dot(lhs_cat(cs32, i, 0, 4), w_cat(h, 12, 4)))
        v_buf[i][z] = stream[-1].astype(BF16)

    def tiles_of(buf, j0, n, z=0):
        return _bf(jnp.concatenate([buf[j0 + j].bitcast(U32)[z] for j in range(n)], axis=0))

    def scores(z, i, j0, n):
        s = lax.dot_general(tiles_of(q_buf, i, 1), tiles_of(k_buf, j0, n, z * CFG['opq']), NT_DIMS,
                            preferred_element_type=F32)
        stream.append(s)
        R = CFG["slab_s"]
        diff = lax.broadcasted_iota(jnp.int32, (R, T), 1) - lax.broadcasted_iota(jnp.int32, (R, T), 0)
        for r in range(0, T, R):
            mx = None if j0 == 0 else mx_buf[0, r:r + R, :]
            for j in range(n):
                t = s[r:r + R, j * T:(j + 1) * T]
                if j0 + j == i:
                    t = jnp.where(diff <= r + z * CFG["zmask"], t, NEG)
                store_f32(bufs[i % 2], z + (j0 + j) * T + r, t)
                mx = t if mx is None else jnp.maximum(mx, t)
            mx_buf[z * CFG['accmem'], r:r + R, :] = mx

    def row_max(z, i):
        m_buf[rows8(z + M_OFF + i % 2 * T, T), :] = jnp.broadcast_to(
            jnp.max(mx_buf[0], axis=1, keepdims=True), (T, T))

    def attend(z, h, i, j0, n):
        R = CFG["slab_a"]
        last = j0 + n == i + 1
        slabs, ls = [], []
        for r in range(0, T, R):
            pace = recent(r // 16 + CFG["lead"] - 8) if CFG["pace"] else None
            if pace is not None:
                m_buf[rows8(z + M_OFF + 2 * T, 8), :] = pace
            m = m_buf[rows8(M_OFF + i % 2 * T + r, R), :]
            l = None if j0 == 0 else l_buf[0, r:r + R, :]
            ps = []
            for j in range(n):
                p = jnp.exp2(load_f32(bufs[i % 2], (j0 + j) * T + r, R) - m)
                l = p if l is None else l + p
                ps.append(p)
            slabs.append(jnp.concatenate(ps, axis=1))
            if last:
                total = jnp.sum(l, axis=1, keepdims=True)
                rcp = pl.reciprocal(total, approx=True)
                ls.append(rcp * (2.0 - total * rcp))
            else:
                l_buf[z * CFG['accmem'], r:r + R, :] = l
        o = _dot(jnp.concatenate(slabs, axis=0).astype(BF16), tiles_of(v_buf, j0, n, z * CFG['opq']))
        stream.append(o)
        R = max(R, 16)
        if last:
            ls = jnp.concatenate(ls, axis=0)
        for r in range(0, T, R):
            t = o[r:r + R]
            if j0 > 0:
                t = t + o_buf[0, r:r + R, :]
            if last:
                ctx[pl.ds(pl.multiple_of(h * S + i * T + r, R), R), :] = (t * ls[r:r + R]).astype(BF16)
            else:
                o_buf[z * CFG['accmem'], r:r + R, :] = t

    def gate_kv(c, c_out, r8, n):
        r = r8 * 8
        pace = recent(CFG["glead"] - 8) if CFG["gpace"] and n < HP else None
        if pace is not None:
            ks32[NC + (c >> 3), 0:8, :] = pltpu.bitcast(pace, U32)
        w0, w1, w2 = ks32[c, rows8(r + 8, n), :], ks32[c, pl.ds(r + 7, n), :], ks32[c, pl.ds(r + 6, n), :]
        e0, o0, e1, o1, o2 = _lo(w0), _hi(w0), _lo(w1), _hi(w1), _hi(w2)
        s0, s1, s2, s3 = (shift_buf[c, j:j + 1, :] for j in range(4))
        even = s3 * o2 + s2 * e1 + s1 * o1 + s0 * e0
        odd = s3 * e1 + s2 * o1 + s1 * e0 + s0 * o0
        vw = vs32[c, rows8(r, n), :]
        buf1[rows8(RES_OFF + c_out * (S // 2) + r, n), :] = pltpu.pack_elementwise(
            [even * _lo(vw), odd * _hi(vw)], packed_dtype=BF16)

    def forward_x(c, a):
        return _dot(_bf(f_buf[...]), _bf(buf1[rows8(RES_OFF + c * (S // 2) + a * HP, HP), :]))

    def forward_h(c, a):
        taps = _bf(hs32[c, :, pl.ds(pl.multiple_of(a * T, T), T)])
        return lax.dot_general(_bf(f_buf[...]), taps, NT_DIMS, preferred_element_type=F32)

    def product(c, g, odd, a0, b0, b1, acc, pin):
        def load(which, chunk):
            slot = (which * 2 + (c & 1)) * NB + chunk
            return spec[slot, rows8(g * 16, 8), :], spec[slot, rows8(g * 16 + 8, 8), :]

        pace = recent(CFG["plead"] - 8) if CFG["ppace"] else None
        if pace is not None:
            spec[(c >> 3) + 4 * NB, 0:8, :] = pace
        taps = {}
        for b in range(b0, b1):
            xr, xi = load(0, b)
            for a in range(max(a0, b), a0 + 2):
                if a - b not in taps:
                    taps[a - b] = load(1, a - b)
                hr, hi = taps[a - b]
                pr, pi = hr * xr - hi * xi, hr * xi + hi * xr
                acc[a] = (acc[a][0] + pr, acc[a][1] + pi) if b else (pr, pi)
        for u, a in enumerate((a0, a0 + 1)):
            zr, zi = acc[a]
            if b1 < a0 + 2:
                if CFG["pin"]:
                    pin(16 * u, pltpu.bitcast(zr, U32))
                    pin(16 * u + 8, pltpu.bitcast(zi, U32))
                continue
            if a:
                tr, ti = acc[a - 1]
                zr, zi = (zr + ti, zi - tr) if odd else (zr - ti, zi + tr)
            y = pltpu.pack_elementwise([zr, zi], packed_dtype=BF16)
            buf0[rows8(RES_OFF + (c * NB + a) * T + g * 8, 8), :] = y
            if CFG['pin']:
                pin(8 * u, y)

    for cp in (w_cp(0) + rows_cp(0) + conv_cp(0) + rows_cp(1) + rows_cp(2) + rows_cp(3) + conv_cp(1)
               + rows_cp(4) + w_cp(1)):
        cp.start()
    f_buf[...] = pltpu.bitcast(fwd_ref[...], U32)
    ks32[0:NC, 0:8, :] = jnp.zeros((NC, 8, T), U32)
    shift_taps = sk_ref[...].astype(F32)
    for j in range(NC):
        shift_buf[j, 0:4, :] = shift_taps[:, j * T:(j + 1) * T]
    for cp in w_cp(0) + rows_cp(0):
        cp.wait()
    for t in range(16):
        w_cur[0, pl.ds(t * HP, HP), :] = unpack_weights(jnp.int32(0), t)
    proj_q(0, 0, 0)
    proj_k(0, 0, 0)
    proj_q(0, 0, 1)
    proj_k(0, 0, 1)
    proj_v(0, 0, 0)
    scores(0, 0, 0, 1)
    row_max(0, 0)
    for cp in conv_cp(0):
        cp.wait()
    for a in range(NB):
        gate_kv(0, 0, a * HP // 8, HP)
        spec[a] = forward_x(0, a)
        spec[2 * NB + a] = forward_h(0, a)
    for cp in rows_cp(1):
        cp.wait()

    def head(h, first):
        c, quarter = h >> 2, h & 3
        cn = jnp.minimum(c + 1, NC - 1)
        hn = jnp.minimum(h + 1, H - 1)
        z = h >> 5

        def dma():
            if first:
                wo_cp.start()

            @pl.when(jnp.logical_and(quarter == 3, c + 2 < NC))
            def _():
                for cp in conv_cp(jnp.minimum(c + 2, NC - 1)):
                    cp.wait()

            @pl.when(jnp.logical_and(quarter == 0, c + 2 < NC))
            def _():
                for cp in conv_cp(jnp.minimum(c + 2, NC - 1)):
                    cp.start()

            @pl.when(jnp.logical_and((h & 1) == 0, h + 2 < H))
            def _():
                for cp in w_cp(jnp.minimum((h >> 1) + 1, H // 2 - 1)):
                    cp.wait()

            @pl.when(jnp.logical_and((h & 1) == 1, h + 3 < H))
            def _():
                for cp in w_cp(jnp.minimum((h >> 1) + 2, H // 2 - 1)):
                    cp.start()

        steps = _head_program()
        stream.clear()
        users = [n for n, st in enumerate(steps) if st[0] in ("scores", "attend")]
        parity = [steps[n][1] % 2 for n in users]
        tasks = {n: [] for n in users}
        PB = CFG["pb"]
        pieces = [(gi, a0, b0, min(b0 + PB, a0 + 2))
                  for gi in range(4) for a0 in range(0, NB, 2) for b0 in range(0, a0 + 2, PB)]
        hosts = [n for n, st in enumerate(steps)
                 if st[0] in (("scores", "attend"), ("scores",), ("attend",), ("scores", "attend", "q", "k", "v"),
                              ("k", "v"), ("q", "k", "v"))[CFG["where"]]]

        def pin_of(st):
            if st[0] in ("scores", "attend"):
                buf, slot = (k_buf if st[0] == "scores" else v_buf)[st[2]].bitcast(U32), z + 1
            elif CFG["pin"] == 2:
                buf, slot = dict(q=q_buf, k=k_buf, v=v_buf)[st[0]][st[1]].bitcast(U32), z + 1
            elif CFG["pin"] == 3:
                buf, slot = spec.bitcast(U32), z + 4 * NB
            else:
                buf, slot = w_cur, z + 2

            def pin(r, y):
                buf[slot, pl.ds(r, 8), :] = y
            return pin

        acc, held = {}, {}
        for u, (gi, a0, b0, b1) in enumerate(pieces if CFG['prod'] else []):
            n = hosts[u * len(hosts) // len(pieces)]
            tasks.setdefault(n, []).append(functools.partial(
                product, c, quarter * 4 + gi, gi % 2, a0, b0, b1, acc, pin_of(steps[n])))

        def forward(name, fn, *args):
            held[name] = fn(*args)

        def spec_store(name, slot):
            spec[slot] = held.pop(name)

        late = [n for n in users if steps[n][0] == "attend" and steps[n][1] >= FWD_ROUND]
        odd, even = ([n for n in late if steps[n][1] % 2 == par] for par in (1, 0))
        for u in range(4 * CFG['fwd']):
            a = quarter * 4 + u
            for r in range(4):
                tasks[odd[(5 * u + r) * len(odd) // 20]].append(
                    functools.partial(gate_kv, cn, c + 1, a * 8 + 2 * r, 16))
            for which, n, fn, tile in ((0, odd[(5 * u + 4) * len(odd) // 20], forward_x, c + 1),
                                       (1, even[u * len(even) // 4], forward_h, cn)):
                tasks[n].append(functools.partial(forward, (which, u), fn, tile, a))
                after = min(n + CFG["lag"], len(steps) - 1)
                tasks.setdefault(after, []).insert(0, functools.partial(
                    spec_store, (which, u), (which * 2 + ((c + 1) & 1)) * NB + a))

        for n, st in enumerate(steps):
            for task in tasks.get(n, ()):
                task()
            kind, i = st[:2]
            if CFG["opq"] and kind in ("scores", "attend"):
                z = (h + i) >> 6
            if kind == "weights":
                w_cur[(h + 1) & 1, pl.ds(i * HP, HP), :] = unpack_weights(hn, i)
            elif kind in ("rows", "conv"):
                for cp in (rows_cp(i) if kind == "rows" else conv_cp(1)) if first else ():
                    cp.wait()
            elif kind == "dma":
                dma()
            elif kind == "scores":
                scores(z, *st[1:])
            elif kind == "attend":
                attend(z, h, *st[1:])
            elif kind == "max":
                row_max(z, i)
            elif kind == "v":
                proj_v(z, h + (i == 0), i)
            else:
                (proj_q if kind == "q" else proj_k)(z, h + (i < 2), i)

    if CFG['peel']:
        head(zero_ref[0], True)
    lax.fori_loop(1, H, lambda h, _: head(h, False), None)

    wo_cp.wait()
    f_buf[:, :] = pltpu.bitcast(jnp.concatenate([inv_ref[:, :T], inv_ref[:, T:]], axis=0), U32)
    gate_w = gw_ref[...].astype(F32).reshape(1, DM)
    skip_d = d_ref[...].astype(F32).reshape(1, DM)
    for j in range(NC):
        shift_buf[j, 0:1, :] = gate_w[:, j * T:(j + 1) * T]
        shift_buf[j, 1:2, :] = skip_d[:, j * T:(j + 1) * T]

    def out_cp(r, slot):
        return pltpu.make_async_copy(
            out_buf.at[slot], out_hbm.at[0, pl.ds(pl.multiple_of(r * RB, RB), RB), :], sem_out.at[slot])

    def mix(r, carry):
        slot = r % 2
        rp = pl.ds(pl.multiple_of(r * (RB // 2), RB // 2), RB // 2)

        @pl.when(r >= 2)
        def _():
            out_cp(r - 2, slot).wait()

        logit = None
        for j in range(NC):
            t = _bf(xs32[rp, lanes(j)]).astype(F32) * shift_buf[j, 0:1, :]
            logit = t if logit is None else logit + t
        gate = 1.0 / (1.0 + jnp.exp(-jnp.sum(logit, axis=1, keepdims=True)))
        g_buf[...] = jnp.broadcast_to(gate, (RB, T))
        inv = jnp.concatenate([_bf(f_buf[0:HP, :]), _bf(f_buf[HP:T, :])], axis=1)
        for j in range(NC):
            b = None
            for h0 in range(0, H, 4):
                lhs = jnp.concatenate(
                    [_bf(ctx32[rows8((h0 + u) * (S // 2) + r * (RB // 2), RB // 2), :]) for u in range(4)],
                    axis=1)
                t = _dot(lhs, _bf(wo32[pl.ds(h0 * HP, 4 * HP), lanes(j)]))
                b = t if b is None else b + t
            y = jnp.concatenate(
                [_dot(inv, _bf(buf0[rows8(RES_OFF + (j * NB + r * (RB // T) + u) * T, T), :]))
                 for u in range(RB // T)], axis=0)
            kv = _bf(buf1[rows8(RES_OFF + j * (S // 2) + r * (RB // 2), RB // 2), :]).astype(F32)
            a = _bf(xs32[rp, lanes(j)]).astype(F32) * (y + kv * shift_buf[j, 1:2, :])
            g = g_buf[...]
            out_buf[slot, :, lanes(j)] = (g * a + (1.0 - g) * b).astype(BF16)
        out_cp(r, slot).start()
        return carry

    lax.fori_loop(0, S // RB, mix, 0)
    for r in (S // RB - 2, S // RB - 1):
        out_cp(r, r % 2).wait()


@jax.jit
def pallas_gated_mix__ssm_conv_h3__compressed_kv_cla__prompt_kernel(
    A_q, A_k, A_v, A_shift_k, A_ssm_k, A_ssm_D, B_x, B_c_kv, B_w_q, B_w_uk, B_w_uv, B_w_o, gate_w,
):
    del B_x
    hbm = pl.BlockSpec(memory_space=pl.ANY)
    vmem = pl.BlockSpec(memory_space=pltpu.VMEM)
    scratch = [
        pltpu.VMEM((S // 2, DM), U32),
        pltpu.VMEM((S // 2, DC), U32),
        pltpu.VMEM((2, DM + 2 * DC, T), U32),
        pltpu.VMEM((H * HP, DM), U32),
        pltpu.VMEM((NC + 1, K_PITCH, T), U32),
        pltpu.VMEM((NC, S // 2, T), U32),
        pltpu.VMEM((NC, HP, S), U32),
        pltpu.VMEM((4 * NB + 1, 2 * T, T), F32),
        pltpu.VMEM((3, 16 * HP, T), U32),
        pltpu.VMEM((RES_OFF + NC * S, T), U32),
        pltpu.VMEM((RES_OFF + (NC + 1) * S // 2, T), U32),
        pltpu.VMEM((1, T, T), F32),
        pltpu.VMEM((1, T, T), F32),
        pltpu.VMEM((1, T, T), F32),
        pltpu.VMEM((H * S + 4 * T + 16, T), BF16),
        pltpu.VMEM((NC, 8, T), F32),
        pltpu.VMEM((T, T), U32),
        pltpu.VMEM((RB, T), F32),
        pltpu.VMEM((2, RB, DM), BF16),
        pltpu.SemaphoreType.DMA((2, len(ROW_CHUNKS) - 1)),
        pltpu.SemaphoreType.DMA((2, 3)),
        pltpu.SemaphoreType.DMA((1,)),
        pltpu.SemaphoreType.DMA((3, NC)),
        pltpu.SemaphoreType.DMA((2,)),
    ] + [pltpu.VMEM((2, T, T), BF16)] * (3 * NB)
    return pl.pallas_call(
        _kernel,
        out_shape=jax.ShapeDtypeStruct((1, S, DM), BF16),
        in_specs=[pl.BlockSpec(memory_space=pltpu.SMEM), hbm, hbm, hbm, vmem, hbm, vmem, hbm, hbm, hbm, hbm, hbm, vmem, vmem, vmem],
        out_specs=hbm,
        scratch_shapes=scratch,
        compiler_params=pltpu.CompilerParams(
            vmem_limit_bytes=110 * 1024 * 1024, disable_bounds_checks=bool(CFG['nobc']),
            flags={k: True for k, on in (("XLA_TPU_FORCE_LP_LLO_SCHEDULER", CFG["lp"]),
                                         ("XLA_TPU_EVENLY_DISTRIBUTE_CRITICAL_NODES", CFG["even"])) if on}),
        name="gated_mix_h3_cla",
    )(
        np.zeros((1,), np.int32), A_q, A_k, A_v, A_shift_k.T, A_ssm_k, A_ssm_D, B_c_kv,
        B_w_q, B_w_uk, B_w_uv, B_w_o.reshape(H * DH, DM), gate_w, _FWD, _INV,
    )
```

```python
import functools
import itertools
import math

import jax
import jax.numpy as jnp
import numpy as np
from jax import lax
import jax.experimental.pallas as pl
import jax.experimental.pallas.tpu as pltpu

S = 2048
DM = 1024
H = 32
DH = 128
DC = 512
T = 128
NB = S // T
NC = DM // T
RB = 256
KG = 4

HP = T // 2
PIN_OFF = NB * T
RES_OFF = PIN_OFF + 4 * 8
K_PITCH = 8 + S // 2

ROW_CHUNKS = (0, 2, 4, 6, 9, 12, 16)

import os
CFG = dict(lp=0, order=1, lag=5, prod=1, fwd=1, dmapos=15, nobc=1, pin=2, pb=2, where=5, kg=4, accmem=0, opq=0, mround=0, peel=1, slab_s=128, slab_a=16, zmask=0, even=0, pace=1, lead=2, ppace=1, plead=0, gpace=1, glead=0, zm=1, sts=0, stq=0, wc=1, rep=1, stop=0, wo=0, c0=11, c1=13, fr=8, where1=3)
CFG.update({k: int(v) for k, v in (kv.split("=") for kv in os.environ.get("KCFG", "").split(",") if kv)})

KG = CFG["kg"]
ZM = CFG["zm"]
F32, BF16, U32 = jnp.float32, jnp.bfloat16, jnp.uint32
Q_SCALE = (DH ** -0.5) * math.log2(math.e)
NEG = -1e30
NT_DIMS = (((1,), (1,)), ((), ()))


def _dft_matrices():
    g = np.arange(16)[:, None]
    s = np.arange(8)[None, :]
    f = 2 * (8 * (g // 2) + s) + g % 2
    th = 2.0 * np.pi * (f[..., None] + 0.5) * np.arange(T) / (2 * T)
    fwd = np.stack([np.cos(th), -np.sin(th)], axis=1).reshape(2 * T, T)
    inv = np.stack([np.cos(th), -np.sin(th)], axis=2).reshape(2 * T, T).T / T
    return fwd.astype(BF16), np.ascontiguousarray(inv).astype(BF16)


_FWD, _INV = _dft_matrices()


def _bf(words):
    return pltpu.bitcast(words, BF16)


def _lo(words):
    return pltpu.bitcast(words << 16, F32)


def _hi(words):
    return pltpu.bitcast(words & jnp.uint32(0xFFFF0000), F32)


def _dot(a, b):
    return jnp.dot(a, b, preferred_element_type=F32)


def _key_groups(i):
    return [(j0, min(KG, i + 1 - j0)) for j0 in range(0, i + 1, KG)]


def _head_program(first):
    steps = []
    for i in range(NB):
        nxt = (i + 1) % NB
        sc = [("scores", nxt) + grp for grp in _key_groups(nxt)]
        at = [("attend", i) + grp for grp in _key_groups(i)]
        q, k, v = ("q", (i + 2) % NB), ("k", (i + 2) % NB), ("v", nxt)
        rnd = [x for u in range(NB) for x in sc[u:u + 1] + at[u:u + 1]]
        if i < NB - 2:
            if CFG["order"] == 0:
                rnd = [q, k, v] + rnd
            else:
                u = 4 // KG
                rnd = [q] + rnd[:u] + [k] + rnd[u:3 * u] + [v] + rnd[3 * u:]
            rnd.append(("max", nxt))
        elif i == NB - 2:
            rnd = [v] + rnd + [("max", nxt), q, k]
        else:
            u = 4 // KG
            rnd = at[:u] + [q] + at[u:2 * u] + [k] + at[2 * u:3 * u] + sc + at[3 * u:] + [v, ("max", nxt)]
        if first and i + 2 in ROW_CHUNKS[1:-1]:
            steps.append(("rows", ROW_CHUNKS.index(i + 2)))
        if first and i in (CFG["c0"], CFG["c1"]):
            steps.append(("conv", int(i > CFG["c0"])))
        steps += [("round", i)] + rnd[:1] + [("weights", i)] + rnd[1:]
        if i == CFG["dmapos"]:
            steps.append(("dma", i))
    return steps


def _kernel(zero_ref, x_hbm, k_hbm, v_hbm, sk_hbm, h_hbm, d_hbm, c_hbm, wq_hbm, wk_hbm, wv_hbm, wo_hbm,
            gw_hbm, fwd_hbm, inv_hbm, out_hbm,
            sk_ref, d_ref, gw_ref, fwd_ref, inv_ref,
            xs32, cs32, w_raw, wo32, ks32, vs32, hs32, spec, w_cur, buf0, buf1, mx_buf, l_buf, o_buf,
            ctx, shift_buf, f_buf, g_buf, out_buf,
            sem_small, sem_rows, sem_w, sem_wo, sem_conv, sem_out, *qkv):
    q_buf, k_buf, v_buf = qkv[:NB], qkv[NB:2 * NB], qkv[2 * NB:]
    x_hbm, k_hbm, v_hbm, h_hbm, c_hbm, wq_hbm, wk_hbm, wv_hbm, wo_hbm = (
        r.bitcast(U32) for r in (x_hbm, k_hbm, v_hbm, h_hbm, c_hbm, wq_hbm, wk_hbm, wv_hbm, wo_hbm))
    bufs = (buf0, buf1)
    ctx32, m_buf = ctx.bitcast(U32), ctx.bitcast(F32)
    M_OFF = H * S // 2

    def lanes(j):
        return pl.ds(j * T, T)

    def rows8(start, n):
        return pl.ds(start if isinstance(start, int) else pl.multiple_of(start, 8), n)

    def load_f32(buf, start, n):
        return pltpu.bitcast(buf[rows8(start, n), :], F32)

    def store_f32(buf, start, value):
        buf[rows8(start, value.shape[0]), :] = pltpu.bitcast(value, U32)

    def rows_cp(n):
        rows = pl.ds(ROW_CHUNKS[n] * HP, (ROW_CHUNKS[n + 1] - ROW_CHUNKS[n]) * HP)
        return [pltpu.make_async_copy(src.at[0, rows], dst.at[rows], sem_rows.at[i, n])
                for i, (src, dst) in enumerate(((c_hbm, cs32), (x_hbm, xs32)))]

    wo_cp = pltpu.make_async_copy(wo_hbm, wo32, sem_wo.at[0])

    def w_cp(p):
        return [pltpu.make_async_copy(src.at[:, p, :], w_raw.at[p & 1, pl.ds(r0, n)], sem_w.at[p & 1, i])
                for i, (src, r0, n) in enumerate(
                    ((wq_hbm, 0, DM), (wk_hbm, DM, DC), (wv_hbm, DM + DC, DC)))]

    def conv_cp(c):
        col = pl.ds(pl.multiple_of(c * T, T), T)
        return [
            pltpu.make_async_copy(k_hbm.at[0, :, col], ks32.at[c, pl.ds(8, S // 2)], sem_conv.at[0, c]),
            pltpu.make_async_copy(v_hbm.at[0, :, col], vs32.at[c], sem_conv.at[1, c]),
            pltpu.make_async_copy(h_hbm.at[pl.ds(pl.multiple_of(c * HP, HP), HP)], hs32.at[c],
                                  sem_conv.at[2, c]),
        ]

    def unpack_weights(h, t):
        slot = (h >> 1) & 1
        sh = ((h & 1) * 16).astype(U32)
        even = w_raw[slot, pl.ds(t * T, HP, stride=2), :]
        odd = w_raw[slot, pl.ds(t * T + 1, HP, stride=2), :]
        return ((even >> sh) & jnp.uint32(0xFFFF)) | ((odd >> sh) << 16)

    def lhs_cat(src, i, j0, n):
        return jnp.concatenate([_bf(src[pl.ds(i * HP, HP), lanes(j0 + j)]) for j in range(n)], axis=1)

    w_cache = {}

    def w_cat(h, t0, n):
        h, ahead = h
        if (ahead, t0) not in w_cache or not CFG["wc"]:
            w_cache[ahead, t0] = _bf(w_cur[(h + ahead) & 1, pl.ds(t0 * HP, n * HP), :])
        return w_cache[ahead, t0]

    stream = []

    def recent(slab):
        n, r = divmod(slab, 8)
        if len(stream) < 2 - n:
            return None
        return stream[n - 2][16 * r + 8:16 * r + 16, 0:T]

    def keep(buf, z, value):
        buf[z * (1 - CFG["stq"])] = value.astype(BF16)
        if CFG["stq"]:
            buf.bitcast(F32)[z + 1, T // 2 - 8:T // 2, :] = value[T - 8:T]

    def proj_q(z, h, i):
        qa, qb = (_dot(lhs_cat(xs32, i, t, 4), w_cat(h, t, 4)) for t in (0, 4))
        q = qa + qb
        keep(q_buf[i], z, q * Q_SCALE)
        stream.extend([qa, qb])

    def proj_k(z, h, i):
        stream.append(_dot(lhs_cat(cs32, i, 0, 4), w_cat(h, 8, 4)))
        keep(k_buf[i], z, stream[-1])

    def proj_v(z, h, i):
        stream.append(_dot(lhs_cat(cs32, i, 0, 4), w_cat(h, 12, 4)))
        keep(v_buf[i], z, stream[-1])

    def tiles_of(buf, j0, n, z=0):
        return _bf(jnp.concatenate([buf[j0 + j].bitcast(U32)[z] for j in range(n)], axis=0))

    def scores(z, i, j0, n):
        s = lax.dot_general(tiles_of(q_buf, i, 1), tiles_of(k_buf, j0, n, z * CFG['opq']), NT_DIMS,
                            preferred_element_type=F32)
        stream.append(s)
        R = CFG["slab_s"]
        diff = lax.broadcasted_iota(jnp.int32, (R, T), 1) - lax.broadcasted_iota(jnp.int32, (R, T), 0)
        for r in range(0, T, R):
            mx = None if j0 == 0 else mx_buf[0, r:r + R, :]
            for j in range(n):
                t = s[r:r + R, j * T:(j + 1) * T]
                if j0 + j == i:
                    t = jnp.where(diff <= r + z * CFG["zmask"], t, NEG)
                store_f32(bufs[i % 2], z * (1 - CFG['sts']) + (j0 + j) * T + r, t)
                mx = t if mx is None else jnp.maximum(mx, t)
            mx_buf[z * CFG['accmem'], r:r + R, :] = mx

    def row_max(z, i):
        if CFG["sts"]:
            store_f32(bufs[i % 2], z + PIN_OFF, mx_buf[0, T - 8:T, :])
        m_buf[rows8(z * ZM + M_OFF + i % 2 * T, T), :] = jnp.broadcast_to(
            jnp.max(mx_buf[0], axis=1, keepdims=True), (T, T))

    def attend(z, h, i, j0, n):
        R = CFG["slab_a"]
        last = j0 + n == i + 1
        slabs, ls = [], []
        for r in range(0, T, R):
            pace = recent(r // 16 + CFG["lead"] - 8) if CFG["pace"] else None
            if pace is not None:
                m_buf[rows8(z * ZM + M_OFF + 2 * T, 8), :] = pace
            m = m_buf[rows8(M_OFF + i % 2 * T + r, R), :]
            l = None if j0 == 0 else l_buf[0, r:r + R, :]
            ps = []
            for j in range(n):
                p = jnp.exp2(load_f32(bufs[i % 2], (j0 + j) * T + r, R) - m)
                l = p if l is None else l + p
                ps.append(p)
            slabs.append(jnp.concatenate(ps, axis=1))
            if last:
                total = jnp.sum(l, axis=1, keepdims=True)
                rcp = pl.reciprocal(total, approx=True)
                ls.append(rcp * (2.0 - total * rcp))
            else:
                l_buf[z * CFG['accmem'], r:r + R, :] = l
        o = _dot(jnp.concatenate(slabs, axis=0).astype(BF16), tiles_of(v_buf, j0, n, z * CFG['opq']))
        stream.append(o)
        R = max(R, 16)
        if last:
            ls = jnp.concatenate(ls, axis=0)
        for r in range(0, T, R):
            t = o[r:r + R]
            if j0 > 0:
                t = t + o_buf[0, r:r + R, :]
            if last:
                ctx[pl.ds(pl.multiple_of(h * S + i * T + r, R), R), :] = (t * ls[r:r + R]).astype(BF16)
            else:
                o_buf[z * CFG['accmem'], r:r + R, :] = t

    def gate_kv(c, c_out, r8, n):
        r = r8 * 8
        pace = recent(CFG["glead"] - 8) if CFG["gpace"] and n < HP else None
        if pace is not None:
            ks32[NC + (c >> 3), 0:8, :] = pltpu.bitcast(pace, U32)
        w0, w1, w2 = ks32[c, rows8(r + 8, n), :], ks32[c, pl.ds(r + 7, n), :], ks32[c, pl.ds(r + 6, n), :]
        e0, o0, e1, o1, o2 = _lo(w0), _hi(w0), _lo(w1), _hi(w1), _hi(w2)
        s0, s1, s2, s3 = (shift_buf[c, j:j + 1, :] for j in range(4))
        even = s3 * o2 + s2 * e1 + s1 * o1 + s0 * e0
        odd = s3 * e1 + s2 * o1 + s1 * e0 + s0 * o0
        vw = vs32[c, rows8(r, n), :]
        buf1[rows8(RES_OFF + c_out * (S // 2) + r, n), :] = pltpu.pack_elementwise(
            [even * _lo(vw), odd * _hi(vw)], packed_dtype=BF16)

    def forward_x(c, a):
        return _dot(_bf(f_buf[...]), _bf(buf1[rows8(RES_OFF + c * (S // 2) + a * HP, HP), :]))

    def forward_h(c, a):
        taps = _bf(hs32[c, :, pl.ds(pl.multiple_of(a * T, T), T)])
        return lax.dot_general(_bf(f_buf[...]), taps, NT_DIMS, preferred_element_type=F32)

    def product(c, g, odd, a0, b0, b1, acc, pin):
        def load(which, chunk):
            slot = (which * 2 + (c & 1)) * NB + chunk
            return spec[slot, rows8(g * 16, 8), :], spec[slot, rows8(g * 16 + 8, 8), :]

        pace = recent(CFG["plead"] - 8) if CFG["ppace"] else None
        if pace is not None:
            spec[(c >> 3) + 4 * NB, 0:8, :] = pace
        taps = {}
        for b in range(b0, b1):
            xr, xi = load(0, b)
            for a in range(max(a0, b), a0 + 2):
                if a - b not in taps:
                    taps[a - b] = load(1, a - b)
                hr, hi = taps[a - b]
                pr, pi = hr * xr - hi * xi, hr * xi + hi * xr
                acc[a] = (acc[a][0] + pr, acc[a][1] + pi) if b else (pr, pi)
        for u, a in enumerate((a0, a0 + 1)):
            zr, zi = acc[a]
            if b1 < a0 + 2:
                if CFG["pin"]:
                    pin(16 * u, pltpu.bitcast(zr, U32))
                    pin(16 * u + 8, pltpu.bitcast(zi, U32))
                continue
            if a:
                tr, ti = acc[a - 1]
                zr, zi = (zr + ti, zi - tr) if odd else (zr - ti, zi + tr)
            y = pltpu.pack_elementwise([zr, zi], packed_dtype=BF16)
            buf0[rows8(RES_OFF + (c * NB + a) * T + g * 8, 8), :] = y
            if CFG['pin']:
                pin(8 * u, y)

    small_cp = [pltpu.make_async_copy(src, dst, sem_small.at[i]) for i, (src, dst) in enumerate(
        ((sk_hbm, sk_ref), (fwd_hbm, fwd_ref), (inv_hbm, inv_ref), (gw_hbm, gw_ref), (d_hbm, d_ref)))]
    for cp in (w_cp(0) + [cp for n in range(len(ROW_CHUNKS) - 1) for cp in rows_cp(n)]
               + small_cp + conv_cp(0) + conv_cp(1) + w_cp(1)):
        cp.start()
    ks32[0:NC, 0:8, :] = jnp.zeros((NC, 8, T), U32)
    for cp in w_cp(0) + rows_cp(0):
        cp.wait()
    for t in range(16):
        w_cur[0, pl.ds(t * HP, HP), :] = unpack_weights(jnp.int32(0), t)
    proj_q(zero_ref[0], (0, 0), 0)
    proj_k(zero_ref[0], (0, 0), 0)
    proj_q(zero_ref[0], (0, 0), 1)
    scores(zero_ref[0], 0, 0, 1)
    proj_k(zero_ref[0], (0, 0), 1)
    proj_v(zero_ref[0], (0, 0), 0)
    row_max(zero_ref[0], 0)

    def first_transforms():
        for cp in small_cp + conv_cp(0):
            cp.wait()
        f_buf[...] = pltpu.bitcast(fwd_ref[...], U32)
        shift_taps = sk_ref[...].astype(F32)
        for j in range(NC):
            shift_buf[j, 0:4, :] = shift_taps[:, j * T:(j + 1) * T]
        for a in range(NB):
            gate_kv(0, 0, a * HP // 8, HP)
            spec[a] = forward_x(0, a)
            spec[2 * NB + a] = forward_h(0, a)

    def head(h, first):
        c, quarter = h >> 2, h & 3
        cn = jnp.minimum(c + 1, NC - 1)
        hn = jnp.minimum(h + 1, H - 1)
        z = h >> 5

        def dma():
            if first:
                wo_cp.start()

            @pl.when(jnp.logical_and(quarter == 3, c + 2 < NC))
            def _():
                for cp in conv_cp(jnp.minimum(c + 2, NC - 1)):
                    cp.wait()

            @pl.when(jnp.logical_and(quarter == 0, c + 2 < NC))
            def _():
                for cp in conv_cp(jnp.minimum(c + 2, NC - 1)):
                    cp.start()

            @pl.when(jnp.logical_and((h & 1) == 0, h + 2 < H))
            def _():
                for cp in w_cp(jnp.minimum((h >> 1) + 1, H // 2 - 1)):
                    cp.wait()

            @pl.when(jnp.logical_and((h & 1) == 1, h + 3 < H))
            def _():
                for cp in w_cp(jnp.minimum((h >> 1) + 2, H // 2 - 1)):
                    cp.start()

        steps = _head_program(first)
        rounds = list(itertools.accumulate(st[0] == "round" for st in steps))
        stream.clear()
        w_cache.clear()
        users = [n for n, st in enumerate(steps) if st[0] in ("scores", "attend")]
        parity = [steps[n][1] % 2 for n in users]
        tasks = {n: [] for n in users}
        PB = CFG["pb"]
        pieces = [(gi, a0, b0, min(b0 + PB, a0 + 2))
                  for gi in range(4) for a0 in range(0, NB, 2) for b0 in range(0, a0 + 2, PB)]
        hosts = [n for n, st in enumerate(steps)
                 if st[0] in (("scores", "attend"), ("scores",), ("attend",), ("scores", "attend", "q", "k", "v"),
                              ("k", "v"), ("q", "k", "v"))[CFG["where1" if first else "where"]]
                 and (not first or rounds[n] > CFG["c0"])]

        def pin_of(st):
            if st[0] in ("scores", "attend"):
                buf, slot = (k_buf if st[0] == "scores" else v_buf)[st[2]].bitcast(U32), z + 1
            elif CFG["pin"] == 2:
                buf, slot = dict(q=q_buf, k=k_buf, v=v_buf)[st[0]][st[1]].bitcast(U32), z + 1
            elif CFG["pin"] == 3:
                buf, slot = spec.bitcast(U32), z + 4 * NB
            else:
                buf, slot = w_cur, z + 2

            def pin(r, y):
                buf[slot, pl.ds(r, 8), :] = y
            return pin

        acc, held = {}, {}
        for u, (gi, a0, b0, b1) in enumerate(pieces if CFG['prod'] else []):
            n = hosts[u * len(hosts) // len(pieces)]
            tasks.setdefault(n, []).append(functools.partial(
                product, c, quarter * 4 + gi, gi % 2, a0, b0, b1, acc, pin_of(steps[n])))

        def forward(name, fn, *args):
            held[name] = fn(*args)

        def spec_store(name, slot):
            spec[slot] = held.pop(name)

        late = [n for n in users if steps[n][0] == "attend" and steps[n][1] >= CFG["c1" if first else "fr"]]
        odd, even = ([n for n in late if steps[n][1] % 2 == par] for par in (1, 0))
        for u in range(4 * CFG['fwd']):
            a = quarter * 4 + u
            for r in range(4):
                tasks[odd[(5 * u + r) * len(odd) // 20]].append(
                    functools.partial(gate_kv, cn, c + 1, a * 8 + 2 * r, 16))
            for which, n, fn, tile in ((0, odd[(5 * u + 4) * len(odd) // 20], forward_x, c + 1),
                                       (1, even[u * len(even) // 4], forward_h, cn)):
                tasks[n].append(functools.partial(forward, (which, u), fn, tile, a))
                after = min(n + CFG["lag"], len(steps) - 1)
                tasks.setdefault(after, []).insert(0, functools.partial(
                    spec_store, (which, u), (which * 2 + ((c + 1) & 1)) * NB + a))

        for n, st in enumerate(steps):
            for task in tasks.get(n, ()):
                task()
            kind, i = st[:2]
            if CFG["opq"] and kind in ("scores", "attend"):
                z = (h + i) >> 6
            if kind == "weights":
                w_cur[(h + 1) & 1, pl.ds(i * HP, HP), :] = unpack_weights(hn, i)
            elif kind == "round":
                pass
            elif kind == "rows":
                for cp in rows_cp(i):
                    cp.wait()
            elif kind == "conv":
                for cp in conv_cp(1) if i else ():
                    cp.wait()
                if not i:
                    first_transforms()
            elif kind == "dma":
                dma()
            elif kind == "scores":
                scores(z, *st[1:])
            elif kind == "attend":
                attend(z, h, *st[1:])
            elif kind == "max":
                row_max(z, i)
            elif kind == "v":
                proj_v(z, (h, int(i == 0)), i)
            else:
                (proj_q if kind == "q" else proj_k)(z, (h, int(i < 2)), i)

    if CFG['peel']:
        head(zero_ref[0], True)
    if CFG["stop"] == 1:
        wo_cp.wait()
        for cp in conv_cp(2):
            cp.wait()
        return
    lax.fori_loop(1, H, lambda h, _: head(h, False), None)
    if CFG["rep"] > 1:
        lax.fori_loop(0, 16, lambda h, _: head(jnp.maximum(h, H - 1), False), None)

    wo_cp.wait()
    if CFG['stop'] == 2:
        return
    f_buf[:, :] = pltpu.bitcast(jnp.concatenate([inv_ref[:, :T], inv_ref[:, T:]], axis=0), U32)
    gate_w = gw_ref[...].astype(F32).reshape(1, DM)
    skip_d = d_ref[...].astype(F32).reshape(1, DM)
    for j in range(NC):
        shift_buf[j, 0:1, :] = gate_w[:, j * T:(j + 1) * T]
        shift_buf[j, 1:2, :] = skip_d[:, j * T:(j + 1) * T]

    def out_cp(r, slot):
        return pltpu.make_async_copy(
            out_buf.at[slot], out_hbm.at[0, pl.ds(pl.multiple_of(r * RB, RB), RB), :], sem_out.at[slot])

    def mix(r, carry):
        slot = r % 2
        rp = pl.ds(pl.multiple_of(r * (RB // 2), RB // 2), RB // 2)

        @pl.when(r >= 2)
        def _():
            out_cp(r - 2, slot).wait()

        logit = None
        for j in range(NC):
            t = _bf(xs32[rp, lanes(j)]).astype(F32) * shift_buf[j, 0:1, :]
            logit = t if logit is None else logit + t
        gate = 1.0 / (1.0 + jnp.exp(-jnp.sum(logit, axis=1, keepdims=True)))
        g_buf[...] = jnp.broadcast_to(gate, (RB, T))
        inv = jnp.concatenate([_bf(f_buf[0:HP, :]), _bf(f_buf[HP:T, :])], axis=1)
        for j in range(NC):
            b = None
            for h0 in range(0, H, 4):
                lhs = jnp.concatenate(
                    [_bf(ctx32[rows8((h0 + u) * (S // 2) + r * (RB // 2), RB // 2), :]) for u in range(4)],
                    axis=1)
                t = _dot(lhs, _bf(wo32[pl.ds(h0 * HP, 4 * HP), lanes(j)]))
                b = t if b is None else b + t
            y = jnp.concatenate(
                [_dot(inv, _bf(buf0[rows8(RES_OFF + (j * NB + r * (RB // T) + u) * T, T), :]))
                 for u in range(RB // T)], axis=0)
            kv = _bf(buf1[rows8(RES_OFF + j * (S // 2) + r * (RB // 2), RB // 2), :]).astype(F32)
            a = _bf(xs32[rp, lanes(j)]).astype(F32) * (y + kv * shift_buf[j, 1:2, :])
            g = g_buf[...]
            out_buf[slot, :, lanes(j)] = (g * a + (1.0 - g) * b).astype(BF16)
        out_cp(r, slot).start()
        return carry

    lax.fori_loop(0, S // RB, mix, 0)
    for r in (S // RB - 2, S // RB - 1):
        out_cp(r, r % 2).wait()


@jax.jit
def pallas_gated_mix__ssm_conv_h3__compressed_kv_cla__prompt_kernel(
    A_q, A_k, A_v, A_shift_k, A_ssm_k, A_ssm_D, B_x, B_c_kv, B_w_q, B_w_uk, B_w_uv, B_w_o, gate_w,
):
    del B_x
    hbm = pl.BlockSpec(memory_space=pl.ANY)
    scratch = [
        pltpu.VMEM((4, DM), BF16),
        pltpu.VMEM((DM,), BF16),
        pltpu.VMEM((DM,), BF16),
        pltpu.VMEM(_FWD.shape, BF16),
        pltpu.VMEM(_INV.shape, BF16),
        pltpu.VMEM((S // 2, DM), U32),
        pltpu.VMEM((S // 2, DC), U32),
        pltpu.VMEM((2, DM + 2 * DC, T), U32),
        pltpu.VMEM((H * HP, DM), U32),
        pltpu.VMEM((NC + 1, K_PITCH, T), U32),
        pltpu.VMEM((NC, S // 2, T), U32),
        pltpu.VMEM((NC, HP, S), U32),
        pltpu.VMEM((4 * NB + 1, 2 * T, T), F32),
        pltpu.VMEM((3, 16 * HP, T), U32),
        pltpu.VMEM((RES_OFF + NC * S, T), U32),
        pltpu.VMEM((RES_OFF + (NC + 1) * S // 2, T), U32),
        pltpu.VMEM((1, T, T), F32),
        pltpu.VMEM((1, T, T), F32),
        pltpu.VMEM((1, T, T), F32),
        pltpu.VMEM((H * S + 4 * T + 16, T), BF16),
        pltpu.VMEM((NC, 8, T), F32),
        pltpu.VMEM((T, T), U32),
        pltpu.VMEM((RB, T), F32),
        pltpu.VMEM((2, RB, DM), BF16),
        pltpu.SemaphoreType.DMA((5,)),
        pltpu.SemaphoreType.DMA((2, len(ROW_CHUNKS) - 1)),
        pltpu.SemaphoreType.DMA((2, 3)),
        pltpu.SemaphoreType.DMA((1,)),
        pltpu.SemaphoreType.DMA((3, NC)),
        pltpu.SemaphoreType.DMA((2,)),
    ] + [pltpu.VMEM((2, T, T), BF16)] * (3 * NB)
    return pl.pallas_call(
        _kernel,
        out_shape=jax.ShapeDtypeStruct((1, S, DM), BF16),
        in_specs=[pl.BlockSpec(memory_space=pltpu.SMEM), *[hbm] * 14],
        out_specs=hbm,
        scratch_shapes=scratch,
        compiler_params=pltpu.CompilerParams(
            vmem_limit_bytes=110 * 1024 * 1024, disable_bounds_checks=bool(CFG['nobc']),
            flags={k: True for k, on in (("XLA_TPU_FORCE_LP_LLO_SCHEDULER", CFG["lp"]),
                                         ("XLA_TPU_EVENLY_DISTRIBUTE_CRITICAL_NODES", CFG["even"])) if on}),
        name="gated_mix_h3_cla",
    )(
        np.zeros((1,), np.int32), A_q, A_k, A_v, A_shift_k.T, A_ssm_k, A_ssm_D, B_c_kv,
        B_w_q, B_w_uk, B_w_uv, B_w_o.reshape(H * DH, DM), gate_w, _FWD, _INV,
    )
```

```python
import functools
import itertools
import math

import jax
import jax.numpy as jnp
import numpy as np
from jax import lax
import jax.experimental.pallas as pl
import jax.experimental.pallas.tpu as pltpu

S = 2048
DM = 1024
H = 32
DH = 128
DC = 512
T = 128
NB = S // T
NC = DM // T
RB = 256
KG = 4

HP = T // 2
PIN_OFF = NB * T
RES_OFF = PIN_OFF + 4 * 8
K_PITCH = 8 + S // 2

ROW_CHUNKS = (0, 2, 4, 6, 9, 12, 16)

import os
CFG = dict(lp=0, order=1, lag=5, prod=1, fwd=1, dmapos=15, nobc=1, pin=2, pb=2, where=5, kg=4, accmem=0, opq=0, mround=0, peel=1, slab_s=128, slab_a=16, zmask=0, even=0, pace=1, lead=2, ppace=1, plead=0, gpace=1, glead=0, zm=1, sts=0, stq=0, wc=1, rep=1, stop=0, wo=0, c0=11, c1=13, fr=8, where1=3)
CFG.update({k: int(v) for k, v in (kv.split("=") for kv in os.environ.get("KCFG", "").split(",") if kv)})

KG = CFG["kg"]
ZM = CFG["zm"]
F32, BF16, U32 = jnp.float32, jnp.bfloat16, jnp.uint32
Q_SCALE = (DH ** -0.5) * math.log2(math.e)
NEG = -1e30
NT_DIMS = (((1,), (1,)), ((), ()))


def _dft_matrices():
    even = 2 * np.arange(64).reshape(8, 8)
    f = np.stack([even, 127 - even], axis=1).reshape(16, 8)
    th = 2.0 * np.pi * (f[..., None] + 0.5) * np.arange(T) / (2 * T)
    fwd = np.stack([np.cos(th), -np.sin(th)], axis=1).reshape(2 * T, T)
    inv = np.stack([np.cos(th[0::2]), -np.sin(th[0::2])], axis=2).reshape(T, T).T / T
    return fwd.astype(BF16), np.concatenate([inv[0::2], inv[1::2]]).astype(BF16)


_FWD, _INV = _dft_matrices()


def _bf(words):
    return pltpu.bitcast(words, BF16)


def _lo(words):
    return pltpu.bitcast(words << 16, F32)


def _hi(words):
    return pltpu.bitcast(words & jnp.uint32(0xFFFF0000), F32)


def _dot(a, b):
    return jnp.dot(a, b, preferred_element_type=F32)


def _key_groups(i):
    return [(j0, min(KG, i + 1 - j0)) for j0 in range(0, i + 1, KG)]


def _head_program(first):
    steps = []
    for i in range(NB):
        nxt = (i + 1) % NB
        sc = [("scores", nxt) + grp for grp in _key_groups(nxt)]
        at = [("attend", i) + grp for grp in _key_groups(i)]
        q, k, v = ("q", (i + 2) % NB), ("k", (i + 2) % NB), ("v", nxt)
        rnd = [x for u in range(NB) for x in sc[u:u + 1] + at[u:u + 1]]
        if i < NB - 2:
            if CFG["order"] == 0:
                rnd = [q, k, v] + rnd
            else:
                u = 4 // KG
                rnd = [q] + rnd[:u] + [k] + rnd[u:3 * u] + [v] + rnd[3 * u:]
            rnd.append(("max", nxt))
        elif i == NB - 2:
            rnd = [v] + rnd + [("max", nxt), q, k]
        else:
            u = 4 // KG
            rnd = at[:u] + [q] + at[u:2 * u] + [k] + at[2 * u:3 * u] + sc + at[3 * u:] + [v, ("max", nxt)]
        if first and i + 2 in ROW_CHUNKS[1:-1]:
            steps.append(("rows", ROW_CHUNKS.index(i + 2)))
        if first and i in (CFG["c0"], CFG["c1"]):
            steps.append(("conv", int(i > CFG["c0"])))
        steps += [("round", i)] + rnd[:1] + [("weights", i)] + rnd[1:]
        if i == CFG["dmapos"]:
            steps.append(("dma", i))
    return steps


def _kernel(zero_ref, x_hbm, k_hbm, v_hbm, sk_hbm, h_hbm, d_hbm, c_hbm, wq_hbm, wk_hbm, wv_hbm, wo_hbm,
            gw_hbm, fwd_hbm, inv_hbm, out_hbm,
            sk_ref, d_ref, gw_ref, fwd_ref, inv_ref,
            xs32, cs32, w_raw, wo32, ks32, vs32, hs32, spec, w_cur, buf0, buf1, mx_buf, l_buf, o_buf,
            ctx, shift_buf, f_buf, g_buf, b_buf, out_buf,
            sem_small, sem_rows, sem_w, sem_wo, sem_conv, sem_out, *qkv):
    q_buf, k_buf, v_buf = qkv[:NB], qkv[NB:2 * NB], qkv[2 * NB:]
    x_hbm, k_hbm, v_hbm, h_hbm, c_hbm, wq_hbm, wk_hbm, wv_hbm, wo_hbm = (
        r.bitcast(U32) for r in (x_hbm, k_hbm, v_hbm, h_hbm, c_hbm, wq_hbm, wk_hbm, wv_hbm, wo_hbm))
    bufs = (buf0, buf1)
    ctx32, m_buf = ctx.bitcast(U32), ctx.bitcast(F32)
    M_OFF = H * S // 2

    def lanes(j):
        return pl.ds(j * T, T)

    def rows8(start, n):
        return pl.ds(start if isinstance(start, int) else pl.multiple_of(start, 8), n)

    def load_f32(buf, start, n):
        return pltpu.bitcast(buf[rows8(start, n), :], F32)

    def store_f32(buf, start, value):
        buf[rows8(start, value.shape[0]), :] = pltpu.bitcast(value, U32)

    def rows_cp(n):
        rows = pl.ds(ROW_CHUNKS[n] * HP, (ROW_CHUNKS[n + 1] - ROW_CHUNKS[n]) * HP)
        return [pltpu.make_async_copy(src.at[0, rows], dst.at[rows], sem_rows.at[i, n])
                for i, (src, dst) in enumerate(((c_hbm, cs32), (x_hbm, xs32)))]

    wo_cp = pltpu.make_async_copy(wo_hbm, wo32, sem_wo.at[0])

    def w_cp(p):
        return [pltpu.make_async_copy(src.at[:, p, :], w_raw.at[p & 1, pl.ds(r0, n)], sem_w.at[p & 1, i])
                for i, (src, r0, n) in enumerate(
                    ((wq_hbm, 0, DM), (wk_hbm, DM, DC), (wv_hbm, DM + DC, DC)))]

    def conv_cp(c):
        col = pl.ds(pl.multiple_of(c * T, T), T)
        return [
            pltpu.make_async_copy(k_hbm.at[0, :, col], ks32.at[c, pl.ds(8, S // 2)], sem_conv.at[0, c]),
            pltpu.make_async_copy(v_hbm.at[0, :, col], vs32.at[c], sem_conv.at[1, c]),
            pltpu.make_async_copy(h_hbm.at[pl.ds(pl.multiple_of(c * HP, HP), HP)], hs32.at[c],
                                  sem_conv.at[2, c]),
        ]

    def unpack_weights(h, t):
        slot = (h >> 1) & 1
        sh = ((h & 1) * 16).astype(U32)
        even = w_raw[slot, pl.ds(t * T, HP, stride=2), :]
        odd = w_raw[slot, pl.ds(t * T + 1, HP, stride=2), :]
        return ((even >> sh) & jnp.uint32(0xFFFF)) | ((odd >> sh) << 16)

    def lhs_cat(src, i, j0, n):
        return jnp.concatenate([_bf(src[pl.ds(i * HP, HP), lanes(j0 + j)]) for j in range(n)], axis=1)

    w_cache = {}

    def w_cat(h, t0, n):
        h, ahead = h
        if (ahead, t0) not in w_cache or not CFG["wc"]:
            w_cache[ahead, t0] = _bf(w_cur[(h + ahead) & 1, pl.ds(t0 * HP, n * HP), :])
        return w_cache[ahead, t0]

    stream = []

    def recent(slab):
        n, r = divmod(slab, 8)
        if len(stream) < 2 - n:
            return None
        return stream[n - 2][16 * r + 8:16 * r + 16, 0:T]

    def keep(buf, z, value):
        buf[z * (1 - CFG["stq"])] = value.astype(BF16)
        if CFG["stq"]:
            buf.bitcast(F32)[z + 1, T // 2 - 8:T // 2, :] = value[T - 8:T]

    def proj_q(z, h, i):
        qa, qb = (_dot(lhs_cat(xs32, i, t, 4), w_cat(h, t, 4)) for t in (0, 4))
        q = qa + qb
        keep(q_buf[i], z, q * Q_SCALE)
        stream.extend([qa, qb])

    def proj_k(z, h, i):
        stream.append(_dot(lhs_cat(cs32, i, 0, 4), w_cat(h, 8, 4)))
        keep(k_buf[i], z, stream[-1])

    def proj_v(z, h, i):
        stream.append(_dot(lhs_cat(cs32, i, 0, 4), w_cat(h, 12, 4)))
        keep(v_buf[i], z, stream[-1])

    def tiles_of(buf, j0, n, z=0):
        return _bf(jnp.concatenate([buf[j0 + j].bitcast(U32)[z] for j in range(n)], axis=0))

    def scores(z, i, j0, n):
        s = lax.dot_general(tiles_of(q_buf, i, 1), tiles_of(k_buf, j0, n, z * CFG['opq']), NT_DIMS,
                            preferred_element_type=F32)
        stream.append(s)
        R = CFG["slab_s"]
        diff = lax.broadcasted_iota(jnp.int32, (R, T), 1) - lax.broadcasted_iota(jnp.int32, (R, T), 0)
        for r in range(0, T, R):
            mx = None if j0 == 0 else mx_buf[0, r:r + R, :]
            for j in range(n):
                t = s[r:r + R, j * T:(j + 1) * T]
                if j0 + j == i:
                    t = jnp.where(diff <= r + z * CFG["zmask"], t, NEG)
                store_f32(bufs[i % 2], z * (1 - CFG['sts']) + (j0 + j) * T + r, t)
                mx = t if mx is None else jnp.maximum(mx, t)
            mx_buf[z * CFG['accmem'], r:r + R, :] = mx

    def row_max(z, i):
        if CFG["sts"]:
            store_f32(bufs[i % 2], z + PIN_OFF, mx_buf[0, T - 8:T, :])
        m_buf[rows8(z * ZM + M_OFF + i % 2 * T, T), :] = jnp.broadcast_to(
            jnp.max(mx_buf[0], axis=1, keepdims=True), (T, T))

    def attend(z, h, i, j0, n):
        R = CFG["slab_a"]
        last = j0 + n == i + 1
        slabs, ls = [], []
        for r in range(0, T, R):
            pace = recent(r // 16 + CFG["lead"] - 8) if CFG["pace"] else None
            if pace is not None:
                m_buf[rows8(z * ZM + M_OFF + 2 * T, 8), :] = pace
            m = m_buf[rows8(M_OFF + i % 2 * T + r, R), :]
            l = None if j0 == 0 else l_buf[0, r:r + R, :]
            ps = []
            for j in range(n):
                p = jnp.exp2(load_f32(bufs[i % 2], (j0 + j) * T + r, R) - m)
                l = p if l is None else l + p
                ps.append(p)
            slabs.append(jnp.concatenate(ps, axis=1))
            if last:
                total = jnp.sum(l, axis=1, keepdims=True)
                rcp = pl.reciprocal(total, approx=True)
                ls.append(rcp * (2.0 - total * rcp))
            else:
                l_buf[z * CFG['accmem'], r:r + R, :] = l
        o = _dot(jnp.concatenate(slabs, axis=0).astype(BF16), tiles_of(v_buf, j0, n, z * CFG['opq']))
        stream.append(o)
        R = max(R, 16)
        if last:
            ls = jnp.concatenate(ls, axis=0)
        for r in range(0, T, R):
            t = o[r:r + R]
            if j0 > 0:
                t = t + o_buf[0, r:r + R, :]
            if last:
                ctx[pl.ds(pl.multiple_of(h * S + i * T + r, R), R), :] = (t * ls[r:r + R]).astype(BF16)
            else:
                o_buf[z * CFG['accmem'], r:r + R, :] = t

    def gate_kv(c, c_out, r8, n):
        r = r8 * 8
        pace = recent(CFG["glead"] - 8) if CFG["gpace"] and n < HP else None
        if pace is not None:
            ks32[NC + (c >> 3), 0:8, :] = pltpu.bitcast(pace, U32)
        w0, w1, w2 = ks32[c, rows8(r + 8, n), :], ks32[c, pl.ds(r + 7, n), :], ks32[c, pl.ds(r + 6, n), :]
        e0, o0, e1, o1, o2 = _lo(w0), _hi(w0), _lo(w1), _hi(w1), _hi(w2)
        s0, s1, s2, s3 = (shift_buf[c, j:j + 1, :] for j in range(4))
        even = s3 * o2 + s2 * e1 + s1 * o1 + s0 * e0
        odd = s3 * e1 + s2 * o1 + s1 * e0 + s0 * o0
        vw = vs32[c, rows8(r, n), :]
        buf1[rows8(RES_OFF + c_out * (S // 2) + r, n), :] = pltpu.pack_elementwise(
            [even * _lo(vw), odd * _hi(vw)], packed_dtype=BF16)

    def forward_x(c, a):
        return _dot(_bf(f_buf[...]), _bf(buf1[rows8(RES_OFF + c * (S // 2) + a * HP, HP), :]))

    def forward_h(c, a):
        taps = _bf(hs32[c, :, pl.ds(pl.multiple_of(a * T, T), T)])
        return lax.dot_general(_bf(f_buf[...]), taps, NT_DIMS, preferred_element_type=F32)

    def product(c, g, odd, a0, b0, b1, acc, pin):
        def load(which, chunk):
            slot = (which * 2 + (c & 1)) * NB + chunk
            return spec[slot, rows8(g * 16, 8), :], spec[slot, rows8(g * 16 + 8, 8), :]

        pace = recent(CFG["plead"] - 8) if CFG["ppace"] else None
        if pace is not None:
            spec[(c >> 3) + 4 * NB, 0:8, :] = pace
        taps = {}
        for b in range(b0, b1):
            xr, xi = load(0, b)
            for a in range(max(a0, b), a0 + 2):
                if a - b not in taps:
                    taps[a - b] = load(1, a - b)
                hr, hi = taps[a - b]
                pr, pi = hr * xr - hi * xi, hr * xi + hi * xr
                acc[odd, a] = (acc[odd, a][0] + pr, acc[odd, a][1] + pi) if b else (pr, pi)
        for u, a in enumerate((a0, a0 + 1)):
            zr, zi = acc[odd, a]
            if b1 < a0 + 2:
                if CFG["pin"]:
                    pin(16 * u, pltpu.bitcast(zr, U32))
                    pin(16 * u + 8, pltpu.bitcast(zi, U32))
                continue
            if a:
                tr, ti = acc[odd, a - 1]
                zr, zi = (zr + ti, zi - tr) if odd else (zr - ti, zi + tr)
            if not odd:
                acc["mirror", a] = zr, zi
                pin(16 * u, pltpu.bitcast(zr, U32))
                pin(16 * u + 8, pltpu.bitcast(zi, U32))
                continue
            mr, mi = acc["mirror", a]
            for half, pair in enumerate(([mr + zr, mi - zi], [mr - zr, mi + zi])):
                y = pltpu.pack_elementwise(pair, packed_dtype=BF16)
                buf0[rows8(RES_OFF + (c * NB + a) * T + half * HP + (g >> 1) * 8, 8), :] = y
                pin(16 * u + 8 * half, y)

    small_cp = [pltpu.make_async_copy(src, dst, sem_small.at[i]) for i, (src, dst) in enumerate(
        ((sk_hbm, sk_ref), (fwd_hbm, fwd_ref), (inv_hbm, inv_ref), (gw_hbm, gw_ref), (d_hbm, d_ref)))]
    for cp in (w_cp(0) + [cp for n in range(len(ROW_CHUNKS) - 1) for cp in rows_cp(n)]
               + small_cp + conv_cp(0) + conv_cp(1) + w_cp(1)):
        cp.start()
    ks32[0:NC, 0:8, :] = jnp.zeros((NC, 8, T), U32)
    for cp in w_cp(0) + rows_cp(0):
        cp.wait()
    for t in range(16):
        w_cur[0, pl.ds(t * HP, HP), :] = unpack_weights(jnp.int32(0), t)
    proj_q(zero_ref[0], (0, 0), 0)
    proj_k(zero_ref[0], (0, 0), 0)
    proj_q(zero_ref[0], (0, 0), 1)
    scores(zero_ref[0], 0, 0, 1)
    proj_k(zero_ref[0], (0, 0), 1)
    proj_v(zero_ref[0], (0, 0), 0)
    row_max(zero_ref[0], 0)

    def first_transforms():
        for cp in small_cp + conv_cp(0):
            cp.wait()
        f_buf[...] = pltpu.bitcast(fwd_ref[...], U32)
        shift_taps = sk_ref[...].astype(F32)
        for j in range(NC):
            shift_buf[j, 0:4, :] = shift_taps[:, j * T:(j + 1) * T]
        for a in range(NB):
            gate_kv(0, 0, a * HP // 8, HP)
            spec[a] = forward_x(0, a)
            spec[2 * NB + a] = forward_h(0, a)

    def head(h, first):
        c, quarter = h >> 2, h & 3
        cn = jnp.minimum(c + 1, NC - 1)
        hn = jnp.minimum(h + 1, H - 1)
        z = h >> 5

        def dma():
            if first:
                wo_cp.start()

            @pl.when(jnp.logical_and(quarter == 3, c + 2 < NC))
            def _():
                for cp in conv_cp(jnp.minimum(c + 2, NC - 1)):
                    cp.wait()

            @pl.when(jnp.logical_and(quarter == 0, c + 2 < NC))
            def _():
                for cp in conv_cp(jnp.minimum(c + 2, NC - 1)):
                    cp.start()

            @pl.when(jnp.logical_and((h & 1) == 0, h + 2 < H))
            def _():
                for cp in w_cp(jnp.minimum((h >> 1) + 1, H // 2 - 1)):
                    cp.wait()

            @pl.when(jnp.logical_and((h & 1) == 1, h + 3 < H))
            def _():
                for cp in w_cp(jnp.minimum((h >> 1) + 2, H // 2 - 1)):
                    cp.start()

        steps = _head_program(first)
        rounds = list(itertools.accumulate(st[0] == "round" for st in steps))
        stream.clear()
        w_cache.clear()
        users = [n for n, st in enumerate(steps) if st[0] in ("scores", "attend")]
        parity = [steps[n][1] % 2 for n in users]
        tasks = {n: [] for n in users}
        PB = CFG["pb"]
        pieces = [(gi, a0, b0, min(b0 + PB, a0 + 2))
                  for g0 in (0, 2) for a0 in range(0, NB, 2) for gi in (g0, g0 + 1)
                  for b0 in range(0, a0 + 2, PB)]
        hosts = [n for n, st in enumerate(steps)
                 if st[0] in (("scores", "attend"), ("scores",), ("attend",), ("scores", "attend", "q", "k", "v"),
                              ("k", "v"), ("q", "k", "v"))[CFG["where1" if first else "where"]]
                 and (not first or rounds[n] > CFG["c0"])]

        def pin_of(st):
            if st[0] in ("scores", "attend"):
                buf, slot = (k_buf if st[0] == "scores" else v_buf)[st[2]].bitcast(U32), z + 1
            elif CFG["pin"] == 2:
                buf, slot = dict(q=q_buf, k=k_buf, v=v_buf)[st[0]][st[1]].bitcast(U32), z + 1
            elif CFG["pin"] == 3:
                buf, slot = spec.bitcast(U32), z + 4 * NB
            else:
                buf, slot = w_cur, z + 2

            def pin(r, y):
                buf[slot, pl.ds(r, 8), :] = y
            return pin

        acc, held = {}, {}
        for u, (gi, a0, b0, b1) in enumerate(pieces if CFG['prod'] else []):
            n = hosts[u * len(hosts) // len(pieces)]
            tasks.setdefault(n, []).append(functools.partial(
                product, c, quarter * 4 + gi, gi % 2, a0, b0, b1, acc, pin_of(steps[n])))

        def forward(name, fn, *args):
            held[name] = fn(*args)

        def spec_store(name, slot):
            spec[slot] = held.pop(name)

        late = [n for n in users if steps[n][0] == "attend" and steps[n][1] >= CFG["c1" if first else "fr"]]
        odd, even = ([n for n in late if steps[n][1] % 2 == par] for par in (1, 0))
        for u in range(4 * CFG['fwd']):
            a = quarter * 4 + u
            for r in range(4):
                tasks[odd[(5 * u + r) * len(odd) // 20]].append(
                    functools.partial(gate_kv, cn, c + 1, a * 8 + 2 * r, 16))
            for which, n, fn, tile in ((0, odd[(5 * u + 4) * len(odd) // 20], forward_x, c + 1),
                                       (1, even[u * len(even) // 4], forward_h, cn)):
                tasks[n].append(functools.partial(forward, (which, u), fn, tile, a))
                after = min(n + CFG["lag"], len(steps) - 1)
                tasks.setdefault(after, []).insert(0, functools.partial(
                    spec_store, (which, u), (which * 2 + ((c + 1) & 1)) * NB + a))

        for n, st in enumerate(steps):
            for task in tasks.get(n, ()):
                task()
            kind, i = st[:2]
            if CFG["opq"] and kind in ("scores", "attend"):
                z = (h + i) >> 6
            if kind == "weights":
                w_cur[(h + 1) & 1, pl.ds(i * HP, HP), :] = unpack_weights(hn, i)
            elif kind == "round":
                pass
            elif kind == "rows":
                for cp in rows_cp(i):
                    cp.wait()
            elif kind == "conv":
                for cp in conv_cp(1) if i else ():
                    cp.wait()
                if not i:
                    first_transforms()
            elif kind == "dma":
                dma()
            elif kind == "scores":
                scores(z, *st[1:])
            elif kind == "attend":
                attend(z, h, *st[1:])
            elif kind == "max":
                row_max(z, i)
            elif kind == "v":
                proj_v(z, (h, int(i == 0)), i)
            else:
                (proj_q if kind == "q" else proj_k)(z, (h, int(i < 2)), i)

    if CFG['peel']:
        head(zero_ref[0], True)
    if CFG["stop"] == 1:
        wo_cp.wait()
        for cp in conv_cp(2):
            cp.wait()
        return
    lax.fori_loop(1, H, lambda h, _: head(h, False), None)
    if CFG["rep"] > 1:
        lax.fori_loop(0, 16, lambda h, _: head(jnp.maximum(h, H - 1), False), None)

    wo_cp.wait()
    if CFG['stop'] == 2:
        return
    f_buf[0:HP, :] = pltpu.bitcast(inv_ref[...], U32)
    gate_w = gw_ref[...].astype(F32).reshape(1, DM)
    skip_d = d_ref[...].astype(F32).reshape(1, DM)
    for j in range(NC):
        shift_buf[j, 0:1, :] = gate_w[:, j * T:(j + 1) * T]
        shift_buf[j, 1:2, :] = skip_d[:, j * T:(j + 1) * T]

    def out_cp(r, slot):
        return pltpu.make_async_copy(
            out_buf.at[slot], out_hbm.bitcast(U32).at[0, rows8(r * (RB // 2), RB // 2), :], sem_out.at[slot])

    def mix(r, carry):
        slot = r % 2
        rp = pl.ds(pl.multiple_of(r * (RB // 2), RB // 2), RB // 2)

        @pl.when(r >= 2)
        def _():
            out_cp(r - 2, slot).wait()

        for half, part in enumerate((_lo, _hi)):
            logit = None
            for j in range(NC):
                t = part(xs32[rp, lanes(j)]) * shift_buf[j, 0:1, :]
                logit = t if logit is None else logit + t
            gate = 1.0 / (1.0 + jnp.exp(-jnp.sum(logit, axis=1, keepdims=True)))
            g_buf[half] = jnp.broadcast_to(gate, (RB // 2, T))
        for j in range(NC):
            b = None
            for h0 in range(0, H, 4):
                lhs = jnp.concatenate(
                    [_bf(ctx32[rows8((h0 + u) * (S // 2) + r * (RB // 2), RB // 2), :]) for u in range(4)],
                    axis=1)
                t = _dot(lhs, _bf(wo32[pl.ds(h0 * HP, 4 * HP), lanes(j)]))
                b = t if b is None else b + t
            b_buf[j] = b
            halves = []
            for half, part in enumerate((_lo, _hi)):
                y = jnp.concatenate(
                    [_dot(_bf(f_buf[half * HP // 2:(half + 1) * HP // 2, :]),
                          _bf(buf0[rows8(RES_OFF + (j * NB + r * (RB // T) + u) * T + half * HP, HP), :]))
                     for u in range(RB // T)], axis=0)
                kv = part(buf1[rows8(RES_OFF + j * (S // 2) + r * (RB // 2), RB // 2), :])
                a = part(xs32[rp, lanes(j)]) * (y + kv * shift_buf[j, 1:2, :])
                g = g_buf[half]
                halves.append(g * a + (1.0 - g) * b_buf[j, pl.ds(half, RB // 2, stride=2), :])
            out_buf[slot, :, lanes(j)] = pltpu.pack_elementwise(halves, packed_dtype=BF16)
        out_cp(r, slot).start()
        return carry

    lax.fori_loop(0, S // RB, mix, 0)
    for r in (S // RB - 2, S // RB - 1):
        out_cp(r, r % 2).wait()


@jax.jit
def pallas_gated_mix__ssm_conv_h3__compressed_kv_cla__prompt_kernel(
    A_q, A_k, A_v, A_shift_k, A_ssm_k, A_ssm_D, B_x, B_c_kv, B_w_q, B_w_uk, B_w_uv, B_w_o, gate_w,
):
    del B_x
    hbm = pl.BlockSpec(memory_space=pl.ANY)
    scratch = [
        pltpu.VMEM((4, DM), BF16),
        pltpu.VMEM((DM,), BF16),
        pltpu.VMEM((DM,), BF16),
        pltpu.VMEM(_FWD.shape, BF16),
        pltpu.VMEM(_INV.shape, BF16),
        pltpu.VMEM((S // 2, DM), U32),
        pltpu.VMEM((S // 2, DC), U32),
        pltpu.VMEM((2, DM + 2 * DC, T), U32),
        pltpu.VMEM((H * HP, DM), U32),
        pltpu.VMEM((NC + 1, K_PITCH, T), U32),
        pltpu.VMEM((NC, S // 2, T), U32),
        pltpu.VMEM((NC, HP, S), U32),
        pltpu.VMEM((4 * NB + 1, 2 * T, T), F32),
        pltpu.VMEM((3, 16 * HP, T), U32),
        pltpu.VMEM((RES_OFF + NC * S, T), U32),
        pltpu.VMEM((RES_OFF + (NC + 1) * S // 2, T), U32),
        pltpu.VMEM((1, T, T), F32),
        pltpu.VMEM((1, T, T), F32),
        pltpu.VMEM((1, T, T), F32),
        pltpu.VMEM((H * S + 4 * T + 16, T), BF16),
        pltpu.VMEM((NC, 8, T), F32),
        pltpu.VMEM((T, T), U32),
        pltpu.VMEM((2, RB // 2, T), F32),
        pltpu.VMEM((NC, RB, T), F32),
        pltpu.VMEM((2, RB // 2, DM), U32),
        pltpu.SemaphoreType.DMA((5,)),
        pltpu.SemaphoreType.DMA((2, len(ROW_CHUNKS) - 1)),
        pltpu.SemaphoreType.DMA((2, 3)),
        pltpu.SemaphoreType.DMA((1,)),
        pltpu.SemaphoreType.DMA((3, NC)),
        pltpu.SemaphoreType.DMA((2,)),
    ] + [pltpu.VMEM((2, T, T), BF16)] * (3 * NB)
    return pl.pallas_call(
        _kernel,
        out_shape=jax.ShapeDtypeStruct((1, S, DM), BF16),
        in_specs=[pl.BlockSpec(memory_space=pltpu.SMEM), *[hbm] * 14],
        out_specs=hbm,
        scratch_shapes=scratch,
        compiler_params=pltpu.CompilerParams(
            vmem_limit_bytes=110 * 1024 * 1024, disable_bounds_checks=bool(CFG['nobc']),
            flags={k: True for k, on in (("XLA_TPU_FORCE_LP_LLO_SCHEDULER", CFG["lp"]),
                                         ("XLA_TPU_EVENLY_DISTRIBUTE_CRITICAL_NODES", CFG["even"])) if on}),
        name="gated_mix_h3_cla",
    )(
        np.zeros((1,), np.int32), A_q, A_k, A_v, A_shift_k.T, A_ssm_k, A_ssm_D, B_c_kv,
        B_w_q, B_w_uk, B_w_uv, B_w_o.reshape(H * DH, DM), gate_w, _FWD, _INV,
    )
```

```python
import functools
import itertools
import math

import jax
import jax.numpy as jnp
import numpy as np
from jax import lax
import jax.experimental.pallas as pl
import jax.experimental.pallas.tpu as pltpu

S = 2048
DM = 1024
H = 32
DH = 128
DC = 512
T = 128
NB = S // T
NC = DM // T
RB = 256
KG = 4

HP = T // 2
PIN_OFF = NB * T
RES_OFF = PIN_OFF + 4 * 8
K_PITCH = 8 + S // 2

ROW_CHUNKS = (0, 2, 4, 6, 9, 12, 16)

import os
CFG = dict(lp=0, order=1, lag=6, prod=1, fwd=1, dmapos=15, nobc=1, pin=2, pb=2, where=5, kg=4, accmem=1, opq=0, mround=0, peel=1, slab_s=128, slab_a=32, zmask=1, even=0, pace=1, lead=1, ppace=1, plead=4, gpace=1, glead=0, zm=1, sts=0, stq=0, wc=1, rep=1, stop=0, wo=0, c0=11, c1=13, fr=6, unroll=1, rdd=0, skew=13, wpos=1, where1=3)
CFG.update({k: int(v) for k, v in (kv.split("=") for kv in os.environ.get("KCFG", "").split(",") if kv)})

KG = CFG["kg"]
ZM = CFG["zm"]
F32, BF16, U32 = jnp.float32, jnp.bfloat16, jnp.uint32
Q_SCALE = (DH ** -0.5) * math.log2(math.e)
NEG = -1e30
NT_DIMS = (((1,), (1,)), ((), ()))


def _dft_matrices():
    even = 2 * np.arange(64).reshape(8, 8)
    f = np.stack([even, 127 - even], axis=1).reshape(16, 8)
    th = 2.0 * np.pi * (f[..., None] + 0.5) * np.arange(T) / (2 * T)
    fwd = np.stack([np.cos(th), -np.sin(th)], axis=1).reshape(2 * T, T)
    inv = np.stack([np.cos(th[0::2]), -np.sin(th[0::2])], axis=2).reshape(T, T).T / T
    return fwd.astype(BF16), np.concatenate([inv[0::2], inv[1::2]]).astype(BF16)


_FWD, _INV = _dft_matrices()


def _bf(words):
    return pltpu.bitcast(words, BF16)


def _lo(words):
    return pltpu.bitcast(words << 16, F32)


def _hi(words):
    return pltpu.bitcast(words & jnp.uint32(0xFFFF0000), F32)


def _dot(a, b):
    return jnp.dot(a, b, preferred_element_type=F32)


def _key_groups(i):
    return [(j0, min(KG, i + 1 - j0)) for j0 in range(0, i + 1, KG)]


def _head_program(first):
    steps = []
    for i in range(NB):
        nxt = (i + 1) % NB
        sc = [("scores", nxt) + grp for grp in _key_groups(nxt)]
        at = [("attend", i) + grp for grp in _key_groups(i)]
        q, k, v = ("q", (i + 2) % NB), ("k", (i + 2) % NB), ("v", nxt)
        rnd = [x for u in range(NB) for x in sc[u:u + 1] + at[u:u + 1]]
        if i < NB - 2:
            if CFG["order"] == 0:
                rnd = [q, k, v] + rnd
            else:
                u = 4 // KG
                rnd = [q] + rnd[:u] + [k] + rnd[u:3 * u] + [v] + rnd[3 * u:]
            rnd.append(("max", nxt))
        elif i == NB - 2:
            rnd = [v] + rnd + [("max", nxt), q, k]
        else:
            u = 4 // KG
            rnd = at[:u] + [q] + at[u:2 * u] + [k] + at[2 * u:3 * u] + sc + at[3 * u:] + [v, ("max", nxt)]
        if first and i + 2 in ROW_CHUNKS[1:-1]:
            steps.append(("rows", ROW_CHUNKS.index(i + 2)))
        if first and i in (CFG["c0"], CFG["c1"]):
            steps.append(("conv", int(i > CFG["c0"])))
        steps += [("round", i)] + rnd[:CFG["wpos"]] + [("weights", i)] + rnd[CFG["wpos"]:]
        if i == CFG["dmapos"]:
            steps.append(("start", i))
    return steps + [("wait", 0)]


def _kernel(zero_ref, x_hbm, k_hbm, v_hbm, sk_hbm, h_hbm, d_hbm, c_hbm, wq_hbm, wk_hbm, wv_hbm, wo_hbm,
            gw_hbm, fwd_hbm, inv_hbm, out_hbm,
            sk_ref, d_ref, gw_ref, fwd_ref, inv_ref,
            xs32, cs32, w_raw, wo32, ks32, vs32, hs32, spec, w_cur, buf0, buf1, mx_buf, l_buf, o_buf,
            ctx, shift_buf, f_buf, g_buf, b_buf, out_buf,
            sem_small, sem_rows, sem_w, sem_wo, sem_conv, sem_out, *qkv):
    q_buf, k_buf, v_buf = qkv[:NB], qkv[NB:2 * NB], qkv[2 * NB:]
    x_hbm, k_hbm, v_hbm, h_hbm, c_hbm, wq_hbm, wk_hbm, wv_hbm, wo_hbm = (
        r.bitcast(U32) for r in (x_hbm, k_hbm, v_hbm, h_hbm, c_hbm, wq_hbm, wk_hbm, wv_hbm, wo_hbm))
    bufs = (buf0, buf1)
    ctx32, m_buf = ctx.bitcast(U32), ctx.bitcast(F32)
    M_OFF = H * S // 2

    def lanes(j):
        return pl.ds(j * T, T)

    def rows8(start, n):
        return pl.ds(start if isinstance(start, int) else pl.multiple_of(start, 8), n)

    def load_f32(buf, start, n):
        return pltpu.bitcast(buf[rows8(start, n), :], F32)

    def store_f32(buf, start, value):
        buf[rows8(start, value.shape[0]), :] = pltpu.bitcast(value, U32)

    def rows_cp(n):
        rows = pl.ds(ROW_CHUNKS[n] * HP, (ROW_CHUNKS[n + 1] - ROW_CHUNKS[n]) * HP)
        return [pltpu.make_async_copy(src.at[0, rows], dst.at[rows], sem_rows.at[i, n])
                for i, (src, dst) in enumerate(((c_hbm, cs32), (x_hbm, xs32)))]

    wo_cp = pltpu.make_async_copy(wo_hbm, wo32, sem_wo.at[0])

    def w_cp(p):
        return [pltpu.make_async_copy(src.at[:, p, :], w_raw.at[p & 1, pl.ds(r0, n)], sem_w.at[p & 1])
                for i, (src, r0, n) in enumerate(
                    ((wq_hbm, 0, DM), (wk_hbm, DM, DC), (wv_hbm, DM + DC, DC)))]

    def w_wait(p):
        pltpu.make_async_copy(w_raw.at[p & 1], w_raw.at[p & 1], sem_w.at[p & 1]).wait()

    def conv_cp(c):
        col = pl.ds(pl.multiple_of(c * T, T), T)
        return [
            pltpu.make_async_copy(k_hbm.at[0, :, col], ks32.at[c, pl.ds(8, S // 2)], sem_conv.at[0, c & 1]),
            pltpu.make_async_copy(v_hbm.at[0, :, col], vs32.at[c], sem_conv.at[1, c & 1]),
            pltpu.make_async_copy(h_hbm.at[pl.ds(pl.multiple_of(c * HP, HP), HP)], hs32.at[c],
                                  sem_conv.at[2, c & 1]),
        ]

    def unpack_weights(h, t):
        slot = (h >> 1) & 1
        sh = ((h & 1) * 16).astype(U32)
        even = w_raw[slot, pl.ds(t * T, HP, stride=2), :]
        odd = w_raw[slot, pl.ds(t * T + 1, HP, stride=2), :]
        return ((even >> sh) & jnp.uint32(0xFFFF)) | ((odd >> sh) << 16)

    def lhs_cat(src, i, j0, n):
        return jnp.concatenate([_bf(src[pl.ds(i * HP, HP), lanes(j0 + j)]) for j in range(n)], axis=1)

    w_cache = {}

    def w_cat(h, t0, n):
        h, ahead = h
        if (ahead, t0) not in w_cache or not CFG["wc"]:
            w_cache[ahead, t0] = _bf(w_cur[(h + ahead) & 1, pl.ds(t0 * HP, n * HP), :])
        return w_cache[ahead, t0]

    stream = []

    def recent(slab):
        n, r = divmod(slab, 8)
        if len(stream) < 2 - n:
            return None
        return stream[n - 2][16 * r + 8:16 * r + 16, 0:T]

    def keep(buf, z, value):
        buf[z * (1 - CFG["stq"])] = value.astype(BF16)
        if CFG["stq"]:
            buf.bitcast(F32)[z + 1, T // 2 - 8:T // 2, :] = value[T - 8:T]

    def proj_q(z, h, i):
        qa, qb = (_dot(lhs_cat(xs32, i, t, 4), w_cat(h, t, 4)) for t in (0, 4))
        q = qa + qb
        keep(q_buf[i], z, q * Q_SCALE)
        stream.extend([qa, qb])

    def proj_k(z, h, i):
        stream.append(_dot(lhs_cat(cs32, i, 0, 4), w_cat(h, 8, 4)))
        keep(k_buf[i], z, stream[-1])

    def proj_v(z, h, i):
        stream.append(_dot(lhs_cat(cs32, i, 0, 4), w_cat(h, 12, 4)))
        keep(v_buf[i], z, stream[-1])

    def tiles_of(buf, j0, n, z=0):
        return _bf(jnp.concatenate([buf[j0 + j].bitcast(U32)[z] for j in range(n)], axis=0))

    def scores(z, i, j0, n):
        s = lax.dot_general(tiles_of(q_buf, i, 1), tiles_of(k_buf, j0, n, z * CFG['opq']), NT_DIMS,
                            preferred_element_type=F32)
        stream.append(s)
        R = CFG["slab_s"]
        diff = lax.broadcasted_iota(jnp.int32, (R, T), 1) - lax.broadcasted_iota(jnp.int32, (R, T), 0)
        for r in range(0, T, R):
            mx = None if j0 == 0 else mx_buf[0, r:r + R, :]
            for j in range(n):
                t = s[r:r + R, j * T:(j + 1) * T]
                if j0 + j == i:
                    t = jnp.where(diff <= r + z * CFG["zmask"], t, NEG)
                store_f32(bufs[i % 2], z * (1 - CFG['sts']) + (j0 + j) * T + r, t)
                mx = t if mx is None else jnp.maximum(mx, t)
            mx_buf[z * CFG['accmem'], r:r + R, :] = mx

    def row_max(z, i):
        if CFG["sts"]:
            store_f32(bufs[i % 2], z + PIN_OFF, mx_buf[0, T - 8:T, :])
        m_buf[rows8(z * ZM + M_OFF + i % 2 * T, T), :] = jnp.broadcast_to(
            jnp.max(mx_buf[0], axis=1, keepdims=True), (T, T))

    def attend(z, h, i, j0, n):
        R = CFG["slab_a"]
        last = j0 + n == i + 1
        slabs, ls = [], []
        for r in range(0, T, R):
            pace = recent(r // 16 + CFG["lead"] - 8) if CFG["pace"] else None
            if pace is not None:
                m_buf[rows8(z * ZM + M_OFF + 2 * T, 8), :] = pace
            m = m_buf[rows8(M_OFF + i % 2 * T + r, R), :]
            l = None if j0 == 0 else l_buf[0, r:r + R, :]
            ps = []
            for j in range(n):
                p = jnp.exp2(load_f32(bufs[i % 2], (j0 + j) * T + r, R) - m)
                l = p if l is None else l + p
                ps.append(p)
            slabs.append(jnp.concatenate(ps, axis=1))
            if last:
                total = jnp.sum(l, axis=1, keepdims=True)
                rcp = pl.reciprocal(total, approx=True)
                ls.append(rcp * (2.0 - total * rcp))
            else:
                l_buf[z * CFG['accmem'], r:r + R, :] = l
        o = _dot(jnp.concatenate(slabs, axis=0).astype(BF16), tiles_of(v_buf, j0, n, z * CFG['opq']))
        stream.append(o)
        R = max(R, 16)
        if last:
            ls = jnp.concatenate(ls, axis=0)
        for r in range(0, T, R):
            t = o[r:r + R]
            if j0 > 0:
                t = t + o_buf[0, r:r + R, :]
            if last:
                ctx[pl.ds(pl.multiple_of(h * S + i * T + r, R), R), :] = (t * ls[r:r + R]).astype(BF16)
            else:
                o_buf[z * CFG['accmem'], r:r + R, :] = t

    def gate_kv(c, c_out, r8, n):
        r = r8 * 8
        pace = recent(CFG["glead"] - 8) if CFG["gpace"] and n < HP else None
        if pace is not None:
            ks32[NC + (c >> 3), 0:8, :] = pltpu.bitcast(pace, U32)
        w0, w1, w2 = ks32[c, rows8(r + 8, n), :], ks32[c, pl.ds(r + 7, n), :], ks32[c, pl.ds(r + 6, n), :]
        e0, o0, e1, o1, o2 = _lo(w0), _hi(w0), _lo(w1), _hi(w1), _hi(w2)
        s0, s1, s2, s3 = (shift_buf[c, j:j + 1, :] for j in range(4))
        even = s3 * o2 + s2 * e1 + s1 * o1 + s0 * e0
        odd = s3 * e1 + s2 * o1 + s1 * e0 + s0 * o0
        vw = vs32[c, rows8(r, n), :]
        buf1[rows8(RES_OFF + c_out * (S // 2) + r, n), :] = pltpu.pack_elementwise(
            [even * _lo(vw), odd * _hi(vw)], packed_dtype=BF16)

    def forward_x(c, a):
        return _dot(_bf(f_buf[...]), _bf(buf1[rows8(RES_OFF + c * (S // 2) + a * HP, HP), :]))

    def forward_h(c, a):
        taps = _bf(hs32[c, :, pl.ds(pl.multiple_of(a * T, T), T)])
        return lax.dot_general(_bf(f_buf[...]), taps, NT_DIMS, preferred_element_type=F32)

    def product(c, g, odd, a0, b0, b1, acc, pin):
        def load(which, chunk):
            slot = (which * 2 + (c & 1)) * NB + chunk
            return spec[slot, rows8(g * 16, 8), :], spec[slot, rows8(g * 16 + 8, 8), :]

        pace = recent(CFG["plead"] - 8) if CFG["ppace"] else None
        if pace is not None:
            spec[(c >> 3) + 4 * NB, 0:8, :] = pace
        taps = {}
        for b in range(b0, b1):
            xr, xi = load(0, b)
            for a in range(max(a0, b), a0 + 2):
                if a - b not in taps:
                    taps[a - b] = load(1, a - b)
                hr, hi = taps[a - b]
                pr, pi = hr * xr - hi * xi, hr * xi + hi * xr
                acc[odd, a] = (acc[odd, a][0] + pr, acc[odd, a][1] + pi) if b else (pr, pi)
        for u, a in enumerate((a0, a0 + 1)):
            zr, zi = acc[odd, a]
            if b1 < a0 + 2:
                if CFG["pin"]:
                    pin(16 * u, pltpu.bitcast(zr, U32))
                    pin(16 * u + 8, pltpu.bitcast(zi, U32))
                continue
            if a:
                tr, ti = acc[odd, a - 1]
                zr, zi = (zr + ti, zi - tr) if odd else (zr - ti, zi + tr)
            if not odd:
                acc["mirror", a] = zr, zi
                pin(16 * u, pltpu.bitcast(zr, U32))
                pin(16 * u + 8, pltpu.bitcast(zi, U32))
                continue
            mr, mi = acc["mirror", a]
            for half, pair in enumerate(([mr + zr, mi - zi], [mr - zr, mi + zi])):
                y = pltpu.pack_elementwise(pair, packed_dtype=BF16)
                buf0[rows8(RES_OFF + (c * NB + a) * T + half * HP + (g >> 1) * 8, 8), :] = y
                pin(16 * u + 8 * half, y)

    small_cp = [pltpu.make_async_copy(src, dst, sem_small.at[i]) for i, (src, dst) in enumerate(
        ((sk_hbm, sk_ref), (fwd_hbm, fwd_ref), (inv_hbm, inv_ref), (gw_hbm, gw_ref), (d_hbm, d_ref)))]
    for cp in (w_cp(0) + [cp for n in range(len(ROW_CHUNKS) - 1) for cp in rows_cp(n)]
               + small_cp + conv_cp(0) + conv_cp(1) + w_cp(1)):
        cp.start()
    ks32[0:NC, 0:8, :] = jnp.zeros((NC, 8, T), U32)
    w_wait(0)
    for cp in rows_cp(0):
        cp.wait()
    for t in range(16):
        w_cur[0, pl.ds(t * HP, HP), :] = unpack_weights(jnp.int32(0), t)
    proj_q(zero_ref[0], (0, 0), 0)
    proj_k(zero_ref[0], (0, 0), 0)
    proj_q(zero_ref[0], (0, 0), 1)
    scores(zero_ref[0], 0, 0, 1)
    proj_k(zero_ref[0], (0, 0), 1)
    proj_v(zero_ref[0], (0, 0), 0)
    row_max(zero_ref[0], 0)

    def first_transforms():
        for cp in small_cp + conv_cp(0):
            cp.wait()
        f_buf[...] = pltpu.bitcast(fwd_ref[...], U32)
        shift_taps = sk_ref[...].astype(F32)
        for j in range(NC):
            shift_buf[j, 0:4, :] = shift_taps[:, j * T:(j + 1) * T]
        for a in range(NB):
            gate_kv(0, 0, a * HP // 8, HP)
            spec[a] = forward_x(0, a)
            spec[2 * NB + a] = forward_h(0, a)

    def head(h, first):
        c, quarter = h >> 2, h & 3
        cn = jnp.minimum(c + 1, NC - 1)
        hn = jnp.minimum(h + 1, H - 1)
        z = h >> 5

        def start_copies():
            if first:
                wo_cp.start()

            @pl.when(jnp.logical_and(quarter == 0, c + 2 < NC))
            def _():
                for cp in conv_cp(jnp.minimum(c + 2, NC - 1)):
                    cp.start()

            @pl.when(jnp.logical_and((h & 1) == 1, h + 3 < H))
            def _():
                for cp in w_cp(jnp.minimum((h >> 1) + 2, H // 2 - 1)):
                    cp.start()

        def wait_copies():
            @pl.when(jnp.logical_and(quarter == 3, c + 2 < NC))
            def _():
                for cp in conv_cp(jnp.minimum(c + 2, NC - 1)):
                    cp.wait()

            @pl.when(jnp.logical_and((h & 1) == 0, h + 2 < H))
            def _():
                w_wait((h >> 1) + 1)

        steps = _head_program(first)
        rounds = list(itertools.accumulate(st[0] == "round" for st in steps))
        stream.clear()
        w_cache.clear()
        users = [n for n, st in enumerate(steps) if st[0] in ("scores", "attend")]
        parity = [steps[n][1] % 2 for n in users]
        tasks = {n: [] for n in users}
        PB = CFG["pb"]
        pieces = [(gi, a0, b0, min(b0 + PB, a0 + 2))
                  for g0 in (0, 2) for a0 in range(0, NB, 2) for gi in (g0, g0 + 1)
                  for b0 in range(0, a0 + 2, PB)]
        hosts = [n for n, st in enumerate(steps)
                 if st[0] in (("scores", "attend"), ("scores",), ("attend",), ("scores", "attend", "q", "k", "v"),
                              ("k", "v"), ("q", "k", "v"))[CFG["where1" if first else "where"]]
                 and (not first or rounds[n] > CFG["c0"])]

        def pin_of(st):
            if st[0] in ("scores", "attend"):
                buf, slot = (k_buf if st[0] == "scores" else v_buf)[st[2]].bitcast(U32), z + 1
            elif CFG["pin"] == 2:
                buf, slot = dict(q=q_buf, k=k_buf, v=v_buf)[st[0]][st[1]].bitcast(U32), z + 1
            elif CFG["pin"] == 3:
                buf, slot = spec.bitcast(U32), z + 4 * NB
            else:
                buf, slot = w_cur, z + 2

            def pin(r, y):
                buf[slot, pl.ds(r, 8), :] = y
            return pin

        acc, held = {}, {}
        for u, (gi, a0, b0, b1) in enumerate(pieces if CFG['prod'] else []):
            n = hosts[int((u / len(pieces)) ** (1 if first else CFG['skew'] / 10) * len(hosts))]
            tasks.setdefault(n, []).append(functools.partial(
                product, c, quarter * 4 + gi, gi % 2, a0, b0, b1, acc, pin_of(steps[n])))

        def forward(name, fn, *args):
            held[name] = fn(*args)

        def spec_store(name, slot):
            spec[slot] = held.pop(name)

        late = [n for n in users if steps[n][0] == "attend" and steps[n][1] >= CFG["c1" if first else "fr"]]
        odd, even = ([n for n in late if steps[n][1] % 2 == par] for par in (1, 0))
        for u in range(4 * CFG['fwd']):
            a = quarter * 4 + u
            for r in range(4):
                tasks[odd[(5 * u + r) * len(odd) // 20]].append(
                    functools.partial(gate_kv, cn, c + 1, a * 8 + 2 * r, 16))
            for which, n, fn, tile in ((0, odd[(5 * u + 4) * len(odd) // 20], forward_x, c + 1),
                                       (1, even[u * len(even) // 4], forward_h, cn)):
                tasks[n].append(functools.partial(forward, (which, u), fn, tile, a))
                after = min(n + CFG["lag"], len(steps) - 1)
                tasks.setdefault(after, []).insert(0, functools.partial(
                    spec_store, (which, u), (which * 2 + ((c + 1) & 1)) * NB + a))

        for n, st in enumerate(steps):
            for task in tasks.get(n, ()):
                task()
            kind, i = st[:2]
            if CFG["opq"] and kind in ("scores", "attend"):
                z = (h + i) >> 6
            if kind == "weights":
                w_cur[(h + 1) & 1, pl.ds(i * HP, HP), :] = unpack_weights(hn, i)
            elif kind == "round":
                pass
            elif kind == "rows":
                for cp in rows_cp(i):
                    cp.wait()
            elif kind == "conv":
                for cp in conv_cp(1) if i else ():
                    cp.wait()
                if not i:
                    first_transforms()
            elif kind == "start":
                start_copies()
            elif kind == "wait":
                wait_copies()
            elif kind == "scores":
                scores(z, *st[1:])
            elif kind == "attend":
                attend(z, h, *st[1:])
            elif kind == "max":
                row_max(z, i)
            elif kind == "v":
                proj_v(z, (h, int(i == 0)), i)
            else:
                (proj_q if kind == "q" else proj_k)(z, (h, int(i < 2)), i)

    if CFG['peel']:
        head(zero_ref[0], True)
    if CFG["stop"] == 1:
        wo_cp.wait()
        for cp in conv_cp(2):
            cp.wait()
        return
    if CFG["unroll"] == 1:
        lax.fori_loop(1, H, lambda h, _: head(h, False), None)
    else:
        def two_heads(p, _):
            head(2 * p + 1, False)
            head(2 * p + 2, False)

        lax.fori_loop(0, H // 2 - 1, two_heads, None)
        head(zero_ref[0] + H - 1, False)
    if CFG["rep"] > 1:
        lax.fori_loop(0, 16, lambda h, _: head(jnp.maximum(h, H - 1), False), None)

    wo_cp.wait()
    if CFG['stop'] == 2:
        return
    f_buf[0:HP, :] = pltpu.bitcast(inv_ref[...], U32)
    gate_w = gw_ref[...].astype(F32).reshape(1, DM)
    skip_d = d_ref[...].astype(F32).reshape(1, DM)
    for j in range(NC):
        shift_buf[j, 0:1, :] = gate_w[:, j * T:(j + 1) * T]
        shift_buf[j, 1:2, :] = skip_d[:, j * T:(j + 1) * T]

    def out_cp(r, slot):
        return pltpu.make_async_copy(
            out_buf.at[slot], out_hbm.bitcast(U32).at[0, rows8(r * (RB // 2), RB // 2), :], sem_out.at[slot])

    def mix(r, carry):
        slot = r % 2
        rp = pl.ds(pl.multiple_of(r * (RB // 2), RB // 2), RB // 2)

        @pl.when(r >= 2)
        def _():
            out_cp(r - 2, slot).wait()

        for half, part in enumerate((_lo, _hi)):
            logit = None
            for j in range(NC):
                t = part(xs32[rp, lanes(j)]) * shift_buf[j, 0:1, :]
                logit = t if logit is None else logit + t
            gate = 1.0 / (1.0 + jnp.exp(-jnp.sum(logit, axis=1, keepdims=True)))
            g_buf[half] = jnp.broadcast_to(gate, (RB // 2, T))
        for j in range(NC):
            b = None
            for h0 in range(0, H, 4):
                lhs = jnp.concatenate(
                    [_bf(ctx32[rows8((h0 + u) * (S // 2) + r * (RB // 2), RB // 2), :]) for u in range(4)],
                    axis=1)
                t = _dot(lhs, _bf(wo32[pl.ds(h0 * HP, 4 * HP), lanes(j)]))
                b = t if b is None else b + t
            b_buf[j] = b
            halves = []
            for half, part in enumerate((_lo, _hi)):
                y = jnp.concatenate(
                    [_dot(_bf(f_buf[half * HP // 2:(half + 1) * HP // 2, :]),
                          _bf(buf0[rows8(RES_OFF + (j * NB + r * (RB // T) + u) * T + half * HP, HP), :]))
                     for u in range(RB // T)], axis=0)
                kv = part(buf1[rows8(RES_OFF + j * (S // 2) + r * (RB // 2), RB // 2), :])
                a = part(xs32[rp, lanes(j)]) * (y + kv * shift_buf[j, 1:2, :])
                g = g_buf[half]
                halves.append(g * a + (1.0 - g) * b_buf[j, pl.ds(half, RB // 2, stride=2), :])
            out_buf[slot, :, lanes(j)] = pltpu.pack_elementwise(halves, packed_dtype=BF16)
        out_cp(r, slot).start()
        return carry

    lax.fori_loop(0, S // RB, mix, 0)
    for r in (S // RB - 2, S // RB - 1):
        out_cp(r, r % 2).wait()


@jax.jit
def pallas_gated_mix__ssm_conv_h3__compressed_kv_cla__prompt_kernel(
    A_q, A_k, A_v, A_shift_k, A_ssm_k, A_ssm_D, B_x, B_c_kv, B_w_q, B_w_uk, B_w_uv, B_w_o, gate_w,
):
    del B_x
    hbm = pl.BlockSpec(memory_space=pl.ANY)
    scratch = [
        pltpu.VMEM((4, DM), BF16),
        pltpu.VMEM((DM,), BF16),
        pltpu.VMEM((DM,), BF16),
        pltpu.VMEM(_FWD.shape, BF16),
        pltpu.VMEM(_INV.shape, BF16),
        pltpu.VMEM((S // 2, DM), U32),
        pltpu.VMEM((S // 2, DC), U32),
        pltpu.VMEM((2, DM + 2 * DC, T), U32),
        pltpu.VMEM((H * HP, DM), U32),
        pltpu.VMEM((NC + 1, K_PITCH, T), U32),
        pltpu.VMEM((NC, S // 2, T), U32),
        pltpu.VMEM((NC, HP, S), U32),
        pltpu.VMEM((4 * NB + 1, 2 * T, T), F32),
        pltpu.VMEM((3, 16 * HP, T), U32),
        pltpu.VMEM((RES_OFF + NC * S, T), U32),
        pltpu.VMEM((RES_OFF + (NC + 1) * S // 2, T), U32),
        pltpu.VMEM((1, T, T), F32),
        pltpu.VMEM((1, T, T), F32),
        pltpu.VMEM((1, T, T), F32),
        pltpu.VMEM((H * S + 4 * T + 16, T), BF16),
        pltpu.VMEM((NC, 8, T), F32),
        pltpu.VMEM((T, T), U32),
        pltpu.VMEM((2, RB // 2, T), F32),
        pltpu.VMEM((NC, RB, T), F32),
        pltpu.VMEM((2, RB // 2, DM), U32),
        pltpu.SemaphoreType.DMA((5,)),
        pltpu.SemaphoreType.DMA((2, len(ROW_CHUNKS) - 1)),
        pltpu.SemaphoreType.DMA((2,)),
        pltpu.SemaphoreType.DMA((1,)),
        pltpu.SemaphoreType.DMA((3, 2)),
        pltpu.SemaphoreType.DMA((2,)),
    ] + [pltpu.VMEM((2, T, T), BF16)] * (3 * NB)
    return pl.pallas_call(
        _kernel,
        out_shape=jax.ShapeDtypeStruct((1, S, DM), BF16),
        in_specs=[pl.BlockSpec(memory_space=pltpu.SMEM), *[hbm] * 14],
        out_specs=hbm,
        scratch_shapes=scratch,
        compiler_params=pltpu.CompilerParams(
            vmem_limit_bytes=110 * 1024 * 1024, disable_bounds_checks=bool(CFG['nobc']),
            flags={k: True for k, on in (("XLA_TPU_FORCE_LP_LLO_SCHEDULER", CFG["lp"]),
                                         ("XLA_TPU_EVENLY_DISTRIBUTE_CRITICAL_NODES", CFG["even"]),
                                         ("XLA_TPU_RESCHEDULE_DMA_DONES", CFG["rdd"])) if on}),
        name="gated_mix_h3_cla",
    )(
        np.zeros((1,), np.int32), A_q, A_k, A_v, A_shift_k.T, A_ssm_k, A_ssm_D, B_c_kv,
        B_w_q, B_w_uk, B_w_uv, B_w_o.reshape(H * DH, DM), gate_w, _FWD, _INV,
    )
```

```python
import functools
import math

import jax
import jax.numpy as jnp
import numpy as np
from jax import lax
import jax.experimental.pallas as pl
import jax.experimental.pallas.tpu as pltpu

S = 2048
DM = 1024
H = 32
DH = 128
DC = 512
T = 128
HP = T // 2
NB = S // T
NC = DM // T
KG = 4
SLAB = 32
RB = 256

MAX_OFF = H * S // 2
RES_OFF = NB * T

ROW_CHUNKS = (0, 2, 4, 6, 9, 12, 16)
TILE0_ROUND, TILE1_ROUND = 11, 13

F32, BF16, U32 = jnp.float32, jnp.bfloat16, jnp.uint32
Q_SCALE = (DH ** -0.5) * math.log2(math.e)
NEG = -1e30
NT_DIMS = (((1,), (1,)), ((), ()))


def _dft_matrices():
    even = 2 * np.arange(64).reshape(8, 8)
    f = np.stack([even, 127 - even], axis=1).reshape(16, 8)
    th = 2.0 * np.pi * (f[..., None] + 0.5) * np.arange(T) / (2 * T)
    fwd = np.stack([np.cos(th), -np.sin(th)], axis=1).reshape(2 * T, T)
    inv = np.stack([np.cos(th[0::2]), -np.sin(th[0::2])], axis=2).reshape(T, T).T / T
    return fwd.astype(BF16), np.concatenate([inv[0::2], inv[1::2]]).astype(BF16)


_FWD, _INV = _dft_matrices()


def _bf(words):
    return pltpu.bitcast(words, BF16)


def _lo(words):
    return pltpu.bitcast(words << 16, F32)


def _hi(words):
    return pltpu.bitcast(words & jnp.uint32(0xFFFF0000), F32)


def _dot(a, b):
    return jnp.dot(a, b, preferred_element_type=F32)


def _key_groups(i):
    return [(j0, min(KG, i + 1 - j0)) for j0 in range(0, i + 1, KG)]


def _head_program():
    steps = []
    for i in range(NB):
        nxt = (i + 1) % NB
        sc = [("scores", nxt) + grp for grp in _key_groups(nxt)]
        at = [("attend", i) + grp for grp in _key_groups(i)]
        q, k, v, mx = ("q", (i + 2) % NB), ("k", (i + 2) % NB), ("v", nxt), ("max", nxt)
        rnd = [st for u in range(NB // KG) for st in sc[u:u + 1] + at[u:u + 1]]
        if i < NB - 2:
            rnd = [q] + rnd[:1] + [k] + rnd[1:3] + [v] + rnd[3:] + [mx]
        elif i == NB - 2:
            rnd = [v] + rnd + [mx, q, k]
        else:
            rnd = [at[0], q, at[1], k, at[2], sc[0], at[3], v, mx]
        steps += [(i,) + st for st in rnd[:2] + [("weights", i)] + rnd[2:]]
    return steps


def _kernel(zero_ref, x_hbm, k_hbm, v_hbm, sk_hbm, h_hbm, d_hbm, c_hbm, wq_hbm, wk_hbm, wv_hbm,
            wo_hbm, gw_hbm, fwd_hbm, inv_hbm, out_hbm,
            sk_buf, d_buf, gw_buf, fwd_buf, inv_buf,
            xs, cs, w_raw, wo, ks, vs, hs, spec, w_cur, buf0, buf1, mx_buf, l_buf, o_buf,
            ctx, row_buf, f_buf, g_buf, b_buf, out_buf,
            sem_small, sem_rows, sem_w, sem_wo, sem_conv, sem_out, *qkv):
    q_buf, k_buf, v_buf = qkv[:NB], qkv[NB:2 * NB], qkv[2 * NB:]
    x_hbm, k_hbm, v_hbm, h_hbm, c_hbm, wq_hbm, wk_hbm, wv_hbm, wo_hbm, out_hbm = (
        r.bitcast(U32) for r in
        (x_hbm, k_hbm, v_hbm, h_hbm, c_hbm, wq_hbm, wk_hbm, wv_hbm, wo_hbm, out_hbm))
    bufs = (buf0, buf1)
    ctx32, m_buf = ctx.bitcast(U32), ctx.bitcast(F32)

    def lanes(j):
        return pl.ds(j * T, T)

    def rows8(start, n):
        return pl.ds(start if isinstance(start, int) else pl.multiple_of(start, 8), n)

    small_cp = [pltpu.make_async_copy(src, dst, sem_small.at[i]) for i, (src, dst) in enumerate(
        ((sk_hbm, sk_buf), (fwd_hbm, fwd_buf), (inv_hbm, inv_buf), (gw_hbm, gw_buf), (d_hbm, d_buf)))]
    wo_cp = pltpu.make_async_copy(wo_hbm, wo, sem_wo.at[0])

    def rows_cp(n):
        rows = pl.ds(ROW_CHUNKS[n] * HP, (ROW_CHUNKS[n + 1] - ROW_CHUNKS[n]) * HP)
        return [pltpu.make_async_copy(src.at[0, rows], dst.at[rows], sem_rows.at[i, n])
                for i, (src, dst) in enumerate(((c_hbm, cs), (x_hbm, xs)))]

    def w_cp(p):
        return [pltpu.make_async_copy(src.at[:, p, :], w_raw.at[p & 1, pl.ds(r0, n)], sem_w.at[p & 1])
                for src, r0, n in ((wq_hbm, 0, DM), (wk_hbm, DM, DC), (wv_hbm, DM + DC, DC))]

    def w_wait(p):
        pltpu.make_async_copy(w_raw.at[p & 1], w_raw.at[p & 1], sem_w.at[p & 1]).wait()

    def conv_cp(c):
        col = pl.ds(pl.multiple_of(c * T, T), T)
        return [
            pltpu.make_async_copy(k_hbm.at[0, :, col], ks.at[c, pl.ds(8, S // 2)], sem_conv.at[0, c & 1]),
            pltpu.make_async_copy(v_hbm.at[0, :, col], vs.at[c], sem_conv.at[1, c & 1]),
            pltpu.make_async_copy(h_hbm.at[pl.ds(pl.multiple_of(c * HP, HP), HP)], hs.at[c],
                                  sem_conv.at[2, c & 1]),
        ]

    stream = []
    w_cache = {}

    def recent(slab):
        return stream[-3][16 * slab + 8:16 * slab + 16, 0:T] if len(stream) >= 3 else None

    def unpack_weights(h, t):
        slot = (h >> 1) & 1
        sh = ((h & 1) * 16).astype(U32)
        even = w_raw[slot, pl.ds(t * T, HP, stride=2), :]
        odd = w_raw[slot, pl.ds(t * T + 1, HP, stride=2), :]
        return ((even >> sh) & jnp.uint32(0xFFFF)) | ((odd >> sh) << 16)

    def project(src, i, j0, h, ahead, t0):
        lhs = jnp.concatenate([_bf(src[pl.ds(i * HP, HP), lanes(j0 + j)]) for j in range(4)], axis=1)
        if (ahead, t0) not in w_cache:
            w_cache[ahead, t0] = _bf(w_cur[(h + ahead) & 1, pl.ds(t0 * HP, 4 * HP), :])
        stream.append(_dot(lhs, w_cache[ahead, t0]))
        return stream[-1]

    def proj_q(z, h, ahead, i):
        q = project(xs, i, 0, h, ahead, 0) + project(xs, i, 4, h, ahead, 4)
        q_buf[i][z] = (q * Q_SCALE).astype(BF16)

    def proj_k(z, h, ahead, i):
        k_buf[i][z] = project(cs, i, 0, h, ahead, 8).astype(BF16)

    def proj_v(z, h, ahead, i):
        v_buf[i][z] = project(cs, i, 0, h, ahead, 12).astype(BF16)

    def tiles_of(buf, j0, n):
        return _bf(jnp.concatenate([buf[j0 + j].bitcast(U32)[0] for j in range(n)], axis=0))

    def scores(z, i, j0, n):
        s = lax.dot_general(tiles_of(q_buf, i, 1), tiles_of(k_buf, j0, n), NT_DIMS,
                            preferred_element_type=F32)
        stream.append(s)
        diff = (lax.broadcasted_iota(jnp.int32, (SLAB, T), 1)
                - lax.broadcasted_iota(jnp.int32, (SLAB, T), 0))
        for r in range(0, T, SLAB):
            mx = None if j0 == 0 else mx_buf[0, r:r + SLAB, :]
            for j in range(n):
                t = s[r:r + SLAB, j * T:(j + 1) * T]
                if j0 + j == i:
                    t = jnp.where(diff <= r, t, NEG)
                bufs[i % 2][rows8(z + (j0 + j) * T + r, SLAB), :] = pltpu.bitcast(t, U32)
                mx = t if mx is None else jnp.maximum(mx, t)
            mx_buf[z, r:r + SLAB, :] = mx

    def row_max(z, i):
        m_buf[rows8(z + MAX_OFF + i % 2 * T, T), :] = jnp.broadcast_to(
            jnp.max(mx_buf[0], axis=1, keepdims=True), (T, T))

    def attend(z, h, i, j0, n):
        last = j0 + n == i + 1
        slabs, scale = [], []
        for r in range(0, T, SLAB):
            pace = recent(r // 16 + 1)
            if pace is not None:
                m_buf[rows8(z + MAX_OFF + 2 * T, 8), :] = pace
            m = m_buf[rows8(MAX_OFF + i % 2 * T + r, SLAB), :]
            l = None if j0 == 0 else l_buf[0, r:r + SLAB, :]
            ps = []
            for j in range(n):
                p = jnp.exp2(pltpu.bitcast(bufs[i % 2][rows8((j0 + j) * T + r, SLAB), :], F32) - m)
                l = p if l is None else l + p
                ps.append(p)
            slabs.append(jnp.concatenate(ps, axis=1))
            if last:
                total = jnp.sum(l, axis=1, keepdims=True)
                rcp = pl.reciprocal(total, approx=True)
                scale.append(rcp * (2.0 - total * rcp))
            else:
                l_buf[z, r:r + SLAB, :] = l
        o = _dot(jnp.concatenate(slabs, axis=0).astype(BF16), tiles_of(v_buf, j0, n))
        stream.append(o)
        for r in range(0, T, SLAB):
            t = o[r:r + SLAB]
            if j0 > 0:
                t = t + o_buf[0, r:r + SLAB, :]
            if last:
                ctx[pl.ds(pl.multiple_of(h * S + i * T + r, SLAB), SLAB), :] = (
                    t * scale[r // SLAB]).astype(BF16)
            else:
                o_buf[z, r:r + SLAB, :] = t

    def gate_kv(z, c, c_out, r, n):
        pace = None if z is None else recent(0)
        if pace is not None:
            ks[z + NC, 0:8, :] = pltpu.bitcast(pace, U32)
        w0, w1, w2 = ks[c, rows8(r + 8, n), :], ks[c, pl.ds(r + 7, n), :], ks[c, pl.ds(r + 6, n), :]
        e0, o0, e1, o1, o2 = _lo(w0), _hi(w0), _lo(w1), _hi(w1), _hi(w2)
        s0, s1, s2, s3 = (row_buf[c, j:j + 1, :] for j in range(4))
        even = s3 * o2 + s2 * e1 + s1 * o1 + s0 * e0
        odd = s3 * e1 + s2 * o1 + s1 * e0 + s0 * o0
        vw = vs[c, rows8(r, n), :]
        buf1[rows8(RES_OFF + c_out * (S // 2) + r, n), :] = pltpu.pack_elementwise(
            [even * _lo(vw), odd * _hi(vw)], packed_dtype=BF16)

    def forward_x(c, a):
        return _dot(_bf(f_buf[...]), _bf(buf1[rows8(RES_OFF + c * (S // 2) + a * HP, HP), :]))

    def forward_h(c, a):
        taps = _bf(hs[c, :, pl.ds(pl.multiple_of(a * T, T), T)])
        return lax.dot_general(_bf(f_buf[...]), taps, NT_DIMS, preferred_element_type=F32)

    def product(z, c, g, odd, a0, b0, acc, pin):
        def load(which, chunk):
            slot = (which * 2 + (c & 1)) * NB + chunk
            return spec[slot, rows8(g * 16, 8), :], spec[slot, rows8(g * 16 + 8, 8), :]

        pace = recent(2)
        if pace is not None:
            spec[z + 4 * NB, 0:8, :] = pace
        taps = {}
        for b in (b0, b0 + 1):
            xr, xi = load(0, b)
            for a in range(max(a0, b), a0 + 2):
                if a - b not in taps:
                    taps[a - b] = load(1, a - b)
                hr, hi = taps[a - b]
                pr, pi = hr * xr - hi * xi, hr * xi + hi * xr
                acc[odd, a] = (acc[odd, a][0] + pr, acc[odd, a][1] + pi) if b else (pr, pi)
        for u, a in enumerate((a0, a0 + 1)):
            zr, zi = acc[odd, a]
            if b0 == a0 and a:
                tr, ti = acc[odd, a - 1]
                zr, zi = (zr + ti, zi - tr) if odd else (zr - ti, zi + tr)
            if b0 == a0 and odd:
                mr, mi = acc["mirror", a]
                for half, pair in enumerate(([mr + zr, mi - zi], [mr - zr, mi + zi])):
                    y = pltpu.pack_elementwise(pair, packed_dtype=BF16)
                    buf0[rows8(RES_OFF + (c * NB + a) * T + half * HP + (g >> 1) * 8, 8), :] = y
                    pin[z + 1, pl.ds(16 * u + 8 * half, 8), :] = y
            else:
                if not odd:
                    acc["mirror", a] = zr, zi
                pin[z + 1, pl.ds(16 * u, 8), :] = pltpu.bitcast(zr, U32)
                pin[z + 1, pl.ds(16 * u + 8, 8), :] = pltpu.bitcast(zi, U32)

    def first_transforms():
        for cp in small_cp + conv_cp(0):
            cp.wait()
        f_buf[...] = pltpu.bitcast(fwd_buf[...], U32)
        shift_taps = sk_buf[...].astype(F32)
        for j in range(NC):
            row_buf[j, 0:4, :] = shift_taps[:, j * T:(j + 1) * T]
        for a in range(NB):
            gate_kv(None, 0, 0, a * HP, HP)
            spec[a] = forward_x(0, a)
            spec[2 * NB + a] = forward_h(0, a)

    ks[0:NC, 0:8, :] = jnp.zeros((NC, 8, T), U32)
    for cp in (w_cp(0) + [cp for n in range(len(ROW_CHUNKS) - 1) for cp in rows_cp(n)]
               + small_cp + conv_cp(0) + conv_cp(1) + w_cp(1)):
        cp.start()
    w_wait(0)
    for cp in rows_cp(0):
        cp.wait()
    for t in range(2 * NC):
        w_cur[0, pl.ds(t * HP, HP), :] = unpack_weights(jnp.int32(0), t)
    zero = zero_ref[0]
    proj_q(zero, 0, 0, 0)
    proj_k(zero, 0, 0, 0)
    proj_q(zero, 0, 0, 1)
    scores(zero, 0, 0, 1)
    proj_k(zero, 0, 0, 1)
    proj_v(zero, 0, 0, 0)
    row_max(zero, 0)

    def head(h, first):
        c, quarter = h >> 2, h & 3
        cn = jnp.minimum(c + 1, NC - 1)
        hn = jnp.minimum(h + 1, H - 1)
        z = h >> 5
        steps = _head_program()
        stream.clear()
        w_cache.clear()

        tasks = [[] for _ in steps]
        acc, held = {}, {}
        hosts = [n for n, st in enumerate(steps)
                 if (st[0] >= TILE0_ROUND and st[1] not in ("weights", "max") if first
                     else st[1] in ("q", "k", "v"))]
        pieces = [(gi, a0, b0) for g0 in (0, 2) for a0 in range(0, NB, 2) for gi in (g0, g0 + 1)
                  for b0 in range(0, a0 + 2, 2)]
        for u, (gi, a0, b0) in enumerate(pieces):
            n = hosts[int((u / len(pieces)) ** (1.0 if first else 1.5) * len(hosts))]
            kind, block = steps[n][1], steps[n][2:4][-1 if steps[n][1] in ("scores", "attend") else 0]
            pin = dict(q=q_buf, k=k_buf, v=v_buf, scores=k_buf, attend=v_buf)[kind][block]
            tasks[n].append(functools.partial(
                product, z, c, quarter * 4 + gi, gi % 2, a0, b0, acc, pin.bitcast(U32)))

        def forward(name, fn, *args):
            held[name] = fn(*args)

        def spec_store(name, slot):
            spec[slot] = held.pop(name)

        late = [n for n, st in enumerate(steps)
                if st[1] == "attend" and (TILE1_ROUND if first else 2) <= st[0] < NB - 1]
        odd, even = ([n for n in late if steps[n][0] % 2 == par] for par in (1, 0))
        for u in range(4):
            a = quarter * 4 + u
            for r in range(4):
                tasks[odd[(5 * u + r) * len(odd) // 20]].append(
                    functools.partial(gate_kv, z, cn, c + 1, a * HP + 16 * r, 16))
            for which, n, fn, tile in ((0, odd[(5 * u + 4) * len(odd) // 20], forward_x, c + 1),
                                       (1, even[u * len(even) // 4], forward_h, cn)):
                tasks[n].append(functools.partial(forward, (which, u), fn, tile, a))
                done = n + 5 - (steps[n + 4][0] - steps[n][0])
                tasks[done].insert(0, functools.partial(
                    spec_store, (which, u), (which * 2 + ((c + 1) & 1)) * NB + a))

        for n, (i, kind, block, *group) in enumerate(steps):
            if first and (n == 0 or steps[n - 1][0] != i):
                if i + 2 in ROW_CHUNKS[1:-1]:
                    for cp in rows_cp(ROW_CHUNKS.index(i + 2)):
                        cp.wait()
                if i == TILE0_ROUND:
                    first_transforms()
                if i == TILE1_ROUND:
                    for cp in conv_cp(1):
                        cp.wait()
            for task in tasks[n]:
                task()
            if kind == "weights":
                w_cur[(h + 1) & 1, pl.ds(i * HP, HP), :] = unpack_weights(hn, i)
            elif kind == "scores":
                scores(z, block, *group)
            elif kind == "attend":
                attend(z, h, block, *group)
            elif kind == "max":
                row_max(z, block)
            else:
                dict(q=proj_q, k=proj_k, v=proj_v)[kind](z, h, int(block < i), block)

        if first:
            wo_cp.start()

        @pl.when(jnp.logical_and(quarter == 0, c + 2 < NC))
        def _():
            for cp in conv_cp(jnp.minimum(c + 2, NC - 1)):
                cp.start()

        @pl.when(jnp.logical_and((h & 1) == 1, h + 3 < H))
        def _():
            for cp in w_cp(jnp.minimum((h >> 1) + 2, H // 2 - 1)):
                cp.start()

        @pl.when(jnp.logical_and(quarter == 3, c + 2 < NC))
        def _():
            for cp in conv_cp(jnp.minimum(c + 2, NC - 1)):
                cp.wait()

        @pl.when(jnp.logical_and((h & 1) == 0, h + 2 < H))
        def _():
            w_wait((h >> 1) + 1)

    head(zero, True)
    lax.fori_loop(1, H, lambda h, _: head(h, False), None)

    wo_cp.wait()
    f_buf[0:HP, :] = pltpu.bitcast(inv_buf[...], U32)
    gate_w = gw_buf[...].astype(F32).reshape(1, DM)
    skip_d = d_buf[...].astype(F32).reshape(1, DM)
    for j in range(NC):
        row_buf[j, 0:1, :] = gate_w[:, j * T:(j + 1) * T]
        row_buf[j, 1:2, :] = skip_d[:, j * T:(j + 1) * T]

    def out_cp(r, slot):
        return pltpu.make_async_copy(
            out_buf.at[slot], out_hbm.at[0, rows8(r * (RB // 2), RB // 2), :], sem_out.at[slot])

    def mix(r, _):
        slot = r % 2
        rp = pl.ds(pl.multiple_of(r * (RB // 2), RB // 2), RB // 2)

        @pl.when(r >= 2)
        def _():
            out_cp(r - 2, slot).wait()

        for half, part in enumerate((_lo, _hi)):
            logit = None
            for j in range(NC):
                t = part(xs[rp, lanes(j)]) * row_buf[j, 0:1, :]
                logit = t if logit is None else logit + t
            gate = 1.0 / (1.0 + jnp.exp(-jnp.sum(logit, axis=1, keepdims=True)))
            g_buf[half] = jnp.broadcast_to(gate, (RB // 2, T))
        for j in range(NC):
            b = None
            for h0 in range(0, H, 4):
                lhs = jnp.concatenate(
                    [_bf(ctx32[rows8((h0 + u) * (S // 2) + r * (RB // 2), RB // 2), :])
                     for u in range(4)], axis=1)
                t = _dot(lhs, _bf(wo[pl.ds(h0 * HP, 4 * HP), lanes(j)]))
                b = t if b is None else b + t
            b_buf[j] = b
            halves = []
            for half, part in enumerate((_lo, _hi)):
                y = jnp.concatenate(
                    [_dot(_bf(f_buf[half * HP // 2:(half + 1) * HP // 2, :]),
                          _bf(buf0[rows8(RES_OFF + (j * NB + r * (RB // T) + u) * T + half * HP, HP), :]))
                     for u in range(RB // T)], axis=0)
                kv = part(buf1[rows8(RES_OFF + j * (S // 2) + r * (RB // 2), RB // 2), :])
                a = part(xs[rp, lanes(j)]) * (y + kv * row_buf[j, 1:2, :])
                g = g_buf[half]
                halves.append(g * a + (1.0 - g) * b_buf[j, pl.ds(half, RB // 2, stride=2), :])
            out_buf[slot, :, lanes(j)] = pltpu.pack_elementwise(halves, packed_dtype=BF16)
        out_cp(r, slot).start()

    lax.fori_loop(0, S // RB, mix, None)
    for r in (S // RB - 2, S // RB - 1):
        out_cp(r, r % 2).wait()


@jax.jit
def pallas_gated_mix__ssm_conv_h3__compressed_kv_cla__prompt_kernel(
    A_q: jax.Array,
    A_k: jax.Array,
    A_v: jax.Array,
    A_shift_k: jax.Array,
    A_ssm_k: jax.Array,
    A_ssm_D: jax.Array,
    B_x: jax.Array,
    B_c_kv: jax.Array,
    B_w_q: jax.Array,
    B_w_uk: jax.Array,
    B_w_uv: jax.Array,
    B_w_o: jax.Array,
    gate_w: jax.Array,
):
    del B_x
    hbm = pl.BlockSpec(memory_space=pl.ANY)
    scratch = [
        pltpu.VMEM((4, DM), BF16),
        pltpu.VMEM((DM,), BF16),
        pltpu.VMEM((DM,), BF16),
        pltpu.VMEM(_FWD.shape, BF16),
        pltpu.VMEM(_INV.shape, BF16),
        pltpu.VMEM((S // 2, DM), U32),
        pltpu.VMEM((S // 2, DC), U32),
        pltpu.VMEM((2, DM + 2 * DC, T), U32),
        pltpu.VMEM((H * HP, DM), U32),
        pltpu.VMEM((NC + 1, 8 + S // 2, T), U32),
        pltpu.VMEM((NC, S // 2, T), U32),
        pltpu.VMEM((NC, HP, S), U32),
        pltpu.VMEM((4 * NB + 1, 2 * T, T), F32),
        pltpu.VMEM((2, 2 * NC * HP, T), U32),
        pltpu.VMEM((RES_OFF + NC * S, T), U32),
        pltpu.VMEM((RES_OFF + (NC + 1) * S // 2, T), U32),
        pltpu.VMEM((1, T, T), F32),
        pltpu.VMEM((1, T, T), F32),
        pltpu.VMEM((1, T, T), F32),
        pltpu.VMEM((H * S + 4 * T + 16, T), BF16),
        pltpu.VMEM((NC, 8, T), F32),
        pltpu.VMEM((T, T), U32),
        pltpu.VMEM((2, RB // 2, T), F32),
        pltpu.VMEM((NC, RB, T), F32),
        pltpu.VMEM((2, RB // 2, DM), U32),
        pltpu.SemaphoreType.DMA((5,)),
        pltpu.SemaphoreType.DMA((2, len(ROW_CHUNKS) - 1)),
        pltpu.SemaphoreType.DMA((2,)),
        pltpu.SemaphoreType.DMA((1,)),
        pltpu.SemaphoreType.DMA((3, 2)),
        pltpu.SemaphoreType.DMA((2,)),
    ] + [pltpu.VMEM((2, T, T), BF16)] * (3 * NB)
    return pl.pallas_call(
        _kernel,
        out_shape=jax.ShapeDtypeStruct((1, S, DM), BF16),
        in_specs=[pl.BlockSpec(memory_space=pltpu.SMEM)] + [hbm] * 14,
        out_specs=hbm,
        scratch_shapes=scratch,
        compiler_params=pltpu.CompilerParams(
            vmem_limit_bytes=96 * 1024 * 1024, disable_bounds_checks=True),
        name="gated_mix_h3_cla",
    )(
        np.zeros((1,), np.int32), A_q, A_k, A_v, A_shift_k.T, A_ssm_k, A_ssm_D, B_c_kv,
        B_w_q, B_w_uk, B_w_uv, B_w_o.reshape(H * DH, DM), gate_w, _FWD, _INV,
    )
```
